```python
import jax
import jax.numpy as jnp

def _softmax(x, axis=-1):
    return jax.nn.softmax(x, axis=axis)
def _gelu(x):
    return jax.nn.gelu(x, approximate=True)
def _silu(x):
    return jax.nn.silu(x)
def _sigmoid(x):
    return jax.nn.sigmoid(x)
def _layernorm(x, axis=-1, eps=1e-5):
    m = jnp.mean(x, axis=axis, keepdims=True)
    v = jnp.var(x, axis=axis, keepdims=True)
    return (x - m) / jnp.sqrt(v + eps)
def _scatter_add(tgt, idx, src, axis=0):
    return tgt.at[idx].add(src)
def _segment_sum(src, seg, n):
    return jax.ops.segment_sum(src, seg, n)
class _Rng:
    def __init__(self, key):
        self._k = key
    def _next(self):
        self._k, sub = jax.random.split(self._k)
        return sub
    def normal(self, shape):
        return jax.random.normal(self._next(), shape, dtype=jnp.bfloat16)
    def randint(self, lo, hi, shape):
        return jax.random.randint(self._next(), shape, lo, hi, dtype=jnp.int32)
    def uniform(self, shape, lo=0.0, hi=1.0):
        return jax.random.uniform(self._next(), shape, jnp.bfloat16, lo, hi)
    def permutation(self, n):
        return jax.random.permutation(self._next(), n)


kernel_name = 'gated_mix__sliding_local_dilated__moe_arch_mod__prompt'

def setup_inputs():
    _rng = _Rng(jax.random.key(int.from_bytes(__import__("os").urandom(4), "little")))
    _w = (lambda a: (lambda t: t.astype(jnp.bfloat16) if jnp.issubdtype(t.dtype, jnp.floating) else t)(jnp.asarray(a)))
    def _A_setup():
        B, S, D = 1, 2048, 640
        return {
            "x": _w((lambda *s: _rng.normal(s) * 0.05)(B, S, D)),
            "wqkv": _w((lambda *s: _rng.normal(s) * 0.05)(D, 3 * D)),
            "wo": _w((lambda *s: _rng.normal(s) * 0.05)(D, D)),
        }
    _A_in = _A_setup()

    def _B_setup():
        B, S, D, F, C = 1, 2048, 640, 1728, 2
        return {
            "x": _w((lambda *s: _rng.normal(s) * 0.05)(B, S, D)),
            "w_r": _w((lambda *s: _rng.normal(s) * 0.05)(D)),
            "w_gate": _w((lambda *s: _rng.normal(s) * 0.05)(D, F)),
            "w_up": _w((lambda *s: _rng.normal(s) * 0.05)(D, F)),
            "w_down": _w((lambda *s: _rng.normal(s) * 0.05)(F, D)),
        }
    _B_in = _B_setup()

    return {
        "A_x": _A_in["x"],
        "A_wqkv": _A_in["wqkv"],
        "A_wo": _A_in["wo"],
        "B_x": _B_in["x"],
        "B_w_r": _B_in["w_r"],
        "B_w_gate": _B_in["w_gate"],
        "B_w_up": _B_in["w_up"],
        "B_w_down": _B_in["w_down"],
        "gate_w": _w((lambda *s: _rng.normal(s) * 0.05)(640)),
    }

def reference(A_x, A_wqkv, A_wo, B_x, B_w_r, B_w_gate, B_w_up, B_w_down, gate_w):
    def _A_ref(x, wqkv, wo):
        B, S, D = x.shape
        H = 32; Dh = D // H
        W, dil = 8, 2
        qkv = (lambda x, *d: x.transpose(*d))((x @ wqkv).reshape(B, S, 3, H, Dh), 2, 0, 3, 1, 4)
        q, k, v = qkv[0], qkv[1], qkv[2]
        scale = Dh ** -0.5
        pos = jnp.arange(S)
        off = jnp.arange(W) * dil
        idx = pos[:, None] - off[None, :]
        mask = idx >= 0
        idx_c = jnp.where(mask, idx, 0).reshape(-1)
        kg = k[:, :, idx_c, :].reshape(B, H, S, W, Dh)
        vg = v[:, :, idx_c, :].reshape(B, H, S, W, Dh)
        logits = jnp.einsum("bhsd,bhswd->bhsw", q, kg) * scale
        logits = jnp.where(mask[None, None, :, :], logits, -1e9)
        attn = _softmax(logits, axis=-1)
        o = jnp.einsum("bhsw,bhswd->bhsd", attn, vg)
        return (lambda x, *d: x.transpose(*d))(o, 0, 2, 1, 3).reshape(B, S, D) @ wo

    def _B_ref(x, w_r, w_gate, w_up, w_down):
        B, S, D = x.shape
        C = 2
        r = x @ w_r
        idx = jnp.argsort(-r, axis=-1)[:, :C]
        idx_e = jnp.repeat(idx.reshape(B, C, 1), D, axis=2)
        x_sel = jnp.take_along_axis(x, idx_e, axis=1)
        g = _silu(x_sel @ w_gate)
        u = x_sel @ w_up
        y = (g * u) @ w_down
        r_sel = _sigmoid(jnp.take_along_axis(r, idx, axis=1))
        y = y * r_sel.reshape(B, C, 1)
        b_off = (jnp.arange(B) * S).reshape(B, 1)
        flat_idx = (idx + b_off).reshape(B * C)
        zero = (x * 0.0).reshape(B * S, D)
        upd = _scatter_add(zero, flat_idx, y.reshape(B * C, D), axis=0)
        return x + upd.reshape(B, S, D)

    x = A_x
    g = _sigmoid((x * gate_w).sum(-1, keepdims=True))
    a = _A_ref(x, A_wqkv, A_wo)
    b = _B_ref(x, B_w_r, B_w_gate, B_w_up, B_w_down)
    return g * a + (1 - g) * b
```

```python
import numpy as np

import jax
import jax.numpy as jnp
from jax import lax
import jax.experimental.pallas as pl
import jax.experimental.pallas.tpu as pltpu

S, D, F = 2048, 640, 1728
H, DH = 32, 20
WIN, DIL = 8, 2
HALO = 16
L = 128
NJ = D // L
TM = 256
NT = S // TM
RB = 16
LAG = 1
SCALE = float(DH) ** -0.5
LOG2E = float(np.log2(np.e))
FFN_STEPS = (2, 3, 4, 5, 6, 7)

f32, bf16, u32 = jnp.float32, jnp.bfloat16, jnp.uint32


def _interleave(*streams):
    items = []
    for si, st in enumerate(streams):
        n = len(st)
        items += [((i + 0.5) / n, si, fn) for i, fn in enumerate(st)]
    items.sort(key=lambda it: (it[0], it[1]))
    for _, _, fn in items:
        fn()


def _pipelined(items, lag=1):
    def tick(t):
        def fn():
            for s in range(depth):
                n = t - s * lag
                if 0 <= n < len(items):
                    next(gens[n], None)
        return fn

    depth = items[0][0]
    gens = [g for _, g in items]
    return [tick(t) for t in range(len(items) + (depth - 1) * lag)]


def _sigmoid(z):
    return 1.0 / (1.0 + jnp.exp(-z))


def _full_rows(ref, r0, n):
    return jnp.concatenate([_get(ref, j, r0, n) for j in range(NJ)], axis=1)


class _Copies:
    def __init__(self, copies):
        self.copies = copies

    def start(self):
        for cp in self.copies:
            cp.start()

    def wait(self):
        for cp in self.copies:
            cp.wait()


def _lanes(j):
    return slice(j * L, (j + 1) * L)


def _get(ref, j, r0, n):
    return pltpu.bitcast(ref[j, pl.ds(r0 // 2, n // 2), :], bf16)


def _put(ref, j, r0, val):
    ref[j, pl.ds(r0, val.shape[0]), :] = val.astype(bf16)


def _row_dots(rows_ref, r0, vec_ref, vs):
    acc = [None] * len(vs)
    for j in range(NJ):
        rows = _get(rows_ref, j, r0, RB).astype(f32)
        for n, v in enumerate(vs):
            t = rows * vec_ref[v, :, _lanes(j)]
            acc[n] = t if acc[n] is None else acc[n] + t
    return [jnp.broadcast_to(jnp.sum(a, axis=1, keepdims=True), (RB, L)) for a in acc]


def _kernel(x_hbm, wqkv_hbm, wo_hbm, wr_ref, wg_hbm, wu_hbm, wd_hbm, gw_ref,
            out_hbm,
            x_v, out_v, w_raw, wo_raw, wg_v, wu_v, wd_v,
            wt_s, wp_v, wo_s, wop_v, gate_s, vec_s, y_s, sel_s, sems, *tiles):
    q_t, k_t, v_t, o_t = (tiles[i * NT:(i + 1) * NT] for i in range(4))

    sem_ids = iter(range(sems.shape[0]))

    def load(src, dst, r0, n, j0=0):
        return _Copies([
            pltpu.make_async_copy(src.at[pl.ds(r0, n), pl.ds(j * L, L)],
                                  dst.at[j, pl.ds(r0, n), :], sems.at[next(sem_ids)])
            for j in range(j0, j0 + NJ)])

    def store(r0, n):
        return _Copies([
            pltpu.make_async_copy(out_v.at[j, pl.ds(r0, n), :],
                                  out_hbm.at[pl.ds(r0, n), pl.ds(j * L, L)], sems.at[next(sem_ids)])
            for j in range(NJ)])

    cp_w = [load(wqkv_hbm, w_raw, 0, D, c * NJ) for c in range(3)]
    cp_x = [load(x_hbm, x_v, 0, TM), load(x_hbm, x_v, TM, S - TM)]
    cp_wo = load(wo_hbm, wo_raw, 0, D)
    fc = F // len(FFN_STEPS)
    cp_f = [[load(src, dst, n * fc, fc)
             for src, dst in ((wg_hbm, wg_v), (wu_hbm, wu_v), (wd_hbm, wd_v))]
            for n in range(len(FFN_STEPS))]
    cp_out = [store(i * TM, TM) for i in range(NT)]

    x_w, out_w, wraw_w, woraw_w, wg_w, wu_w, wd_w, wp_w, wop_w = (
        r.bitcast(u32) for r in (x_v, out_v, w_raw, wo_raw, wg_v, wu_v, wd_v, wp_v, wop_v))
    o_w = [r.bitcast(u32) for r in o_t]

    def w_transpose(c, kb, cb):
        def fn():
            blk = _get(wraw_w, c * NJ + cb, kb * L, L).astype(f32)
            wt_s[kb, pl.ds(c * D + cb * L, L), :] = blk.T
        return fn

    def w_gather(c, j):
        def fn():
            for kb in range(NJ):
                parts = [wt_s[kb, pl.ds(c * D + 4 * j + dd, H, stride=DH), :] for dd in range(4)]
                _put(wp_v, kb, c * D + j * L, jnp.concatenate(parts, axis=0))
        return fn

    def wo_unpack(nb):
        def fn():
            wo_s[nb] = _get(woraw_w, nb, 0, D).astype(f32)
        return fn

    def wo_gather(nb):
        def fn():
            for j in range(NJ):
                parts = [wo_s[nb, pl.ds(4 * j + dd, H, stride=DH), :] for dd in range(4)]
                _put(wop_v, nb, j * L, jnp.concatenate(parts, axis=0))
        return fn

    def qkv(i, c, j):
        def fn():
            y = lax.dot_general(_full_rows(x_w, i * TM, TM), _full_rows(wp_w, c * D + j * L, L),
                                (((1,), (1,)), ((), ())), preferred_element_type=f32)
            if c == 0:
                q_t[i][j] = y
                return
            dst = k_t if c == 1 else v_t
            dst[i][j, pl.ds(HALO, TM), :] = y
            if i + 1 < NT:
                dst[i + 1][j, pl.ds(0, HALO), :] = y[TM - HALO:]
            if i == 0:
                dst[0][j, pl.ds(0, HALO), :] = jnp.broadcast_to(y[0:1], (HALO, L))
        return fn

    def attend(i, r0):
        q = [q_t[i][j, pl.ds(r0, RB), :] for j in range(NJ)]
        z = []
        for w in range(WIN):
            acc = None
            for j in range(NJ):
                t = q[j] * k_t[i][j, pl.ds(HALO + r0 - DIL * w, RB), :]
                acc = t if acc is None else acc + t
            z.append((acc, pltpu.roll(acc, 2 * H, 1)))
        yield
        z = [a + b for a, b in z]
        z = [(a, pltpu.roll(a, H, 1)) for a in z]
        yield
        z = [a + b for a, b in z]
        if i == 0 and r0 < DIL * (WIN - 1):
            pos = r0 + lax.broadcasted_iota(jnp.int32, (RB, L), 0)
            z = [jnp.where(pos >= DIL * w, z[w] * SCALE, -1e9) for w in range(WIN)]
            c = LOG2E
        else:
            c = SCALE * LOG2E
        m = z[0]
        for w in range(1, WIN):
            m = jnp.maximum(m, z[w])
        e = [jnp.exp2((z[w] - m) * c) for w in range(WIN)]
        yield
        den = e[0]
        for w in range(1, WIN):
            den = den + e[w]
        inv = 1.0 / den
        for j in range(NJ):
            acc = None
            for w in range(WIN):
                t = e[w] * v_t[i][j, pl.ds(HALO + r0 - DIL * w, RB), :]
                acc = t if acc is None else acc + t
            _put(o_t[i], j, r0, acc * inv)

    def project(i, nb):
        def fn():
            a = jnp.dot(_full_rows(o_w[i], 0, TM), _get(wop_w, nb, 0, D), preferred_element_type=f32)
            g = gate_s[pl.ds(i * TM, TM), :]
            b = _get(x_w, nb, i * TM, TM).astype(f32)
            b = b + b * 0.0
            _put(out_v, nb, i * TM, g * a + (1.0 - g) * b)
        return fn

    lane = lax.broadcasted_iota(jnp.int32, (RB, L), 1)
    score = [jnp.zeros((RB, L), f32)]

    def route(n):
        g, r = _row_dots(x_w, n * RB, vec_s, (0, 1))
        yield
        score[0] = jnp.where(lane == n, r, score[0])
        e = jnp.exp(-g)
        yield
        gate_s[pl.ds(n * RB, RB), :] = 1.0 / (1.0 + e)

    def row_group(ref, idx):
        word = pl.multiple_of((idx // RB) * (RB // 2), RB // 2)
        rows = [pltpu.bitcast(ref[j, pl.ds(word, RB // 2), :], bf16) for j in range(NJ)]
        hit = lax.broadcasted_iota(jnp.int32, (RB, D), 0) == idx % RB
        return jnp.concatenate(rows, axis=1).astype(f32), hit, word

    def select_top2():
        r = score[0].astype(bf16).astype(f32) + 0.0
        bits = pltpu.bitcast(r, jnp.int32) >> 16
        key = jnp.where(bits < 0, bits ^ 0x7FFF, bits).astype(f32)
        key = jnp.where(r != r, -1e6, key)
        pos = (lane * RB + lax.broadcasted_iota(jnp.int32, (RB, L), 0)).astype(f32)
        for t in range(2):
            first = jnp.min(jnp.where(key == jnp.max(key), pos, float(S)))
            chosen = pos == first
            vec_s[4 + t, :, 0:L] = _sigmoid(
                jnp.broadcast_to(jnp.sum(jnp.where(chosen, r, 0.0), keepdims=True), (RB, L)))
            key = jnp.where(chosen, -2e6, key)
            idx = jnp.clip(first.astype(jnp.int32), 0, S - 1)
            sel_s[t] = idx
            grp, hit, _ = row_group(x_w, idx)
            vec_s[2 + t] = jnp.broadcast_to(
                jnp.sum(jnp.where(hit, grp, 0.0), axis=0, keepdims=True), (RB, D))

    y_acc = {}

    def ffn(f0):
        gp = _row_dots(wg_w, f0, vec_s, (2, 3))
        up = _row_dots(wu_w, f0, vec_s, (2, 3))
        yield
        e = [jnp.exp(-a) for a in gp]
        yield
        sig = [1.0 / (1.0 + a) for a in e]
        yield
        h = [gp[t] * sig[t] * up[t] for t in range(2)]
        for j in range(NJ):
            wd = _get(wd_w, j, f0, RB).astype(f32)
            for t in range(2):
                p = h[t] * wd
                p = p[0:8] + p[8:16]
                y_acc[t, j] = y_acc[t, j] + p if (t, j) in y_acc else p

    def ffn_finish():
        for t in range(2):
            for j in range(NJ):
                y = jnp.sum(y_acc[t, j], axis=0, keepdims=True)
                y_s[t, :, _lanes(j)] = jnp.broadcast_to(y, (RB, L)) * vec_s[4 + t, :, 0:L]

    def patch(t):
        idx = sel_s[t]
        old, hit, word = row_group(out_w, idx)
        g = _sigmoid(jnp.sum(vec_s[2 + t] * vec_s[0], axis=1, keepdims=True))
        new = jnp.where(hit, old + (1.0 - g) * y_s[t], old).astype(bf16)
        for j in range(NJ):
            out_w[j, pl.ds(word, RB // 2), :] = pltpu.bitcast(new[:, _lanes(j)], u32)
        return pl.multiple_of((idx // RB) * RB, RB)

    def qkv_step(i):
        return [qkv(i, c, j) for c in range(3) for j in range(NJ)]

    def attend_step(i):
        return _pipelined([(4, attend(i, r0)) for r0 in range(0, TM, RB)], LAG)

    def project_step(i):
        return [project(i, nb) for nb in range(NJ)]

    def transpose_step(c):
        return [w_transpose(c, kb, cb) for cb in range(NJ) for kb in range(NJ)]

    cp_w[0].start()
    cp_x[0].start()
    cp_w[1].start()
    for n, ref in enumerate((gw_ref, wr_ref)):
        vec_s[n] = jnp.broadcast_to(ref[...].astype(f32).reshape(1, D), (RB, D))

    cp_w[0].wait()
    cp_w[2].start()
    _interleave(transpose_step(0))
    cp_x[0].wait()
    for c in range(3):
        if c < 2:
            cp_w[c + 1].wait()
        if c == 0:
            cp_x[1].start()
        if c == 1:
            cp_wo.start()
        main = []
        for j in range(NJ):
            main += [w_gather(c, j), qkv(0, c, j)]
        _interleave(main, *([transpose_step(c + 1)] if c < 2 else []))

    for step in range(1, NT + 2):
        streams = []
        mxu = qkv_step(step) if step < NT else []
        if step >= 2:
            mxu = mxu + project_step(step - 2)
        streams.append(mxu)
        if step <= NT:
            streams.append(attend_step(step - 1))
        if step == 1:
            for cp in cp_f[0]:
                cp.start()
            cp_x[1].wait()
            cp_wo.wait()
            streams.append(_pipelined([(3, route(n)) for n in range(S // RB)], 4))
            streams.append([fn for nb in range(NJ) for fn in (wo_unpack(nb), wo_gather(nb))])
        if step in FFN_STEPS:
            n = FFN_STEPS.index(step)
            for cp in cp_f[n]:
                cp.wait()
            if n + 1 < len(FFN_STEPS):
                for cp in cp_f[n + 1]:
                    cp.start()
            streams.append(_pipelined([(4, ffn(f0)) for f0 in range(n * fc, (n + 1) * fc, RB)]))
        _interleave(*streams)
        if step == 1:
            select_top2()
        if step == FFN_STEPS[-1]:
            ffn_finish()
        if 2 <= step <= NT:
            cp_out[step - 2].start()

    for i in range(NT - 1):
        cp_out[i].wait()
    base = [patch(0), patch(1)]
    cp_last = cp_out[NT - 1]
    cp_last.start()
    cp_fix = [store(b, RB) for b in base]
    sent = S - TM
    resend = [base[0] < sent, jnp.logical_and(base[1] < sent, base[1] != base[0])]
    for cp, cond in zip(cp_fix, resend):
        pl.when(cond)(cp.start)
    for cp, cond in zip(cp_fix, resend):
        pl.when(cond)(cp.wait)
    cp_last.wait()


@jax.jit
def pallas_gated_mix__sliding_local_dilated__moe_arch_mod__prompt_kernel(
    A_x: jax.Array,
    A_wqkv: jax.Array,
    A_wo: jax.Array,
    B_x: jax.Array,
    B_w_r: jax.Array,
    B_w_gate: jax.Array,
    B_w_up: jax.Array,
    B_w_down: jax.Array,
    gate_w: jax.Array,
):
    hbm = pl.BlockSpec(memory_space=pl.ANY)
    vmem = pl.BlockSpec(memory_space=pltpu.VMEM)
    n_sems = NJ * (3 + 2 + 1 + 3 * len(FFN_STEPS) + NT + 2)
    scratch = [
        pltpu.VMEM((NJ, S, L), bf16),
        pltpu.VMEM((NJ, S, L), bf16),
        pltpu.VMEM((3 * NJ, D, L), bf16),
        pltpu.VMEM((NJ, D, L), bf16),
        pltpu.VMEM((NJ, F, L), bf16),
        pltpu.VMEM((NJ, F, L), bf16),
        pltpu.VMEM((NJ, F, L), bf16),
        pltpu.VMEM((NJ, 3 * D, L), f32),
        pltpu.VMEM((NJ, 3 * D, L), bf16),
        pltpu.VMEM((NJ, D, L), f32),
        pltpu.VMEM((NJ, D, L), bf16),
        pltpu.VMEM((S, L), f32),
        pltpu.VMEM((6, RB, D), f32),
        pltpu.VMEM((2, RB, D), f32),
        pltpu.SMEM((2,), jnp.int32),
        pltpu.SemaphoreType.DMA((n_sems,)),
    ]
    scratch += [pltpu.VMEM((NJ, TM, L), f32)] * NT
    scratch += [pltpu.VMEM((NJ, HALO + TM, L), f32)] * (2 * NT)
    scratch += [pltpu.VMEM((NJ, TM, L), bf16)] * NT
    out = pl.pallas_call(
        _kernel,
        out_shape=jax.ShapeDtypeStruct((S, D), bf16),
        in_specs=[hbm, hbm, hbm, vmem, hbm, hbm, hbm, vmem],
        out_specs=hbm,
        scratch_shapes=scratch,
        compiler_params=pltpu.CompilerParams(vmem_limit_bytes=100 * 2**20),
        name="gated_mix",
    )(A_x.reshape(S, D), A_wqkv, A_wo, B_w_r,
      B_w_gate.T, B_w_up.T, B_w_down, gate_w)
    return out.reshape(1, S, D)
```

```python
import numpy as np

import jax
import jax.numpy as jnp
from jax import lax
import jax.experimental.pallas as pl
import jax.experimental.pallas.tpu as pltpu

S, D, F = 2048, 640, 1728
H, DH = 32, 20
WIN, DIL = 8, 2
HALO = 16
L = 128
NJ = D // L
TM = 256
NT = S // TM
RB = 16
SCALE = float(DH) ** -0.5
LOG2E = float(np.log2(np.e))
INLINE_FROM = 5

T_ROUTE = (12.0, 30.0)
T_SELECT = (31.0, 39.0)
T_FFN = (40.0, 138.0)
FFN_PARTS = 4

f32, bf16, u32, i32 = jnp.float32, jnp.bfloat16, jnp.uint32, jnp.int32


class _Schedule:
    def __init__(self):
        self.items = []

    def at(self, pos, fn):
        self.items.append((pos, len(self.items), fn))

    def spread(self, t0, t1, fns):
        for n, fn in enumerate(fns):
            self.at(t0 + (n + 0.5) * (t1 - t0) / len(fns), fn)

    def pipeline(self, t0, t1, gens, depth, lag=1):
        step = (t1 - t0) / (len(gens) + (depth - 1) * lag)
        for n, gen in enumerate(gens):
            for s in range(depth):
                self.at(t0 + (n + s * lag + 0.5 + 0.01 * s) * step,
                        lambda gen=gen: next(gen, None))

    def emit(self):
        for _, _, fn in sorted(self.items, key=lambda it: it[:2]):
            fn()


class _Copies:
    def __init__(self, copies):
        self.copies = copies

    def start(self):
        for cp in self.copies:
            cp.start()

    def wait(self):
        for cp in self.copies:
            cp.wait()


def _recip(d):
    d = jnp.minimum(d, 1e30)
    r = pl.reciprocal(d, approx=True)
    return r * (2.0 - d * r)


def _sigmoid(z):
    return _recip(1.0 + jnp.exp(-z))


def _lanes(j):
    return slice(j * L, (j + 1) * L)


def _get(ref, j, r0, n):
    return pltpu.bitcast(ref[j, pl.ds(r0 // 2, n // 2), :], bf16)


def _full_rows(ref, r0, n):
    return jnp.concatenate([_get(ref, j, r0, n) for j in range(NJ)], axis=1)


def _put(ref, j, r0, val):
    ref[j, pl.ds(r0, val.shape[0]), :] = val.astype(bf16)


def _row_dots(rows_ref, r0, vec_ref, vs):
    acc = [None] * len(vs)
    for j in range(NJ):
        rows = _get(rows_ref, j, r0, RB).astype(f32)
        for n, v in enumerate(vs):
            t = rows * vec_ref[v, :, _lanes(j)]
            acc[n] = t if acc[n] is None else acc[n] + t
    return [jnp.broadcast_to(jnp.sum(a, axis=1, keepdims=True), (RB, L)) for a in acc]


def _kernel(x_hbm, wqkv_hbm, wo_hbm, wr_hbm, wg_hbm, wu_hbm, wd_hbm, gw_hbm,
            out_hbm,
            x_v, out_v, w_raw, wo_raw, wg_v, wu_v, wd_v, gw_v, wr_v,
            wt_s, wp_v, wo_s, wop_v, gate_s, vec_s, y_s, sel_s, sems, *tiles):
    q_t, k_t, v_t, o_t = (tiles[i * NT:(i + 1) * NT] for i in range(4))
    x_w, out_w, wg_w, wu_w, wd_w, wp_w, wop_w = (
        r.bitcast(u32) for r in (x_v, out_v, wg_v, wu_v, wd_v, wp_v, wop_v))
    o_w = [r.bitcast(u32) for r in o_t]

    sem_ids = iter(range(sems.shape[0]))

    def copy(src, dst):
        return pltpu.make_async_copy(src, dst, sems.at[next(sem_ids)])

    def load(src, dst, r0, n):
        return _Copies([copy(src.at[pl.ds(r0, n), pl.ds(j * L, L)], dst.at[j, pl.ds(r0, n), :])
                        for j in range(NJ)])

    def store(r0, n, groups):
        return _Copies([copy(out_v.at[j, pl.ds(r0, n), :], out_hbm.at[pl.ds(r0, n), pl.ds(j * L, L)])
                        for j in groups])

    def w_transpose(c, kb, cb):
        def fn():
            blk = w_raw[pl.ds(kb * L, L), pl.ds(c * D + cb * L, L)].astype(f32)
            wt_s[kb, pl.ds(c * D + cb * L, L), :] = blk.T
        return fn

    def w_gather(c, j):
        def fn():
            for kb in range(NJ):
                parts = [wt_s[kb, pl.ds(c * D + 4 * j + dd, H, stride=DH), :] for dd in range(4)]
                _put(wp_v, kb, c * D + j * L, jnp.concatenate(parts, axis=0))
        return fn

    def wo_widen(nb):
        def fn():
            wo_s[nb] = wo_raw[:, _lanes(nb)].astype(f32)
        return fn

    def wo_gather(nb):
        def fn():
            for j in range(NJ):
                parts = [wo_s[nb, pl.ds(4 * j + dd, H, stride=DH), :] for dd in range(4)]
                _put(wop_v, nb, j * L, jnp.concatenate(parts, axis=0))
        return fn

    def qkv(i, c, j):
        def fn():
            y = lax.dot_general(_full_rows(x_w, i * TM, TM), _full_rows(wp_w, c * D + j * L, L),
                                (((1,), (1,)), ((), ())), preferred_element_type=f32)
            if c == 0:
                q_t[i][j] = y
                return
            dst = k_t if c == 1 else v_t
            dst[i][j, pl.ds(HALO, TM), :] = y
            if i + 1 < NT:
                dst[i + 1][j, pl.ds(0, HALO), :] = y[TM - HALO:]
            if i == 0:
                dst[0][j, pl.ds(0, HALO), :] = jnp.broadcast_to(y[0:1], (HALO, L))
        return fn

    def attend(i, r0):
        q = [q_t[i][j, pl.ds(r0, RB), :] for j in range(NJ)]
        z = []
        for w in range(WIN):
            acc = None
            for j in range(NJ):
                t = q[j] * k_t[i][j, pl.ds(HALO + r0 - DIL * w, RB), :]
                acc = t if acc is None else acc + t
            z.append((acc, pltpu.roll(acc, 2 * H, 1)))
        yield
        z = [a + b for a, b in z]
        z = [(a, pltpu.roll(a, H, 1)) for a in z]
        yield
        z = [a + b for a, b in z]
        if i == 0 and r0 < DIL * (WIN - 1):
            pos = r0 + lax.broadcasted_iota(i32, (RB, L), 0)
            z = [jnp.where(pos >= DIL * w, z[w] * SCALE, -1e9) for w in range(WIN)]
            c = LOG2E
        else:
            c = SCALE * LOG2E
        m = z[0]
        for w in range(1, WIN):
            m = jnp.maximum(m, z[w])
        e = [jnp.exp2((z[w] - m) * c) for w in range(WIN)]
        yield
        den = e[0]
        for w in range(1, WIN):
            den = den + e[w]
        inv = _recip(den)
        for j in range(NJ):
            acc = None
            for w in range(WIN):
                t = e[w] * v_t[i][j, pl.ds(HALO + r0 - DIL * w, RB), :]
                acc = t if acc is None else acc + t
            _put(o_t[i], j, r0, acc * inv)

    def project(i, nb):
        def fn():
            a = jnp.dot(_full_rows(o_w[i], 0, TM), _get(wop_w, nb, 0, D), preferred_element_type=f32)
            g = gate_s[pl.ds(i * TM, TM), :]
            x = _get(x_w, nb, i * TM, TM).astype(f32)
            upd = x * 0.0
            if i >= INLINE_FROM:
                row = i * TM + lax.broadcasted_iota(i32, (TM, L), 0)
                y0, y1 = (y_s[t, 0:1, _lanes(nb)] for t in range(2))
                upd = upd + jnp.where(row == sel_s[0], y0, jnp.where(row == sel_s[1], y1, 0.0))
            _put(out_v, nb, i * TM, g * a + (1.0 - g) * (x + upd))
        return fn

    lane = lax.broadcasted_iota(i32, (RB, L), 1)
    score = [jnp.zeros((RB, L), f32)]

    def route(n):
        g, r = _row_dots(x_w, n * RB, vec_s, (0, 1))
        yield
        score[0] = jnp.where(lane == n, r, score[0])
        e = jnp.exp(-g)
        yield
        gate_s[pl.ds(n * RB, RB), :] = _recip(1.0 + e)

    def row_group(ref, base, idx):
        word = pl.multiple_of(base // 2, RB // 2)
        rows = [pltpu.bitcast(ref[j, pl.ds(word, RB // 2), :], bf16) for j in range(NJ)]
        hit = lax.broadcasted_iota(i32, (RB, D), 0) == idx - base
        return jnp.concatenate(rows, axis=1).astype(f32), hit, word

    def select_top2():
        r = score[0].astype(bf16).astype(f32)
        r = jnp.where(r == 0.0, 0.0, r)
        bits = pltpu.bitcast(r, i32) >> 16
        key = jnp.where(bits < 0, bits ^ 0x7FFF, bits).astype(f32)
        key = jnp.where(r != r, -1e6, key)
        pos = (lane * RB + lax.broadcasted_iota(i32, (RB, L), 0)).astype(f32)
        for t in range(2):
            best = jnp.max(key, keepdims=True)
            yield
            first = jnp.min(jnp.where(key == best, pos, float(S)), keepdims=True)
            yield
            chosen = pos == first
            key = jnp.where(chosen, -2e6, key)
            r_sel = jnp.sum(jnp.where(chosen, r, 0.0), keepdims=True)
            idx = jnp.clip(first.astype(i32)[0, 0], 0, S - 1)
            yield
            sel_s[t] = idx
            vec_s[4 + t, :, 0:L] = _sigmoid(jnp.broadcast_to(r_sel, (RB, L)))
            grp, hit, _ = row_group(x_w, (idx // RB) * RB, idx)
            vec_s[2 + t] = jnp.broadcast_to(
                jnp.sum(jnp.where(hit, grp, 0.0), axis=0, keepdims=True), (RB, D))
            yield

    y_acc = {}

    def ffn(f0):
        gp = _row_dots(wg_w, f0, vec_s, (2, 3))
        up = _row_dots(wu_w, f0, vec_s, (2, 3))
        yield
        e = [jnp.exp(-a) for a in gp]
        yield
        sig = [_recip(1.0 + a) for a in e]
        yield
        h = [gp[t] * sig[t] * up[t] for t in range(2)]
        for j in range(NJ):
            wd = _get(wd_w, j, f0, RB).astype(f32)
            for t in range(2):
                p = h[t] * wd
                p = p[0:8] + p[8:16]
                y_acc[t, j] = y_acc[t, j] + p if (t, j) in y_acc else p

    def ffn_finish():
        for t in range(2):
            for j in range(NJ):
                y = jnp.sum(y_acc[t, j], axis=0, keepdims=True)
                y_s[t, :, _lanes(j)] = jnp.broadcast_to(y, (RB, L)) * vec_s[4 + t, :, 0:L]

    resend = []

    def patch(t):
        def fn():
            idx = sel_s[t]
            base = jnp.minimum((idx // RB) * RB, INLINE_FROM * TM - RB)
            old, hit, word = row_group(out_w, base, idx)
            g = _sigmoid(jnp.sum(vec_s[2 + t] * vec_s[0], axis=1, keepdims=True))
            new = jnp.where(hit, old + (1.0 - g) * y_s[t], old).astype(bf16)
            for j in range(NJ):
                out_w[j, pl.ds(word, RB // 2), :] = pltpu.bitcast(new[:, _lanes(j)], u32)
            resend.append(store(pl.multiple_of(base, RB), RB, range(NJ)))
        return fn

    sch = _Schedule()
    mxu = []
    for c in range(3):
        mxu += [("qkv", i, c, j) for i in range(2) for j in range(NJ)]
    for i in range(2, NT):
        mxu += [("qkv", i, c, j) for c in range(3) for j in range(NJ)]
        mxu += [("out", i - 2, nb) for nb in range(NJ)]
    mxu += [("out", i, nb) for i in range(NT - 2, NT) for nb in range(NJ)]
    slot = {op: n for n, op in enumerate(mxu)}

    cp_w = [copy(wqkv_hbm.at[:, pl.ds(c * D, D)], w_raw.at[:, pl.ds(c * D, D)]) for c in range(3)]
    cp_x = [load(x_hbm, x_v, 0, TM), load(x_hbm, x_v, TM, TM), load(x_hbm, x_v, 2 * TM, S - 2 * TM)]
    cp_vec = _Copies([copy(gw_hbm, gw_v), copy(wr_hbm, wr_v)])
    cp_wo = copy(wo_hbm, wo_raw)
    nf = F // RB
    cuts = [RB * (nf * n // FFN_PARTS) for n in range(FFN_PARTS + 1)]
    cp_f = [_Copies([load(src, dst, cuts[n], cuts[n + 1] - cuts[n])
                     for src, dst in ((wg_hbm, wg_v), (wu_hbm, wu_v), (wd_hbm, wd_v))])
            for n in range(FFN_PARTS)]
    cp_out = {op: store(op[1] * TM, TM, [op[2]]) for op in mxu if op[0] == "out"}

    for op, n in slot.items():
        sch.at(n, qkv(*op[1:]) if op[0] == "qkv" else project(*op[1:]))
        if op[0] == "out":
            sch.at(n + 1.5, cp_out[op].start)

    for n, cp in enumerate((cp_w[0], cp_x[0], cp_x[1], cp_vec)):
        sch.at(-9 + n, cp.start)
    sch.at(-4, cp_w[0].wait)
    sch.at(-3.9, cp_w[1].start)
    sch.spread(-3, -2, [w_transpose(0, kb, cb) for cb in range(NJ) for kb in range(NJ)])
    sch.at(-1, cp_x[0].wait)
    sch.at(slot["qkv", 1, 0, 0] - 0.5, cp_x[1].wait)
    sch.at(2.5, cp_w[2].start)
    sch.at(4.5, cp_x[2].start)
    sch.at(10.5, cp_wo.start)
    for c in range(3):
        first = slot["qkv", 0, c, 0]
        if c > 0:
            sch.at(first - 4.9, cp_w[c].wait)
            sch.spread(first - 4.8, first - 0.8,
                       [w_transpose(c, kb, cb) for cb in range(NJ) for kb in range(NJ)])
        for j in range(NJ):
            sch.at(first + j - 0.7, w_gather(c, j))
    first = slot["out", 0, 0]
    sch.at(first - 12, cp_wo.wait)
    sch.spread(first - 11, first - 1, [fn for nb in range(NJ) for fn in (wo_widen(nb), wo_gather(nb))])

    def vectors():
        cp_vec.wait()
        for n, ref in enumerate((gw_v, wr_v)):
            vec_s[n] = jnp.broadcast_to(ref[...].astype(f32).reshape(1, D), (RB, D))

    t0, t1 = T_ROUTE
    sch.at(t0 - 1, vectors)
    sch.at(t0 + (t1 - t0) * 0.24, cp_x[2].wait)
    sch.pipeline(t0, t1, [route(n) for n in range(S // RB)], 3, 4)
    picker = select_top2()
    sch.spread(*T_SELECT, [lambda: next(picker)] * 8)

    for i in range(NT):
        ready = slot["qkv", max(i, 1), 2, NJ - 1] + 1
        t0, t1 = ready, ready + 20
        if i < 2:
            t0, t1 = ready + 7.5 * i, ready + 7.5 * (i + 1)
        if i == NT - 1:
            t1 = slot["out", i, 0] - 0.5
        sch.pipeline(t0, t1, [attend(i, r0) for r0 in range(0, TM, RB)], 4)

    t0, t1 = T_FFN
    for n in range(FFN_PARTS):
        need = t0 + (t1 - t0) * (cuts[n] // RB) / (nf + 3)
        sch.at(need - 20, cp_f[n].start)
        sch.at(need, cp_f[n].wait)
    sch.pipeline(t0, t1, [ffn(f0) for f0 in range(0, F, RB)], 4)
    sch.at(t1 + 0.1, ffn_finish)

    for op, cp in cp_out.items():
        sch.at(t1 + 1 if op[1] < INLINE_FROM else len(mxu) + 2, cp.wait)
    for t in range(2):
        sch.at(t1 + 2 + t, patch(t))
        sch.at(t1 + 4 + 5 * t, lambda t=t: resend[t].start())
        sch.at(t1 + 8.5 + 5 * t, lambda t=t: resend[t].wait())
    sch.emit()


@jax.jit
def pallas_gated_mix__sliding_local_dilated__moe_arch_mod__prompt_kernel(
    A_x: jax.Array,
    A_wqkv: jax.Array,
    A_wo: jax.Array,
    B_x: jax.Array,
    B_w_r: jax.Array,
    B_w_gate: jax.Array,
    B_w_up: jax.Array,
    B_w_down: jax.Array,
    gate_w: jax.Array,
):
    n_sems = 3 + 2 + 1 + NJ * (3 + 3 * FFN_PARTS + NT + 2)
    scratch = [
        pltpu.VMEM((NJ, S, L), bf16),
        pltpu.VMEM((NJ, S, L), bf16),
        pltpu.VMEM((D, 3 * D), bf16),
        pltpu.VMEM((D, D), bf16),
        pltpu.VMEM((NJ, F, L), bf16),
        pltpu.VMEM((NJ, F, L), bf16),
        pltpu.VMEM((NJ, F, L), bf16),
        pltpu.VMEM((D,), bf16),
        pltpu.VMEM((D,), bf16),
        pltpu.VMEM((NJ, 3 * D, L), f32),
        pltpu.VMEM((NJ, 3 * D, L), bf16),
        pltpu.VMEM((NJ, D, L), f32),
        pltpu.VMEM((NJ, D, L), bf16),
        pltpu.VMEM((S, L), f32),
        pltpu.VMEM((6, RB, D), f32),
        pltpu.VMEM((2, RB, D), f32),
        pltpu.SMEM((2,), i32),
        pltpu.SemaphoreType.DMA((n_sems,)),
    ]
    scratch += [pltpu.VMEM((NJ, TM, L), f32)] * NT
    scratch += [pltpu.VMEM((NJ, HALO + TM, L), f32)] * (2 * NT)
    scratch += [pltpu.VMEM((NJ, TM, L), bf16)] * NT
    out = pl.pallas_call(
        _kernel,
        out_shape=jax.ShapeDtypeStruct((S, D), bf16),
        in_specs=[pl.BlockSpec(memory_space=pl.ANY)] * 8,
        out_specs=pl.BlockSpec(memory_space=pl.ANY),
        scratch_shapes=scratch,
        compiler_params=pltpu.CompilerParams(vmem_limit_bytes=100 * 2**20),
        name="gated_mix",
    )(A_x.reshape(S, D), A_wqkv, A_wo, B_w_r,
      B_w_gate.T, B_w_up.T, B_w_down, gate_w)
    return out.reshape(1, S, D)
```

```python
import numpy as np

import jax
import jax.numpy as jnp
from jax import lax
import jax.experimental.pallas as pl
import jax.experimental.pallas.tpu as pltpu

S, D, F = 2048, 640, 1728
H, DH = 32, 20
WIN, DIL = 8, 2
HALO = 16
L = 128
NJ = D // L
TM = 256
NT = S // TM
RB = 16
SCALE = float(DH) ** -0.5
LOG2E = float(np.log2(np.e))
INLINE_FROM = 5

T_ROUTE = (12.0, 30.0)
T_SELECT = (31.0, 39.0)
T_FFN = (40.0, 138.0)
FFN_PARTS = 4
FLAGS = None
MS = 128
RA = 8
ATT_LAG = 1
FFN_LAG = 1
PACE = False

f32, bf16, u32, i32 = jnp.float32, jnp.bfloat16, jnp.uint32, jnp.int32


class _Schedule:
    def __init__(self):
        self.items = []

    def at(self, pos, fn):
        self.items.append((pos, len(self.items), fn))

    def spread(self, t0, t1, fns):
        for n, fn in enumerate(fns):
            self.at(t0 + (n + 0.5) * (t1 - t0) / len(fns), fn)

    def pipeline(self, t0, t1, gens, depth, lag=1):
        step = (t1 - t0) / (len(gens) + (depth - 1) * lag)
        for n, gen in enumerate(gens):
            for s in range(depth):
                self.at(t0 + (n + s * lag + 0.5 + 0.01 * s) * step,
                        lambda gen=gen: next(gen, None))

    def emit(self):
        for _, _, fn in sorted(self.items, key=lambda it: it[:2]):
            fn()


class _Copies:
    def __init__(self, copies):
        self.copies = copies

    def start(self):
        for cp in self.copies:
            cp.start()

    def wait(self):
        for cp in self.copies:
            cp.wait()


def _recip(d):
    r = pl.reciprocal(d, approx=True)
    return r * (2.0 - d * r)


def _exp_neg(z):
    return jnp.minimum(jnp.exp(-z), 1e38)


def _sigmoid(z):
    return _recip(1.0 + _exp_neg(z))


def _lanes(j):
    return slice(j * L, (j + 1) * L)


def _get(ref, j, r0, n):
    return pltpu.bitcast(ref[j, pl.ds(r0 // 2, n // 2), :], bf16)


def _full_rows(ref, r0, n):
    return jnp.concatenate([_get(ref, j, r0, n) for j in range(NJ)], axis=1)


def _put(ref, j, r0, val):
    ref[j, pl.ds(r0, val.shape[0]), :] = val.astype(bf16)


def _row_dots(rows_ref, r0, vec_ref, vs):
    acc = [None] * len(vs)
    for j in range(NJ):
        rows = _get(rows_ref, j, r0, RB).astype(f32)
        for n, v in enumerate(vs):
            vec = vec_ref[v, 0:8, _lanes(j)]
            t = rows * jnp.concatenate([vec, vec], axis=0)
            acc[n] = t if acc[n] is None else acc[n] + t
    return [jnp.broadcast_to(jnp.sum(a, axis=1, keepdims=True), (RB, L)) for a in acc]


def _kernel(x_hbm, wqkv_hbm, wo_hbm, wr_hbm, wg_hbm, wu_hbm, wd_hbm, gw_hbm,
            out_hbm,
            x_v, out_v, w_raw, wo_raw, wg_v, wu_v, wd_v, gw_v, wr_v,
            wt_s, wp_v, wo_s, wop_v, gate_s, vec_s, y_s, sel_s, sems, *tiles):
    q_t, k_t, v_t, o_t = (tiles[i * NT:(i + 1) * NT] for i in range(4))
    x_w, out_w, wg_w, wu_w, wd_w, wp_w, wop_w = (
        r.bitcast(u32) for r in (x_v, out_v, wg_v, wu_v, wd_v, wp_v, wop_v))
    o_w = [r.bitcast(u32) for r in o_t]

    sem_ids = iter(range(sems.shape[0]))

    def copy(src, dst):
        return pltpu.make_async_copy(src, dst, sems.at[next(sem_ids)])

    def load(src, dst, r0, n):
        return _Copies([copy(src.at[pl.ds(r0, n), pl.ds(j * L, L)], dst.at[j, pl.ds(r0, n), :])
                        for j in range(NJ)])

    def store(r0, n, groups):
        return _Copies([copy(out_v.at[j, pl.ds(r0, n), :], out_hbm.at[pl.ds(r0, n), pl.ds(j * L, L)])
                        for j in groups])

    def w_transpose(c, kb, cb):
        def fn():
            blk = w_raw[pl.ds(kb * L, L), pl.ds(c * D + cb * L, L)].astype(f32)
            wt_s[kb, pl.ds(c * D + cb * L, L), :] = blk.T
        return fn

    def w_gather(c, j):
        def fn():
            for kb in range(NJ):
                parts = [wt_s[kb, pl.ds(c * D + 4 * j + dd, H, stride=DH), :] for dd in range(4)]
                _put(wp_v, kb, c * D + j * L, jnp.concatenate(parts, axis=0))
        return fn

    def wo_widen(nb):
        def fn():
            wo_s[nb] = wo_raw[:, _lanes(nb)].astype(f32)
        return fn

    def wo_gather(nb):
        def fn():
            for j in range(NJ):
                parts = [wo_s[nb, pl.ds(4 * j + dd, H, stride=DH), :] for dd in range(4)]
                _put(wop_v, nb, j * L, jnp.concatenate(parts, axis=0))
        return fn

    sel_s[2] = jnp.min(lax.broadcasted_iota(i32, (8, L), 1).astype(f32)).astype(i32)
    paced = {}

    def pace(y):
        spare = pl.multiple_of(sel_s[2] * 8, 8)
        for ref, lead, row in (paced.values() if PACE else []):
            ref[lead, pl.ds(row + spare, 8), 0:L] = y[0:8]

    def qkv(i, c, j, m0):
        def fn():
            y = lax.dot_general(_full_rows(x_w, i * TM + m0, MS), _full_rows(wp_w, c * D + j * L, L),
                                (((1,), (1,)), ((), ())), preferred_element_type=f32)
            pace(y)
            if c == 0:
                q_t[i][j, pl.ds(m0, MS), :] = y
                return
            dst = k_t if c == 1 else v_t
            dst[i][j, pl.ds(HALO + m0, MS), :] = y
            if i + 1 < NT and m0 + MS == TM:
                dst[i + 1][j, pl.ds(0, HALO), :] = y[MS - HALO:]
            if i == 0 and m0 == 0:
                dst[0][j, pl.ds(0, HALO), :] = jnp.broadcast_to(y[0:1], (HALO, L))
        return fn

    half = {}

    def attend(i, r0):
        q = [q_t[i][j, pl.ds(r0, RA), :] for j in range(NJ)]
        z = []
        for w in range(WIN):
            acc = None
            for j in range(NJ):
                t = q[j] * k_t[i][j, pl.ds(HALO + r0 - DIL * w, RA), :]
                acc = t if acc is None else acc + t
            z.append((acc, pltpu.roll(acc, 2 * H, 1)))
        yield
        z = [a + b for a, b in z]
        z = [(a, pltpu.roll(a, H, 1)) for a in z]
        yield
        z = [a + b for a, b in z]
        if i == 0 and r0 < DIL * (WIN - 1):
            pos = r0 + lax.broadcasted_iota(i32, (RA, L), 0)
            z = [jnp.where(pos >= DIL * w, z[w] * SCALE, -1e9) for w in range(WIN)]
            c = LOG2E
        else:
            c = SCALE * LOG2E
        m = z[0]
        for w in range(1, WIN):
            m = jnp.maximum(m, z[w])
        e = [jnp.exp2((z[w] - m) * c) for w in range(WIN)]
        yield
        den = e[0]
        for w in range(1, WIN):
            den = den + e[w]
        inv = _recip(den)
        for j in range(NJ):
            acc = None
            for w in range(WIN):
                t = e[w] * v_t[i][j, pl.ds(HALO + r0 - DIL * w, RA), :]
                acc = t if acc is None else acc + t
            o = acc * inv
            if RA == RB:
                _put(o_t[i], j, r0, o)
            elif r0 % RB == 0:
                half[i, j] = o
            else:
                _put(o_t[i], j, r0 - RA, jnp.concatenate([half.pop((i, j)), o], axis=0))

    def project(i, nb, m0):
        def fn():
            r0 = i * TM + m0
            a = jnp.dot(_full_rows(o_w[i], m0, MS), _get(wop_w, nb, 0, D), preferred_element_type=f32)
            pace(a)
            g = gate_s[pl.ds(r0, MS), :]
            b = _get(x_w, nb, r0, MS).astype(f32)
            if i >= INLINE_FROM:
                row = r0 + lax.broadcasted_iota(i32, (MS, L), 0)
                y0, y1 = (y_s[t, 0:1, _lanes(nb)] for t in range(2))
                b = b + jnp.where(row == sel_s[0], y0, jnp.where(row == sel_s[1], y1, 0.0))
            _put(out_v, nb, r0, b + g * (a - b))
        return fn

    lane = lax.broadcasted_iota(i32, (RB, L), 1)
    score = [jnp.zeros((RB, L), f32)]

    def route(n):
        g, r = _row_dots(x_w, n * RB, vec_s, (0, 1))
        yield
        score[0] = jnp.where(lane == n, r, score[0])
        e = _exp_neg(g)
        yield
        gate_s[pl.ds(n * RB, RB), :] = _recip(1.0 + e)

    def row_group(ref, base, idx):
        word = pl.multiple_of(base // 2, RB // 2)
        rows = [pltpu.bitcast(ref[j, pl.ds(word, RB // 2), :], bf16) for j in range(NJ)]
        hit = lax.broadcasted_iota(i32, (RB, D), 0) == idx - base
        return jnp.concatenate(rows, axis=1).astype(f32), hit, word

    def select_top2():
        r = score[0].astype(bf16).astype(f32)
        r = jnp.where(r == 0.0, 0.0, r)
        bits = pltpu.bitcast(r, i32) >> 16
        key = jnp.where(bits < 0, bits ^ 0x7FFF, bits).astype(f32)
        key = jnp.where(r != r, -1e6, key)
        pos = (lane * RB + lax.broadcasted_iota(i32, (RB, L), 0)).astype(f32)
        for t in range(2):
            best = jnp.max(key, keepdims=True)
            yield
            first = jnp.min(jnp.where(key == best, pos, float(S)), keepdims=True)
            yield
            chosen = pos == first
            key = jnp.where(chosen, -2e6, key)
            r_sel = jnp.sum(jnp.where(chosen, r, 0.0), keepdims=True)
            idx = jnp.clip(first.astype(i32)[0, 0], 0, S - 1)
            yield
            sel_s[t] = idx
            vec_s[4 + t, :, 0:L] = _sigmoid(jnp.broadcast_to(r_sel, (RB, L)))
            grp, hit, _ = row_group(x_w, (idx // RB) * RB, idx)
            vec_s[2 + t] = jnp.broadcast_to(
                jnp.sum(jnp.where(hit, grp, 0.0), axis=0, keepdims=True), (RB, D))
            yield

    y_acc = {}

    def ffn(f0):
        gp = _row_dots(wg_w, f0, vec_s, (2, 3))
        up = _row_dots(wu_w, f0, vec_s, (2, 3))
        yield
        e = [_exp_neg(a) for a in gp]
        yield
        sig = [_recip(1.0 + a) for a in e]
        yield
        h = [gp[t] * sig[t] * up[t] for t in range(2)]
        for j in range(NJ):
            wd = _get(wd_w, j, f0, RB).astype(f32)
            for t in range(2):
                p = h[t] * wd
                p = p[0:8] + p[8:16]
                y_acc[t, j] = y_acc[t, j] + p if (t, j) in y_acc else p

    def ffn_finish():
        for t in range(2):
            for j in range(NJ):
                y = jnp.sum(y_acc[t, j], axis=0, keepdims=True)
                y_s[t, :, _lanes(j)] = jnp.broadcast_to(y, (RB, L)) * vec_s[4 + t, :, 0:L]

    resend = []

    def patch(t):
        def fn():
            idx = sel_s[t]
            base = jnp.minimum((idx // RB) * RB, INLINE_FROM * TM - RB)
            old, hit, word = row_group(out_w, base, idx)
            g = _sigmoid(jnp.sum(vec_s[2 + t] * vec_s[0], axis=1, keepdims=True))
            new = jnp.where(hit, old + (1.0 - g) * y_s[t], old).astype(bf16)
            for j in range(NJ):
                out_w[j, pl.ds(word, RB // 2), :] = pltpu.bitcast(new[:, _lanes(j)], u32)
            resend.append(store(pl.multiple_of(base, RB), RB, range(NJ)))
        return fn

    sch = _Schedule()
    mxu = []
    for c in range(3):
        mxu += [("qkv", i, c, j) for i in range(2) for j in range(NJ)]
    for i in range(2, NT):
        mxu += [("qkv", i, c, j) for c in range(3) for j in range(NJ)]
        mxu += [("out", i - 2, nb) for nb in range(NJ)]
    mxu += [("out", i, nb) for i in range(NT - 2, NT) for nb in range(NJ)]
    slot = {op: n for n, op in enumerate(mxu)}

    cp_w = [copy(wqkv_hbm.at[:, pl.ds(c * D, D)], w_raw.at[:, pl.ds(c * D, D)]) for c in range(3)]
    cp_x = [load(x_hbm, x_v, 0, TM), load(x_hbm, x_v, TM, TM), load(x_hbm, x_v, 2 * TM, S - 2 * TM)]
    cp_vec = _Copies([copy(gw_hbm, gw_v), copy(wr_hbm, wr_v)])
    cp_wo = copy(wo_hbm, wo_raw)
    nf = F // RB
    cuts = [RB * (nf * n // FFN_PARTS) for n in range(FFN_PARTS + 1)]
    cp_f = [_Copies([load(src, dst, cuts[n], cuts[n + 1] - cuts[n])
                     for src, dst in ((wg_hbm, wg_v), (wu_hbm, wu_v), (wd_hbm, wd_v))])
            for n in range(FFN_PARTS)]
    cp_out = {op: store(op[1] * TM, TM, [op[2]]) for op in mxu if op[0] == "out"}

    for op, n in slot.items():
        for m0 in range(0, TM, MS):
            sch.at(n + m0 / TM, (qkv if op[0] == "qkv" else project)(*op[1:], m0))
        if op[0] == "out":
            sch.at(n + 1.5, cp_out[op].start)

    for n, cp in enumerate((cp_w[0], cp_x[0], cp_x[1], cp_vec)):
        sch.at(-9 + n, cp.start)
    sch.at(-4, cp_w[0].wait)
    sch.at(-3.9, cp_w[1].start)
    sch.spread(-3, -2, [w_transpose(0, kb, cb) for cb in range(NJ) for kb in range(NJ)])
    sch.at(-1, cp_x[0].wait)
    sch.at(slot["qkv", 1, 0, 0] - 0.5, cp_x[1].wait)
    sch.at(2.5, cp_w[2].start)
    sch.at(4.5, cp_x[2].start)
    sch.at(10.5, cp_wo.start)
    for c in range(3):
        first = slot["qkv", 0, c, 0]
        if c > 0:
            sch.at(first - 4.9, cp_w[c].wait)
            sch.spread(first - 4.8, first - 0.8,
                       [w_transpose(c, kb, cb) for cb in range(NJ) for kb in range(NJ)])
        for j in range(NJ):
            sch.at(first + j - 0.7, w_gather(c, j))
    first = slot["out", 0, 0]
    sch.at(first - 12, cp_wo.wait)
    sch.spread(first - 11, first - 1, [fn for nb in range(NJ) for fn in (wo_widen(nb), wo_gather(nb))])

    def vectors():
        cp_vec.wait()
        for n, ref in enumerate((gw_v, wr_v)):
            vec_s[n] = jnp.broadcast_to(ref[...].astype(f32).reshape(1, D), (RB, D))

    t0, t1 = T_ROUTE
    sch.at(t0 - 1, vectors)
    sch.at(t0 + (t1 - t0) * 0.24, cp_x[2].wait)
    sch.pipeline(t0, t1, [route(n) for n in range(S // RB)], 3, 4)
    picker = select_top2()
    sch.spread(*T_SELECT, [lambda: next(picker)] * 8)

    for i in range(NT):
        ready = slot["qkv", max(i, 1), 2, NJ - 1] + 1
        t0, t1 = ready, ready + 20
        if i < 2:
            t0, t1 = ready + 7.5 * i, ready + 7.5 * (i + 1)
        if i == NT - 1:
            t1 = slot["out", i, 0] - 0.5
        sch.pipeline(t0, t1, [attend(i, r0) for r0 in range(0, TM, RA)], 4, ATT_LAG)
        marks = [(q_t[i], 0, TM), (v_t[i], 0, HALO + TM)]
        sch.at(t0 - 1.01, lambda i=i, marks=marks: paced.update({(i, n): m for n, m in enumerate(marks)}))
        sch.at(t1 - 0.01, lambda i=i: [paced.pop((i, n)) for n in range(2)])

    t0, t1 = T_FFN
    for n in range(FFN_PARTS):
        need = t0 + (t1 - t0) * (cuts[n] // RB) / (nf + 3)
        sch.at(need - 20, cp_f[n].start)
        sch.at(need, cp_f[n].wait)
    sch.pipeline(t0, t1, [ffn(f0) for f0 in range(0, F, RB)], 4, FFN_LAG)
    sch.at(t1 + 0.1, ffn_finish)
    sch.at(T_ROUTE[0], lambda: paced.update(vec=(vec_s, 6, 0)))
    sch.at(t1, lambda: paced.pop('vec'))

    for op, cp in cp_out.items():
        sch.at(t1 + 1 if op[1] < INLINE_FROM else len(mxu) + 2, cp.wait)
    for t in range(2):
        sch.at(t1 + 2 + t, patch(t))
        sch.at(t1 + 4 + 5 * t, lambda t=t: resend[t].start())
        sch.at(t1 + 8.5 + 5 * t, lambda t=t: resend[t].wait())
    sch.emit()


@jax.jit
def pallas_gated_mix__sliding_local_dilated__moe_arch_mod__prompt_kernel(
    A_x: jax.Array,
    A_wqkv: jax.Array,
    A_wo: jax.Array,
    B_x: jax.Array,
    B_w_r: jax.Array,
    B_w_gate: jax.Array,
    B_w_up: jax.Array,
    B_w_down: jax.Array,
    gate_w: jax.Array,
):
    n_sems = 3 + 2 + 1 + NJ * (3 + 3 * FFN_PARTS + NT + 2)
    scratch = [
        pltpu.VMEM((NJ, S, L), bf16),
        pltpu.VMEM((NJ, S, L), bf16),
        pltpu.VMEM((D, 3 * D), bf16),
        pltpu.VMEM((D, D), bf16),
        pltpu.VMEM((NJ, F, L), bf16),
        pltpu.VMEM((NJ, F, L), bf16),
        pltpu.VMEM((NJ, F, L), bf16),
        pltpu.VMEM((D,), bf16),
        pltpu.VMEM((D,), bf16),
        pltpu.VMEM((NJ, 3 * D, L), f32),
        pltpu.VMEM((NJ, 3 * D, L), bf16),
        pltpu.VMEM((NJ, D, L), f32),
        pltpu.VMEM((NJ, D, L), bf16),
        pltpu.VMEM((S, L), f32),
        pltpu.VMEM((7, RB, D), f32),
        pltpu.VMEM((2, RB, D), f32),
        pltpu.SMEM((3,), i32),
        pltpu.SemaphoreType.DMA((n_sems,)),
    ]
    scratch += [pltpu.VMEM((NJ, TM + 8, L), f32)] * NT
    scratch += [pltpu.VMEM((NJ, HALO + TM + 8, L), f32)] * (2 * NT)
    scratch += [pltpu.VMEM((NJ, TM, L), bf16)] * NT
    out = pl.pallas_call(
        _kernel,
        out_shape=jax.ShapeDtypeStruct((S, D), bf16),
        in_specs=[pl.BlockSpec(memory_space=pl.ANY)] * 8,
        out_specs=pl.BlockSpec(memory_space=pl.ANY),
        scratch_shapes=scratch,
        compiler_params=pltpu.CompilerParams(vmem_limit_bytes=100 * 2**20, flags=FLAGS),
        name="gated_mix",
    )(A_x.reshape(S, D), A_wqkv, A_wo, B_w_r,
      B_w_gate.T, B_w_up.T, B_w_down, gate_w)
    return out.reshape(1, S, D)
```

```python
import numpy as np

import jax
import jax.numpy as jnp
from jax import lax
import jax.experimental.pallas as pl
import jax.experimental.pallas.tpu as pltpu

S, D, F = 2048, 640, 1728
H, DH = 32, 20
WIN, DIL = 8, 2
HALO = 16
L = 128
NJ = D // L
TM = 256
NT = S // TM
RB = 16
SCALE = float(DH) ** -0.5
LOG2E = float(np.log2(np.e))
INLINE_FROM = 5

HEAD = 2
OUT_LAG = 2
T_START = (-6.5, 0.5, 8.0, 24.0)
T_W = (None, 6.5, 15.0)
T_EARLY = (10.0, 15.0)
T_ROUTE = (26.0, 37.0)
T_WO = 26.0
T_SELECT = (38.0, 45.0)
T_FFN = (46.0, 138.0)
FFN_CUT = 640
FLAGS = None
MS = 128
RA = 8
ATT_LAG = 1
FFN_LAG = 1
SKEW = 0.04
REV = False
ATT_DEPTH = 4
FFN_DEPTH = 4

f32, bf16, u32, i32 = jnp.float32, jnp.bfloat16, jnp.uint32, jnp.int32


class _Schedule:
    def __init__(self):
        self.items = []

    def at(self, pos, fn):
        self.items.append((pos, len(self.items), fn))

    def spread(self, t0, t1, fns):
        for n, fn in enumerate(fns):
            self.at(t0 + (n + 0.5) * (t1 - t0) / len(fns), fn)

    def pipeline(self, t0, t1, gens, depth, lag=1, warp=lambda t: t):
        step = (t1 - t0) / (len(gens) + (depth - 1) * lag)
        for n, gen in enumerate(gens):
            for s in range(depth):
                phase = (depth - s if REV else s) * SKEW / depth
                self.at(warp(t0 + (n + s * lag + 0.5 * (1 - SKEW) + phase) * step),
                        lambda gen=gen: next(gen, None))

    def emit(self):
        for _, _, fn in sorted(self.items, key=lambda it: it[:2]):
            fn()


class _Copies:
    def __init__(self, copies):
        self.copies = copies

    def start(self):
        for cp in self.copies:
            cp.start()

    def wait(self):
        for cp in self.copies:
            cp.wait()


def _recip(d):
    r = pl.reciprocal(d, approx=True)
    return r * (2.0 - d * r)


def _exp_neg(z):
    return jnp.minimum(jnp.exp(-z), 1e38)


def _sigmoid(z):
    return _recip(1.0 + _exp_neg(z))


def _lanes(j):
    return slice(j * L, (j + 1) * L)


def _get(ref, j, r0, n):
    return pltpu.bitcast(ref[j, pl.ds(r0 // 2, n // 2), :], bf16)


def _full_rows(ref, r0, n):
    return jnp.concatenate([_get(ref, j, r0, n) for j in range(NJ)], axis=1)


def _put(ref, j, r0, val):
    ref[j, pl.ds(r0, val.shape[0]), :] = val.astype(bf16)


def _row_dots(rows_ref, r0, vec_ref, vs):
    acc = [None] * len(vs)
    for j in range(NJ):
        rows = _get(rows_ref, j, r0, RB).astype(f32)
        for n, v in enumerate(vs):
            vec = vec_ref[v, 0:8, _lanes(j)]
            t = rows * jnp.concatenate([vec, vec], axis=0)
            acc[n] = t if acc[n] is None else acc[n] + t
    return [jnp.broadcast_to(jnp.sum(a, axis=1, keepdims=True), (RB, L)) for a in acc]


def _kernel(x_hbm, wqkv_hbm, wo_hbm, wr_hbm, wg_hbm, wu_hbm, wd_hbm, gw_hbm,
            out_hbm,
            x_v, out_v, w_raw, wo_raw, wg_v, wu_v, wd_v, gw_v, wr_v,
            wt_s, wp_v, wo_s, wop_v, gate_s, vec_s, y_s, sel_s, sems, *tiles):
    q_t, k_t, v_t, o_t = (tiles[i * NT:(i + 1) * NT] for i in range(4))
    x_w, out_w, wg_w, wu_w, wd_w, wp_w, wop_w = (
        r.bitcast(u32) for r in (x_v, out_v, wg_v, wu_v, wd_v, wp_v, wop_v))
    o_w = [r.bitcast(u32) for r in o_t]

    sem_ids = iter(range(sems.shape[0]))

    def copy(src, dst):
        return pltpu.make_async_copy(src, dst, sems.at[next(sem_ids)])

    def load(src, dst, r0, n):
        return _Copies([copy(src.at[pl.ds(r0, n), pl.ds(j * L, L)], dst.at[j, pl.ds(r0, n), :])
                        for j in range(NJ)])

    def store(r0, n, groups):
        return _Copies([copy(out_v.at[j, pl.ds(r0, n), :], out_hbm.at[pl.ds(r0, n), pl.ds(j * L, L)])
                        for j in groups])

    def w_transpose(c, kb, cb):
        def fn():
            blk = w_raw[pl.ds(kb * L, L), pl.ds(c * D + cb * L, L)].astype(f32)
            wt_s[kb, pl.ds(c * D + cb * L, L), :] = blk.T
        return fn

    def w_gather(c, j):
        def fn():
            for kb in range(NJ):
                parts = [wt_s[kb, pl.ds(c * D + 4 * j + dd, H, stride=DH), :] for dd in range(4)]
                _put(wp_v, kb, c * D + j * L, jnp.concatenate(parts, axis=0))
        return fn

    def wo_widen(nb):
        def fn():
            wo_s[nb] = wo_raw[:, _lanes(nb)].astype(f32)
        return fn

    def wo_gather(nb):
        def fn():
            for j in range(NJ):
                parts = [wo_s[nb, pl.ds(4 * j + dd, H, stride=DH), :] for dd in range(4)]
                _put(wop_v, nb, j * L, jnp.concatenate(parts, axis=0))
        return fn

    def qkv(i, c, j, m0):
        def fn():
            y = lax.dot_general(_full_rows(x_w, i * TM + m0, MS), _full_rows(wp_w, c * D + j * L, L),
                                (((1,), (1,)), ((), ())), preferred_element_type=f32)
            if c == 0:
                q_t[i][j, pl.ds(m0, MS), :] = y
                return
            dst = k_t if c == 1 else v_t
            dst[i][j, pl.ds(HALO + m0, MS), :] = y
            if i + 1 < NT and m0 + MS == TM:
                dst[i + 1][j, pl.ds(0, HALO), :] = y[MS - HALO:]
            if i == 0 and m0 == 0:
                dst[0][j, pl.ds(0, HALO), :] = jnp.broadcast_to(y[0:1], (HALO, L))
        return fn

    half = {}

    def attend(i, r0):
        q = [q_t[i][j, pl.ds(r0, RA), :] for j in range(NJ)]
        z = []
        for w in range(WIN):
            acc = None
            for j in range(NJ):
                t = q[j] * k_t[i][j, pl.ds(HALO + r0 - DIL * w, RA), :]
                acc = t if acc is None else acc + t
            z.append((acc, pltpu.roll(acc, 2 * H, 1)))
        yield
        z = [a + b for a, b in z]
        z = [(a, pltpu.roll(a, H, 1)) for a in z]
        yield
        z = [a + b for a, b in z]
        if i == 0 and r0 < DIL * (WIN - 1):
            pos = r0 + lax.broadcasted_iota(i32, (RA, L), 0)
            z = [jnp.where(pos >= DIL * w, z[w] * SCALE, -1e9) for w in range(WIN)]
            c = LOG2E
        else:
            c = SCALE * LOG2E
        m = z[0]
        for w in range(1, WIN):
            m = jnp.maximum(m, z[w])
        e = [jnp.exp2((z[w] - m) * c) for w in range(WIN)]
        if ATT_DEPTH == 4:
            yield
        den = e[0]
        for w in range(1, WIN):
            den = den + e[w]
        inv = _recip(den)
        for j in range(NJ):
            acc = None
            for w in range(WIN):
                t = e[w] * v_t[i][j, pl.ds(HALO + r0 - DIL * w, RA), :]
                acc = t if acc is None else acc + t
            o = acc * inv
            if RA == RB:
                _put(o_t[i], j, r0, o)
            elif r0 % RB == 0:
                half[i, j] = o
            else:
                _put(o_t[i], j, r0 - RA, jnp.concatenate([half.pop((i, j)), o], axis=0))

    def project(i, nb, m0):
        def fn():
            r0 = i * TM + m0
            a = jnp.dot(_full_rows(o_w[i], m0, MS), _get(wop_w, nb, 0, D), preferred_element_type=f32)
            g = gate_s[pl.ds(r0, MS), :]
            b = _get(x_w, nb, r0, MS).astype(f32)
            if i >= INLINE_FROM:
                row = r0 + lax.broadcasted_iota(i32, (MS, L), 0)
                y0, y1 = (y_s[t, 0:1, _lanes(nb)] for t in range(2))
                b = b + jnp.where(row == sel_s[0], y0, jnp.where(row == sel_s[1], y1, 0.0))
            _put(out_v, nb, r0, b + g * (a - b))
        return fn

    lane = lax.broadcasted_iota(i32, (RB, L), 1)
    score = [jnp.zeros((RB, L), f32)]

    def route(n):
        g, r = _row_dots(x_w, n * RB, vec_s, (0, 1))
        yield
        score[0] = jnp.where(lane == n, r, score[0])
        e = _exp_neg(g)
        yield
        gate_s[pl.ds(n * RB, RB), :] = _recip(1.0 + e)

    def row_group(ref, base, idx):
        word = pl.multiple_of(base // 2, RB // 2)
        rows = [pltpu.bitcast(ref[j, pl.ds(word, RB // 2), :], bf16) for j in range(NJ)]
        hit = lax.broadcasted_iota(i32, (RB, D), 0) == idx - base
        return jnp.concatenate(rows, axis=1).astype(f32), hit, word

    def select_top2():
        r = score[0].astype(bf16).astype(f32)
        r = jnp.where(r == 0.0, 0.0, r)
        bits = pltpu.bitcast(r, i32) >> 16
        key = jnp.where(bits < 0, bits ^ 0x7FFF, bits).astype(f32)
        key = jnp.where(r != r, -1e6, key)
        pos = (lane * RB + lax.broadcasted_iota(i32, (RB, L), 0)).astype(f32)
        for t in range(2):
            best = jnp.max(key, keepdims=True)
            yield
            first = jnp.min(jnp.where(key == best, pos, float(S)), keepdims=True)
            yield
            chosen = pos == first
            key = jnp.where(chosen, -2e6, key)
            r_sel = jnp.sum(jnp.where(chosen, r, 0.0), keepdims=True)
            idx = jnp.clip(first.astype(i32)[0, 0], 0, S - 1)
            yield
            sel_s[t] = idx
            vec_s[4 + t, :, 0:L] = _sigmoid(jnp.broadcast_to(r_sel, (RB, L)))
            grp, hit, _ = row_group(x_w, (idx // RB) * RB, idx)
            vec_s[2 + t] = jnp.broadcast_to(
                jnp.sum(jnp.where(hit, grp, 0.0), axis=0, keepdims=True), (RB, D))
            yield

    y_acc = {}

    def ffn(f0):
        gp = _row_dots(wg_w, f0, vec_s, (2, 3))
        up = _row_dots(wu_w, f0, vec_s, (2, 3))
        yield
        e = [_exp_neg(a) for a in gp]
        if FFN_DEPTH >= 3:
            yield
        sig = [_recip(1.0 + a) for a in e]
        if FFN_DEPTH >= 4:
            yield
        h = [gp[t] * sig[t] * up[t] for t in range(2)]
        for j in range(NJ):
            wd = _get(wd_w, j, f0, RB).astype(f32)
            for t in range(2):
                p = h[t] * wd
                p = p[0:8] + p[8:16]
                y_acc[t, j] = y_acc[t, j] + p if (t, j) in y_acc else p

    def ffn_finish():
        for t in range(2):
            for j in range(NJ):
                y = jnp.sum(y_acc[t, j], axis=0, keepdims=True)
                y_s[t, :, _lanes(j)] = jnp.broadcast_to(y, (RB, L)) * vec_s[4 + t, :, 0:L]

    def patch(t):
        idx = sel_s[t]
        base = jnp.minimum((idx // RB) * RB, INLINE_FROM * TM - RB)
        old, hit, word = row_group(out_w, base, idx)
        g = _sigmoid(jnp.sum(vec_s[2 + t] * vec_s[0], axis=1, keepdims=True))
        new = jnp.where(hit, old + (1.0 - g) * y_s[t], old).astype(bf16)
        for j in range(NJ):
            out_w[j, pl.ds(word, RB // 2), :] = pltpu.bitcast(new[:, _lanes(j)], u32)

    sch = _Schedule()
    mxu = [("qkv", i, c, j) for c in range(3) for i in range(HEAD) for j in range(NJ)]
    for i in range(HEAD, NT + OUT_LAG):
        if i < NT:
            mxu += [("qkv", i, c, j) for c in range(3) for j in range(NJ)]
        if i >= OUT_LAG:
            mxu += [("out", i - OUT_LAG, nb) for nb in range(NJ)]
    slot = {op: n for n, op in enumerate(mxu)}
    for op, n in slot.items():
        for m0 in range(0, TM, MS):
            sch.at(n + m0 / TM, (qkv if op[0] == "qkv" else project)(*op[1:], m0))

    cp_w0 = [copy(wqkv_hbm.at[pl.ds(kb * L, L), pl.ds(0, D)], w_raw.at[pl.ds(kb * L, L), pl.ds(0, D)])
             for kb in range(NJ)]
    cp_w = {c: copy(wqkv_hbm.at[:, pl.ds(c * D, D)], w_raw.at[:, pl.ds(c * D, D)]) for c in (1, 2)}
    cp_x = [load(x_hbm, x_v, 0, TM), load(x_hbm, x_v, TM, (HEAD - 1) * TM),
            load(x_hbm, x_v, HEAD * TM, S - HEAD * TM)]
    cp_vec = _Copies([copy(gw_hbm, gw_v), copy(wr_hbm, wr_v)])
    cp_wo = copy(wo_hbm, wo_raw)
    cuts = (0, FFN_CUT, F)
    cp_f = [_Copies([load(src, dst, cuts[n], cuts[n + 1] - cuts[n])
                     for src, dst in ((wg_hbm, wg_v), (wu_hbm, wu_v), (wd_hbm, wd_v))])
            for n in range(2)]
    for cp in cp_w0 + [cp_x[0]]:
        sch.at(-9, cp.start)
    for kb in range(NJ):
        sch.at(-8 + kb, cp_w0[kb].wait)
        sch.spread(-8 + kb, -7 + kb, [w_transpose(0, kb, cb) for cb in range(NJ)])
    for pos, starts, waits in (
            (T_START[0], (cp_x[1], cp_w[1], cp_vec), ()),
            (-2, (), (cp_x[0],)),
            (T_START[1], (cp_w[2], cp_x[2]), ()),
            (NJ - 0.1, (), (cp_x[1], cp_vec)),
            (T_W[1], (), (cp_w[1],)),
            (T_START[2], (cp_wo, cp_f[0]), ()),
            (T_W[2], (), (cp_w[2],)),
            (T_ROUTE[0], (), (cp_x[2],)),
            (T_START[3], (cp_f[1],), ()),
            (T_WO, (), (cp_wo,)),
            (T_FFN[0], (), (cp_f[0],)),
            (T_FFN[0] + (T_FFN[1] - T_FFN[0]) * FFN_CUT / F - 2, (), (cp_f[1],))):
        for cp in starts:
            sch.at(pos, cp.start)
        for cp in waits:
            sch.at(pos, cp.wait)

    for c in range(3):
        first = slot["qkv", 0, c, 0]
        if c > 0:
            sch.spread(T_W[c], first - 0.8,
                       [w_transpose(c, kb, cb) for cb in range(NJ) for kb in range(NJ)])
        for j in range(NJ):
            sch.at(first + j - 0.7, w_gather(c, j))
    first = slot["out", 0, 0]
    sch.spread(T_WO, min(first - 0.5, T_WO + 10), [fn for nb in range(NJ) for fn in (wo_widen(nb), wo_gather(nb))])

    def vectors():
        for n, ref in enumerate((gw_v, wr_v)):
            vec_s[n] = jnp.broadcast_to(ref[...].astype(f32).reshape(1, D), (RB, D))

    sch.at(5, vectors)
    early = HEAD * TM // RB
    sch.pipeline(*T_EARLY, [route(n) for n in range(early)], 3, 2)
    sch.pipeline(*T_ROUTE, [route(n) for n in range(early, S // RB)], 3, 2)
    picker = select_top2()
    sch.spread(*T_SELECT, [lambda: next(picker)] * 8)

    t0 = 0
    for i in range(NT):
        t0 = max(t0, slot["qkv", max(i, HEAD - 1), 2, NJ - 1] + 1)
        t1 = t0 + min((slot["out", n, 0] - 0.5 - t0) / (n - i + 1) for n in range(i, NT))
        sch.pipeline(t0, t1, [attend(i, r0) for r0 in range(0, TM, RA)], ATT_DEPTH, ATT_LAG)
        t0 = t1

    t0, t1 = T_FFN
    sch.pipeline(t0, t1, [ffn(f0) for f0 in range(0, F, RB)], FFN_DEPTH, FFN_LAG)
    sch.at(t1 + 0.1, ffn_finish)

    cp_out = [store(0, INLINE_FROM * TM, range(NJ))]
    for t in range(2):
        sch.at(t1 + 1 + t, lambda t=t: patch(t))
    sch.at(t1 + 3.5, cp_out[0].start)
    for op, n in slot.items():
        if op[0] == "out" and op[1] >= INLINE_FROM:
            cp_out.append(store(op[1] * TM, TM, [op[2]]))
            sch.at(n + 1.25, cp_out[-1].start)
    for cp in cp_out:
        sch.at(len(mxu) + 2, cp.wait)
    sch.emit()


@jax.jit
def pallas_gated_mix__sliding_local_dilated__moe_arch_mod__prompt_kernel(
    A_x: jax.Array,
    A_wqkv: jax.Array,
    A_wo: jax.Array,
    B_x: jax.Array,
    B_w_r: jax.Array,
    B_w_gate: jax.Array,
    B_w_up: jax.Array,
    B_w_down: jax.Array,
    gate_w: jax.Array,
):
    n_sems = 2 + 2 + 1 + NJ * (1 + 3 + 6 + 1 + NT - INLINE_FROM)
    scratch = [
        pltpu.VMEM((NJ, S, L), bf16),
        pltpu.VMEM((NJ, S, L), bf16),
        pltpu.VMEM((D, 3 * D), bf16),
        pltpu.VMEM((D, D), bf16),
        pltpu.VMEM((NJ, F, L), bf16),
        pltpu.VMEM((NJ, F, L), bf16),
        pltpu.VMEM((NJ, F, L), bf16),
        pltpu.VMEM((D,), bf16),
        pltpu.VMEM((D,), bf16),
        pltpu.VMEM((NJ, 3 * D, L), f32),
        pltpu.VMEM((NJ, 3 * D, L), bf16),
        pltpu.VMEM((NJ, D, L), f32),
        pltpu.VMEM((NJ, D, L), bf16),
        pltpu.VMEM((S, L), f32),
        pltpu.VMEM((6, RB, D), f32),
        pltpu.VMEM((2, RB, D), f32),
        pltpu.SMEM((2,), i32),
        pltpu.SemaphoreType.DMA((n_sems,)),
    ]
    scratch += [pltpu.VMEM((NJ, TM, L), f32)] * NT
    scratch += [pltpu.VMEM((NJ, HALO + TM, L), f32)] * (2 * NT)
    scratch += [pltpu.VMEM((NJ, TM, L), bf16)] * NT
    out = pl.pallas_call(
        _kernel,
        out_shape=jax.ShapeDtypeStruct((S, D), bf16),
        in_specs=[pl.BlockSpec(memory_space=pl.ANY)] * 8,
        out_specs=pl.BlockSpec(memory_space=pl.ANY),
        scratch_shapes=scratch,
        compiler_params=pltpu.CompilerParams(vmem_limit_bytes=100 * 2**20, flags=FLAGS),
        name="gated_mix",
    )(A_x.reshape(S, D), A_wqkv, A_wo, B_w_r,
      B_w_gate.T, B_w_up.T, B_w_down, gate_w)
    return out.reshape(1, S, D)
```

```python
import numpy as np

import jax
import jax.numpy as jnp
from jax import lax
import jax.experimental.pallas as pl
import jax.experimental.pallas.tpu as pltpu

S, D, F = 2048, 640, 1728
H, DH = 32, 20
WIN, DIL = 8, 2
HALO = 16
L = 128
NJ = D // L
TM = 256
NT = S // TM
RB = 16
SCALE = float(DH) ** -0.5
LOG2E = float(np.log2(np.e))
INLINE_FROM = 1280

HEAD = 2
OUT_LAG = 2
T_START = (-5.5, -4.5, 2.5, 36.0)
T_W = (None, 6.5, 15.0)
T_EARLY = (10.0, 15.0)
T_ROUTE = (27.0, 37.0)
T_SELECT = (38.0, 45.0)
T_FFN = (46.0, 138.0)
FFN_CUT = 640
FLAGS = None
MS = 128
RA = 8
ATT_LAG = 1
FFN_LAG = 1
SKEW = 0.04
REV = False
ATT_DEPTH = 4
FFN_DEPTH = 4

f32, bf16, u32, i32 = jnp.float32, jnp.bfloat16, jnp.uint32, jnp.int32


class _Schedule:
    def __init__(self):
        self.items = []

    def at(self, pos, fn):
        self.items.append((pos, len(self.items), fn))

    def spread(self, t0, t1, fns):
        for n, fn in enumerate(fns):
            self.at(t0 + (n + 0.5) * (t1 - t0) / len(fns), fn)

    def pipeline(self, t0, t1, gens, depth, lag=1, warp=lambda t: t):
        step = (t1 - t0) / (len(gens) + (depth - 1) * lag)
        for n, gen in enumerate(gens):
            for s in range(depth):
                phase = (depth - s if REV else s) * SKEW / depth
                self.at(warp(t0 + (n + s * lag + 0.5 * (1 - SKEW) + phase) * step),
                        lambda gen=gen: next(gen, None))

    def emit(self):
        for _, _, fn in sorted(self.items, key=lambda it: it[:2]):
            fn()


class _Copies:
    def __init__(self, copies):
        self.copies = copies

    def start(self):
        for cp in self.copies:
            cp.start()

    def wait(self):
        for cp in self.copies:
            cp.wait()


def _recip(d):
    r = pl.reciprocal(d, approx=True)
    return r * (2.0 - d * r)


def _exp_neg(z):
    return jnp.minimum(jnp.exp(-z), 1e38)


def _sigmoid(z):
    return _recip(1.0 + _exp_neg(z))


def _lanes(j):
    return slice(j * L, (j + 1) * L)


def _get(ref, j, r0, n):
    return pltpu.bitcast(ref[j, pl.ds(r0 // 2, n // 2), :], bf16)


def _full_rows(ref, r0, n):
    return jnp.concatenate([_get(ref, j, r0, n) for j in range(NJ)], axis=1)


def _put(ref, j, r0, val):
    ref[j, pl.ds(r0, val.shape[0]), :] = val.astype(bf16)


def _row_dots(rows_ref, r0, vec_ref, vs):
    acc = [None] * len(vs)
    for j in range(NJ):
        rows = _get(rows_ref, j, r0, RB).astype(f32)
        for n, v in enumerate(vs):
            vec = vec_ref[v, 0:8, _lanes(j)]
            t = rows * jnp.concatenate([vec, vec], axis=0)
            acc[n] = t if acc[n] is None else acc[n] + t
    return [jnp.broadcast_to(jnp.sum(a, axis=1, keepdims=True), (RB, L)) for a in acc]


def _kernel(x_hbm, wqkv_hbm, wo_hbm, wr_hbm, wg_hbm, wu_hbm, wd_hbm, gw_hbm,
            out_hbm,
            x_v, out_v, w_raw, wo_raw, wg_v, wu_v, wd_v, gw_v, wr_v,
            wt_s, wp_v, wo_s, wop_v, gate_s, vec_s, y_s, sel_s, sems, *tiles):
    q_t, k_t, v_t, o_t = (tiles[i * NT:(i + 1) * NT] for i in range(4))
    x_w, out_w, wg_w, wu_w, wd_w, wp_w, wop_w = (
        r.bitcast(u32) for r in (x_v, out_v, wg_v, wu_v, wd_v, wp_v, wop_v))
    o_w = [r.bitcast(u32) for r in o_t]

    sem_ids = iter(range(sems.shape[0]))

    def copy(src, dst):
        return pltpu.make_async_copy(src, dst, sems.at[next(sem_ids)])

    def load(src, dst, r0, n):
        return _Copies([copy(src.at[pl.ds(r0, n), pl.ds(j * L, L)], dst.at[j, pl.ds(r0, n), :])
                        for j in range(NJ)])

    def store(r0, n, groups):
        return _Copies([copy(out_v.at[j, pl.ds(r0, n), :], out_hbm.at[pl.ds(r0, n), pl.ds(j * L, L)])
                        for j in groups])

    def w_transpose(c, kb, cb):
        def fn():
            blk = w_raw[pl.ds(kb * L, L), pl.ds(c * D + cb * L, L)].astype(f32)
            wt_s[kb, pl.ds(c * D + cb * L, L), :] = blk.T
        return fn

    def w_gather(c, j):
        def fn():
            for kb in range(NJ):
                parts = [wt_s[kb, pl.ds(c * D + 4 * j + dd, H, stride=DH), :] for dd in range(4)]
                _put(wp_v, kb, c * D + j * L, jnp.concatenate(parts, axis=0))
        return fn

    def wo_widen(nb):
        def fn():
            wo_s[nb] = wo_raw[:, _lanes(nb)].astype(f32)
        return fn

    def wo_gather(nb):
        def fn():
            for j in range(NJ):
                parts = [wo_s[nb, pl.ds(4 * j + dd, H, stride=DH), :] for dd in range(4)]
                _put(wop_v, nb, j * L, jnp.concatenate(parts, axis=0))
        return fn

    def qkv(i, c, j, m0):
        def fn():
            y = lax.dot_general(_full_rows(x_w, i * TM + m0, MS), _full_rows(wp_w, c * D + j * L, L),
                                (((1,), (1,)), ((), ())), preferred_element_type=f32)
            if c == 0:
                q_t[i][j, pl.ds(m0, MS), :] = y
                return
            dst = k_t if c == 1 else v_t
            dst[i][j, pl.ds(HALO + m0, MS), :] = y
            if i + 1 < NT and m0 + MS == TM:
                dst[i + 1][j, pl.ds(0, HALO), :] = y[MS - HALO:]
            if i == 0 and m0 == 0:
                dst[0][j, pl.ds(0, HALO), :] = jnp.broadcast_to(y[0:1], (HALO, L))
        return fn

    half = {}

    def attend(i, r0):
        q = [q_t[i][j, pl.ds(r0, RA), :] for j in range(NJ)]
        z = []
        for w in range(WIN):
            acc = None
            for j in range(NJ):
                t = q[j] * k_t[i][j, pl.ds(HALO + r0 - DIL * w, RA), :]
                acc = t if acc is None else acc + t
            z.append((acc, pltpu.roll(acc, 2 * H, 1)))
        yield
        z = [a + b for a, b in z]
        z = [(a, pltpu.roll(a, H, 1)) for a in z]
        yield
        z = [a + b for a, b in z]
        if i == 0 and r0 < DIL * (WIN - 1):
            pos = r0 + lax.broadcasted_iota(i32, (RA, L), 0)
            z = [jnp.where(pos >= DIL * w, z[w] * SCALE, -1e9) for w in range(WIN)]
            c = LOG2E
        else:
            c = SCALE * LOG2E
        m = z[0]
        for w in range(1, WIN):
            m = jnp.maximum(m, z[w])
        e = [jnp.exp2((z[w] - m) * c) for w in range(WIN)]
        if ATT_DEPTH == 4:
            yield
        den = e[0]
        for w in range(1, WIN):
            den = den + e[w]
        inv = _recip(den)
        for j in range(NJ):
            acc = None
            for w in range(WIN):
                t = e[w] * v_t[i][j, pl.ds(HALO + r0 - DIL * w, RA), :]
                acc = t if acc is None else acc + t
            o = acc * inv
            if RA == RB:
                _put(o_t[i], j, r0, o)
            elif r0 % RB == 0:
                half[i, j] = o
            else:
                _put(o_t[i], j, r0 - RA, jnp.concatenate([half.pop((i, j)), o], axis=0))

    def project(i, nb, m0):
        def fn():
            r0 = i * TM + m0
            a = jnp.dot(_full_rows(o_w[i], m0, MS), _get(wop_w, nb, 0, D), preferred_element_type=f32)
            g = gate_s[pl.ds(r0, MS), :]
            b = _get(x_w, nb, r0, MS).astype(f32)
            if r0 >= INLINE_FROM:
                row = r0 + lax.broadcasted_iota(i32, (MS, L), 0)
                y0, y1 = (y_s[t, 0:1, _lanes(nb)] for t in range(2))
                b = b + jnp.where(row == sel_s[0], y0, jnp.where(row == sel_s[1], y1, 0.0))
            _put(out_v, nb, r0, b + g * (a - b))
        return fn

    lane = lax.broadcasted_iota(i32, (RB, L), 1)
    score = [jnp.zeros((RB, L), f32)]

    def route(n):
        g, r = _row_dots(x_w, n * RB, vec_s, (0, 1))
        yield
        score[0] = jnp.where(lane == n, r, score[0])
        e = _exp_neg(g)
        yield
        gate_s[pl.ds(n * RB, RB), :] = _recip(1.0 + e)

    def row_group(ref, base, idx):
        word = pl.multiple_of(base // 2, RB // 2)
        rows = [pltpu.bitcast(ref[j, pl.ds(word, RB // 2), :], bf16) for j in range(NJ)]
        hit = lax.broadcasted_iota(i32, (RB, D), 0) == idx - base
        return jnp.concatenate(rows, axis=1).astype(f32), hit, word

    def select_top2():
        r = score[0].astype(bf16).astype(f32)
        r = jnp.where(r == 0.0, 0.0, r)
        bits = pltpu.bitcast(r, i32) >> 16
        key = jnp.where(bits < 0, bits ^ 0x7FFF, bits).astype(f32)
        key = jnp.where(r != r, -1e6, key)
        pos = (lane * RB + lax.broadcasted_iota(i32, (RB, L), 0)).astype(f32)
        for t in range(2):
            best = jnp.max(key, keepdims=True)
            yield
            first = jnp.min(jnp.where(key == best, pos, float(S)), keepdims=True)
            yield
            chosen = pos == first
            key = jnp.where(chosen, -2e6, key)
            r_sel = jnp.sum(jnp.where(chosen, r, 0.0), keepdims=True)
            idx = jnp.clip(first.astype(i32)[0, 0], 0, S - 1)
            yield
            sel_s[t] = idx
            vec_s[4 + t, :, 0:L] = _sigmoid(jnp.broadcast_to(r_sel, (RB, L)))
            grp, hit, _ = row_group(x_w, (idx // RB) * RB, idx)
            vec_s[2 + t] = jnp.broadcast_to(
                jnp.sum(jnp.where(hit, grp, 0.0), axis=0, keepdims=True), (RB, D))
            yield

    y_acc = {}

    def ffn(f0):
        gp = _row_dots(wg_w, f0, vec_s, (2, 3))
        up = _row_dots(wu_w, f0, vec_s, (2, 3))
        yield
        e = [_exp_neg(a) for a in gp]
        if FFN_DEPTH >= 3:
            yield
        sig = [_recip(1.0 + a) for a in e]
        if FFN_DEPTH >= 4:
            yield
        h = [gp[t] * sig[t] * up[t] for t in range(2)]
        for j in range(NJ):
            wd = _get(wd_w, j, f0, RB).astype(f32)
            for t in range(2):
                p = h[t] * wd
                p = p[0:8] + p[8:16]
                y_acc[t, j] = y_acc[t, j] + p if (t, j) in y_acc else p

    def ffn_finish():
        for t in range(2):
            for j in range(NJ):
                y = jnp.sum(y_acc[t, j], axis=0, keepdims=True)
                y_s[t, :, _lanes(j)] = jnp.broadcast_to(y, (RB, L)) * vec_s[4 + t, :, 0:L]

    def patch(t):
        idx = sel_s[t]
        base = jnp.minimum((idx // RB) * RB, INLINE_FROM - RB)
        old, hit, word = row_group(out_w, base, idx)
        g = _sigmoid(jnp.sum(vec_s[2 + t] * vec_s[0], axis=1, keepdims=True))
        new = jnp.where(hit, old + (1.0 - g) * y_s[t], old).astype(bf16)
        for j in range(NJ):
            out_w[j, pl.ds(word, RB // 2), :] = pltpu.bitcast(new[:, _lanes(j)], u32)

    sch = _Schedule()
    halves = range(0, TM, MS)
    mxu = [("qkv", i, c, j, m0) for c in range(3) for i in range(HEAD) for m0 in halves for j in range(NJ)]
    for i in range(HEAD, NT + OUT_LAG):
        if i < NT:
            mxu += [("qkv", i, c, j, m0) for c in range(3) for j in range(NJ) for m0 in halves]
        if i >= OUT_LAG:
            mxu += [("out", i - OUT_LAG, nb, m0) for nb in range(NJ) for m0 in halves]
    dt = MS / 256
    slot = {op: n * dt for n, op in enumerate(mxu)}
    for op, t in slot.items():
        sch.at(t, (qkv if op[0] == "qkv" else project)(*op[1:]))

    cp_w0 = [copy(wqkv_hbm.at[pl.ds(kb * L, L), pl.ds(0, D)], w_raw.at[pl.ds(kb * L, L), pl.ds(0, D)])
             for kb in range(NJ)]
    cp_w = {c: copy(wqkv_hbm.at[:, pl.ds(c * D, D)], w_raw.at[:, pl.ds(c * D, D)]) for c in (1, 2)}
    cp_x = [load(x_hbm, x_v, 0, MS), load(x_hbm, x_v, MS, HEAD * TM - MS),
            load(x_hbm, x_v, HEAD * TM, S - HEAD * TM)]
    cp_vec = _Copies([copy(gw_hbm, gw_v), copy(wr_hbm, wr_v)])
    cp_wo = copy(wo_hbm, wo_raw)
    cuts = (0, FFN_CUT, F)
    cp_f = [_Copies([load(src, dst, cuts[n], cuts[n + 1] - cuts[n])
                     for src, dst in ((wg_hbm, wg_v), (wu_hbm, wu_v), (wd_hbm, wd_v))])
            for n in range(2)]
    for cp in [cp_x[0]] + cp_w0:
        sch.at(-9, cp.start)
    sch.at(-8.5, cp_x[0].wait)
    for kb in range(NJ):
        sch.at(-8 + kb, cp_w0[kb].wait)
        sch.spread(-8 + kb, -7 + kb, [w_transpose(0, kb, cb) for cb in range(NJ)])
    for pos, starts, waits in (
            (T_START[0], (cp_x[1], cp_vec), ()),
            (T_START[1], (cp_w[1],), ()),
            (NJ * dt - 0.1, (), (cp_x[1], cp_vec)),
            (T_START[2], (cp_w[2],), ()),
            (T_W[1], (cp_x[2],), (cp_w[1],)),
            (T_W[2], (cp_wo,), (cp_w[2],)),
            (T_ROUTE[0], (cp_f[0],), (cp_x[2], cp_wo)),
            (T_START[3], (cp_f[1],), ()),
            (T_FFN[0], (), (cp_f[0],)),
            (T_FFN[0] + (T_FFN[1] - T_FFN[0]) * FFN_CUT / F - 2, (), (cp_f[1],))):
        for cp in starts:
            sch.at(pos, cp.start)
        for cp in waits:
            sch.at(pos, cp.wait)

    for c in range(3):
        first = slot["qkv", 0, c, 0, 0]
        if c > 0:
            sch.spread(T_W[c], first - 0.8,
                       [w_transpose(c, kb, cb) for cb in range(NJ) for kb in range(NJ)])
        for j in range(NJ):
            sch.at(first + (j - 1.4) * dt, w_gather(c, j))
    first = slot["out", 0, 0, 0]
    sch.spread(T_ROUTE[0], min(first - 0.5, T_ROUTE[0] + 10), [fn for nb in range(NJ) for fn in (wo_widen(nb), wo_gather(nb))])

    def vectors():
        for n, ref in enumerate((gw_v, wr_v)):
            vec_s[n] = jnp.broadcast_to(ref[...].astype(f32).reshape(1, D), (RB, D))

    sch.at(5, vectors)
    early = HEAD * TM // RB
    sch.pipeline(*T_EARLY, [route(n) for n in range(early)], 3, 2)
    sch.pipeline(*T_ROUTE, [route(n) for n in range(early, S // RB)], 3, 2)
    picker = select_top2()
    sch.spread(*T_SELECT, [lambda: next(picker)] * 8)

    t0 = 0
    for i in range(NT):
        t0 = max(t0, slot["qkv", max(i, HEAD - 1), 2, NJ - 1, TM - MS] + dt)
        t1 = t0 + min((slot["out", n, 0, 0] - 0.5 - t0) / (n - i + 1) for n in range(i, NT))
        sch.pipeline(t0, t1, [attend(i, r0) for r0 in range(0, TM, RA)], ATT_DEPTH, ATT_LAG)
        t0 = t1

    t0, t1 = T_FFN
    sch.pipeline(t0, t1, [ffn(f0) for f0 in range(0, F, RB)], FFN_DEPTH, FFN_LAG)
    sch.at(t1 + 0.1, ffn_finish)

    cp_out = [store(0, INLINE_FROM, range(NJ))]
    for t in range(2):
        sch.at(t1 + 1 + t, lambda t=t: patch(t))
    sch.at(t1 + 3.5, cp_out[0].start)
    for op, n in slot.items():
        if op[0] == "out" and op[1] * TM >= INLINE_FROM and op[3] == TM - MS:
            cp_out.append(store(op[1] * TM, TM, [op[2]]))
            sch.at(n + 0.75, cp_out[-1].start)
    for cp in cp_out:
        sch.at(len(mxu) * dt + 2, cp.wait)
    sch.emit()


@jax.jit
def pallas_gated_mix__sliding_local_dilated__moe_arch_mod__prompt_kernel(
    A_x: jax.Array,
    A_wqkv: jax.Array,
    A_wo: jax.Array,
    B_x: jax.Array,
    B_w_r: jax.Array,
    B_w_gate: jax.Array,
    B_w_up: jax.Array,
    B_w_down: jax.Array,
    gate_w: jax.Array,
):
    n_sems = 2 + 2 + 1 + NJ * (1 + 3 + 6 + 1 + (S - INLINE_FROM) // TM)
    scratch = [
        pltpu.VMEM((NJ, S, L), bf16),
        pltpu.VMEM((NJ, S, L), bf16),
        pltpu.VMEM((D, 3 * D), bf16),
        pltpu.VMEM((D, D), bf16),
        pltpu.VMEM((NJ, F, L), bf16),
        pltpu.VMEM((NJ, F, L), bf16),
        pltpu.VMEM((NJ, F, L), bf16),
        pltpu.VMEM((D,), bf16),
        pltpu.VMEM((D,), bf16),
        pltpu.VMEM((NJ, 3 * D, L), f32),
        pltpu.VMEM((NJ, 3 * D, L), bf16),
        pltpu.VMEM((NJ, D, L), f32),
        pltpu.VMEM((NJ, D, L), bf16),
        pltpu.VMEM((S, L), f32),
        pltpu.VMEM((6, RB, D), f32),
        pltpu.VMEM((2, RB, D), f32),
        pltpu.SMEM((2,), i32),
        pltpu.SemaphoreType.DMA((n_sems,)),
    ]
    scratch += [pltpu.VMEM((NJ, TM, L), f32)] * NT
    scratch += [pltpu.VMEM((NJ, HALO + TM, L), f32)] * (2 * NT)
    scratch += [pltpu.VMEM((NJ, TM, L), bf16)] * NT
    out = pl.pallas_call(
        _kernel,
        out_shape=jax.ShapeDtypeStruct((S, D), bf16),
        in_specs=[pl.BlockSpec(memory_space=pl.ANY)] * 8,
        out_specs=pl.BlockSpec(memory_space=pl.ANY),
        scratch_shapes=scratch,
        compiler_params=pltpu.CompilerParams(vmem_limit_bytes=100 * 2**20, flags=FLAGS),
        name="gated_mix",
    )(A_x.reshape(S, D), A_wqkv, A_wo, B_w_r,
      B_w_gate.T, B_w_up.T, B_w_down, gate_w)
    return out.reshape(1, S, D)
```

```python
import numpy as np

import jax
import jax.numpy as jnp
from jax import lax
import jax.experimental.pallas as pl
import jax.experimental.pallas.tpu as pltpu

S, D, F = 2048, 640, 1728
H, DH = 32, 20
WIN, DIL = 8, 2
HALO = 16
L = 128
NJ = D // L
TM = 256
NT = S // TM
RB = 16
SCALE = float(DH) ** -0.5
LOG2E = float(np.log2(np.e))

HEAD = 2
OUT_LAG = 2
LATE = (NT - OUT_LAG - 1) * TM
T_START = (-5.5, -4.5, 2.5, 36.0)
T_W = (None, 6.5, 15.0)
T_EARLY = (10.0, 15.0)
T_ROUTE = (27.0, 37.0)
T_SELECT = (38.0, 45.0)
T_FFN = (46.0, 138.0)
FFN_CUT = 640
FLAGS = None
ATT0 = 1
MS = 128
RA = 8
ATT_LAG = 1
FFN_LAG = 1
SKEW = 0.04
REV = False
ATT_DEPTH = 4
FFN_DEPTH = 4

f32, bf16, u32, i32 = jnp.float32, jnp.bfloat16, jnp.uint32, jnp.int32


class _Schedule:
    def __init__(self):
        self.items = []

    def at(self, pos, fn):
        self.items.append((pos, len(self.items), fn))

    def spread(self, t0, t1, fns):
        for n, fn in enumerate(fns):
            self.at(t0 + (n + 0.5) * (t1 - t0) / len(fns), fn)

    def pipeline(self, t0, t1, gens, depth, lag=1, warp=lambda t: t):
        step = (t1 - t0) / (len(gens) + (depth - 1) * lag)
        for n, gen in enumerate(gens):
            for s in range(depth):
                phase = (depth - s if REV else s) * SKEW / depth
                self.at(warp(t0 + (n + s * lag + 0.5 * (1 - SKEW) + phase) * step),
                        lambda gen=gen: next(gen, None))

    def emit(self):
        for _, _, fn in sorted(self.items, key=lambda it: it[:2]):
            fn()


class _Copies:
    def __init__(self, copies):
        self.copies = copies

    def start(self):
        for cp in self.copies:
            cp.start()

    def wait(self):
        for cp in self.copies:
            cp.wait()


def _recip(d):
    r = pl.reciprocal(d, approx=True)
    return r * (2.0 - d * r)


def _exp_neg(z):
    return jnp.minimum(jnp.exp2(z * -LOG2E), 1e38)


def _sigmoid(z):
    return _recip(1.0 + _exp_neg(z))


def _lanes(j):
    return slice(j * L, (j + 1) * L)


def _get(ref, j, r0, n):
    return pltpu.bitcast(ref[j, pl.ds(r0 // 2, n // 2), :], bf16)


def _full_rows(ref, r0, n):
    return jnp.concatenate([_get(ref, j, r0, n) for j in range(NJ)], axis=1)


def _put(ref, j, r0, val):
    ref[j, pl.ds(r0, val.shape[0]), :] = val.astype(bf16)


def _row_dots(rows_ref, r0, vec_ref, vs):
    acc = [None] * len(vs)
    for j in range(NJ):
        rows = _get(rows_ref, j, r0, RB).astype(f32)
        for n, v in enumerate(vs):
            vec = vec_ref[v, 0:8, _lanes(j)]
            t = rows * jnp.concatenate([vec, vec], axis=0)
            acc[n] = t if acc[n] is None else acc[n] + t
    return [jnp.broadcast_to(jnp.sum(a, axis=1, keepdims=True), (RB, L)) for a in acc]


def _kernel(x_hbm, wqkv_hbm, wo_hbm, wr_hbm, wg_hbm, wu_hbm, wd_hbm, gw_hbm,
            out_hbm,
            x_v, out_v, w_raw, wo_raw, wg_v, wu_v, wd_v, gw_v, wr_v,
            wt_s, wp_v, wo_s, wop_v, gate_s, vec_s, y_s, sel_s, sems, *tiles):
    q_t, k_t, v_t, o_t = (tiles[i * NT:(i + 1) * NT] for i in range(4))
    x_w, out_w, wg_w, wu_w, wd_w, wp_w, wop_w = (
        r.bitcast(u32) for r in (x_v, out_v, wg_v, wu_v, wd_v, wp_v, wop_v))
    o_w = [r.bitcast(u32) for r in o_t]

    sem_ids = iter(range(sems.shape[0]))

    def copy(src, dst):
        return pltpu.make_async_copy(src, dst, sems.at[next(sem_ids)])

    def load(src, dst, r0, n):
        return _Copies([copy(src.at[pl.ds(r0, n), pl.ds(j * L, L)], dst.at[j, pl.ds(r0, n), :])
                        for j in range(NJ)])

    def store(r0, n, groups):
        return _Copies([copy(out_v.at[j, pl.ds(r0, n), :], out_hbm.at[pl.ds(r0, n), pl.ds(j * L, L)])
                        for j in groups])

    def w_transpose(c, kb, cb):
        def fn():
            blk = w_raw[pl.ds(kb * L, L), pl.ds(c * D + cb * L, L)].astype(f32)
            wt_s[kb, pl.ds(c * D + cb * L, L), :] = blk.T
        return fn

    def w_gather(c, j):
        def fn():
            for kb in range(NJ):
                parts = [wt_s[kb, pl.ds(c * D + 4 * j + dd, H, stride=DH), :] for dd in range(4)]
                _put(wp_v, kb, c * D + j * L, jnp.concatenate(parts, axis=0))
        return fn

    def wo_widen(nb):
        def fn():
            wo_s[nb] = wo_raw[:, _lanes(nb)].astype(f32)
        return fn

    def wo_gather(nb):
        def fn():
            for j in range(NJ):
                parts = [wo_s[nb, pl.ds(4 * j + dd, H, stride=DH), :] for dd in range(4)]
                _put(wop_v, nb, j * L, jnp.concatenate(parts, axis=0))
        return fn

    def qkv(i, c, j, m0):
        def fn():
            y = lax.dot_general(_full_rows(x_w, i * TM + m0, MS), _full_rows(wp_w, c * D + j * L, L),
                                (((1,), (1,)), ((), ())), preferred_element_type=f32)
            if c == 0:
                q_t[i][j, pl.ds(m0, MS), :] = y
                return
            dst = k_t if c == 1 else v_t
            dst[i][j, pl.ds(HALO + m0, MS), :] = y
            if i + 1 < NT and m0 + MS == TM:
                dst[i + 1][j, pl.ds(0, HALO), :] = y[MS - HALO:]
            if i == 0 and m0 == 0:
                dst[0][j, pl.ds(0, HALO), :] = jnp.broadcast_to(y[0:1], (HALO, L))
        return fn

    half = {}

    def attend(i, r0):
        q = [q_t[i][j, pl.ds(r0, RA), :] for j in range(NJ)]
        z = []
        for w in range(WIN):
            acc = None
            for j in range(NJ):
                t = q[j] * k_t[i][j, pl.ds(HALO + r0 - DIL * w, RA), :]
                acc = t if acc is None else acc + t
            z.append((acc, pltpu.roll(acc, 2 * H, 1)))
        yield
        z = [a + b for a, b in z]
        z = [(a, pltpu.roll(a, H, 1)) for a in z]
        yield
        z = [a + b for a, b in z]
        if i == 0 and r0 < DIL * (WIN - 1):
            pos = r0 + lax.broadcasted_iota(i32, (RA, L), 0)
            z = [jnp.where(pos >= DIL * w, z[w] * SCALE, -1e9) for w in range(WIN)]
            c = LOG2E
        else:
            c = SCALE * LOG2E
        m = z[0]
        for w in range(1, WIN):
            m = jnp.maximum(m, z[w])
        e = [jnp.exp2((z[w] - m) * c) for w in range(WIN)]
        if ATT_DEPTH == 4:
            yield
        den = e[0]
        for w in range(1, WIN):
            den = den + e[w]
        inv = _recip(den)
        for j in range(NJ):
            acc = None
            for w in range(WIN):
                t = e[w] * v_t[i][j, pl.ds(HALO + r0 - DIL * w, RA), :]
                acc = t if acc is None else acc + t
            o = acc * inv
            if RA == RB:
                _put(o_t[i], j, r0, o)
            elif r0 % RB == 0:
                half[i, j] = o
            else:
                _put(o_t[i], j, r0 - RA, jnp.concatenate([half.pop((i, j)), o], axis=0))

    def project(i, nb, m0):
        def fn():
            r0 = i * TM + m0
            a = jnp.dot(_full_rows(o_w[i], m0, MS), _get(wop_w, nb, 0, D), preferred_element_type=f32)
            g = gate_s[pl.ds(r0, MS), :]
            b = _get(x_w, nb, r0, MS).astype(f32)
            _put(out_v, nb, r0, b + g * (a - b))
        return fn

    lane = lax.broadcasted_iota(i32, (RB, L), 1)
    score = [jnp.zeros((RB, L), f32)]

    def route(n):
        g, r = _row_dots(x_w, n * RB, vec_s, (0, 1))
        yield
        score[0] = jnp.where(lane == n, r, score[0])
        e = _exp_neg(g)
        yield
        gate_s[pl.ds(n * RB, RB), :] = _recip(1.0 + e)

    def row_group(ref, base, idx):
        word = pl.multiple_of(base // 2, RB // 2)
        rows = [pltpu.bitcast(ref[j, pl.ds(word, RB // 2), :], bf16) for j in range(NJ)]
        hit = lax.broadcasted_iota(i32, (RB, D), 0) == idx - base
        return jnp.concatenate(rows, axis=1).astype(f32), hit, word

    def select_top2():
        r = score[0].astype(bf16).astype(f32)
        r = jnp.where(r == 0.0, 0.0, r)
        bits = pltpu.bitcast(r, i32) >> 16
        key = jnp.where(bits < 0, bits ^ 0x7FFF, bits)
        key = jnp.where(r != r, -(1 << 15) - 1, key).astype(f32)
        row = lax.broadcasted_iota(i32, (RB, L), 0).astype(f32)
        back = (L - 1 - lane[0:1]).astype(f32)
        in_lane = []
        for _ in range(2):
            best = jnp.max(key, axis=0, keepdims=True)
            first = jnp.min(jnp.where(key == best, row, float(RB)), axis=0, keepdims=True)
            here = row == first
            in_lane.append((best * L + back, first, jnp.sum(jnp.where(here, r, 0.0), axis=0, keepdims=True)))
            key = jnp.where(here, -float(1 << 16), key)
        top = jnp.max(in_lane[0][0], axis=1, keepdims=True)
        yield
        won = in_lane[0][0] == top
        rest = [jnp.where(won, b, a) for a, b in zip(*in_lane)]
        top = jnp.max(rest[0], axis=1, keepdims=True)
        yield
        picks = []
        for cand, hit in ((in_lane[0], won), (rest, rest[0] == top)):
            pos = (L - 1 - back) * RB + cand[1]
            picks.append([jnp.sum(jnp.where(hit, v, 0.0), axis=1, keepdims=True) for v in (pos, cand[2])])
        yield
        ids = [jnp.clip(pos.astype(i32)[0, 0], 0, S - 1) for pos, _ in picks]
        yield
        for t, idx in enumerate(ids):
            sel_s[t] = idx
            vec_s[4 + t, :, 0:L] = _sigmoid(jnp.broadcast_to(picks[t][1], (RB, L)))
            grp, hit, _ = row_group(x_w, (idx // RB) * RB, idx)
            vec_s[2 + t] = jnp.broadcast_to(
                jnp.sum(jnp.where(hit, grp, 0.0), axis=0, keepdims=True), (RB, D))

    y_acc = {}

    def ffn(f0):
        gp = _row_dots(wg_w, f0, vec_s, (2, 3))
        up = _row_dots(wu_w, f0, vec_s, (2, 3))
        yield
        e = [_exp_neg(a) for a in gp]
        if FFN_DEPTH >= 3:
            yield
        sig = [_recip(1.0 + a) for a in e]
        if FFN_DEPTH >= 4:
            yield
        h = [gp[t] * sig[t] * up[t] for t in range(2)]
        for j in range(NJ):
            wd = _get(wd_w, j, f0, RB).astype(f32)
            for t in range(2):
                p = h[t] * wd
                p = p[0:8] + p[8:16]
                y_acc[t, j] = y_acc[t, j] + p if (t, j) in y_acc else p

    def ffn_finish():
        for t in range(2):
            for j in range(NJ):
                y = jnp.sum(y_acc[t, j], axis=0, keepdims=True)
                y_s[t, :, _lanes(j)] = jnp.broadcast_to(y, (RB, L)) * vec_s[4 + t, :, 0:L]

    def add_to_row(ref, base, idx, term):
        old, hit, word = row_group(ref, base, idx)
        new = jnp.where(hit, old + term, old).astype(bf16)
        for j in range(NJ):
            ref[j, pl.ds(word, RB // 2), :] = pltpu.bitcast(new[:, _lanes(j)], u32)

    def patch_output(t):
        idx = sel_s[t]
        g = _sigmoid(jnp.sum(vec_s[2 + t] * vec_s[0], axis=1, keepdims=True))
        add_to_row(out_w, jnp.minimum((idx // RB) * RB, LATE - RB), idx, (1.0 - g) * y_s[t])

    def patch_residual(t):
        idx = sel_s[t]
        add_to_row(x_w, (idx // RB) * RB, idx, y_s[t])

    sch = _Schedule()
    halves = range(0, TM, MS)
    mxu = [("qkv", i, c, j, m0) for c in range(3) for i in range(HEAD) for m0 in halves for j in range(NJ)]
    for i in range(HEAD, NT + OUT_LAG):
        if i < NT:
            mxu += [("qkv", i, c, j, m0) for c in range(3) for j in range(NJ) for m0 in halves]
        if i >= OUT_LAG:
            mxu += [("out", i - OUT_LAG, nb, m0) for nb in range(NJ) for m0 in halves]
    dt = MS / 256
    slot = {op: n * dt for n, op in enumerate(mxu)}
    for op, t in slot.items():
        sch.at(t, (qkv if op[0] == "qkv" else project)(*op[1:]))

    cp_w0 = [copy(wqkv_hbm.at[pl.ds(kb * L, L), pl.ds(0, D)], w_raw.at[pl.ds(kb * L, L), pl.ds(0, D)])
             for kb in range(NJ)]
    cp_w = {c: copy(wqkv_hbm.at[:, pl.ds(c * D, D)], w_raw.at[:, pl.ds(c * D, D)]) for c in (1, 2)}
    cp_x = [load(x_hbm, x_v, 0, MS), load(x_hbm, x_v, MS, HEAD * TM - MS),
            load(x_hbm, x_v, HEAD * TM, S - HEAD * TM)]
    cp_vec = _Copies([copy(gw_hbm, gw_v), copy(wr_hbm, wr_v)])
    cp_wo = copy(wo_hbm, wo_raw)
    cuts = (0, FFN_CUT, F)
    cp_f = [_Copies([load(src, dst, cuts[n], cuts[n + 1] - cuts[n])
                     for src, dst in ((wg_hbm, wg_v), (wu_hbm, wu_v), (wd_hbm, wd_v))])
            for n in range(2)]
    for cp in [cp_x[0]] + cp_w0:
        sch.at(-9, cp.start)
    sch.at(-8.5, cp_x[0].wait)
    for kb in range(NJ):
        sch.at(-8 + kb, cp_w0[kb].wait)
        sch.spread(-8 + kb, -7 + kb, [w_transpose(0, kb, cb) for cb in range(NJ)])
    for pos, starts, waits in (
            (T_START[0], (cp_x[1], cp_vec), ()),
            (T_START[1], (cp_w[1],), ()),
            (NJ * dt - 0.1, (), (cp_x[1], cp_vec)),
            (T_START[2], (cp_w[2],), ()),
            (T_W[1], (cp_x[2],), (cp_w[1],)),
            (T_W[2], (cp_wo,), (cp_w[2],)),
            (T_ROUTE[0], (cp_f[0],), (cp_x[2], cp_wo)),
            (T_START[3], (cp_f[1],), ()),
            (T_FFN[0], (), (cp_f[0],)),
            (T_FFN[0] + (T_FFN[1] - T_FFN[0]) * FFN_CUT / F - 2, (), (cp_f[1],))):
        for cp in starts:
            sch.at(pos, cp.start)
        for cp in waits:
            sch.at(pos, cp.wait)

    for c in range(3):
        first = slot["qkv", 0, c, 0, 0]
        if c > 0:
            sch.spread(T_W[c], first - 0.8,
                       [w_transpose(c, kb, cb) for cb in range(NJ) for kb in range(NJ)])
        for j in range(NJ):
            sch.at(first + (j - 1.4) * dt, w_gather(c, j))
    first = slot["out", 0, 0, 0]
    sch.spread(T_ROUTE[0], min(first - 0.5, T_ROUTE[0] + 10), [fn for nb in range(NJ) for fn in (wo_widen(nb), wo_gather(nb))])

    def vectors():
        for n, ref in enumerate((gw_v, wr_v)):
            vec_s[n] = jnp.broadcast_to(ref[...].astype(f32).reshape(1, D), (RB, D))

    sch.at(5, vectors)
    early = HEAD * TM // RB
    sch.pipeline(*T_EARLY, [route(n) for n in range(early)], 3, 2)
    sch.pipeline(*T_ROUTE, [route(n) for n in range(early, S // RB)], 3, 2)
    picker = select_top2()
    sch.spread(*T_SELECT, [lambda: next(picker, None)] * 5)

    t0 = 0
    for i in range(NT):
        t0 = max(t0, slot["qkv", max(i, ATT0), 2, NJ - 1, TM - MS] + dt)
        t1 = t0 + min((slot["out", n, 0, 0] - 0.5 - t0) / (n - i + 1) for n in range(i, NT))
        sch.pipeline(t0, t1, [attend(i, r0) for r0 in range(0, TM, RA)], ATT_DEPTH, ATT_LAG)
        t0 = t1

    t0, t1 = T_FFN
    sch.pipeline(t0, t1, [ffn(f0) for f0 in range(0, F, RB)], FFN_DEPTH, FFN_LAG)
    sch.at(t1 + 0.1, ffn_finish)

    cp_out = [store(0, LATE, range(NJ))]
    for t in range(2):
        sch.at(t1 + 1 + t, lambda t=t: patch_output(t))
        sch.at(slot["qkv", NT - 1, 2, NJ - 1, TM - MS] + 0.1, lambda t=t: patch_residual(t))
    sch.at(t1 + 3.5, cp_out[0].start)
    for op, n in slot.items():
        if op[0] == "out" and op[1] * TM >= LATE and op[3] == TM - MS:
            cp_out.append(store(op[1] * TM, TM, [op[2]]))
            sch.at(n + 0.75, cp_out[-1].start)
    for cp in cp_out:
        sch.at(len(mxu) * dt + 2, cp.wait)
    sch.emit()


@jax.jit
def pallas_gated_mix__sliding_local_dilated__moe_arch_mod__prompt_kernel(
    A_x: jax.Array,
    A_wqkv: jax.Array,
    A_wo: jax.Array,
    B_x: jax.Array,
    B_w_r: jax.Array,
    B_w_gate: jax.Array,
    B_w_up: jax.Array,
    B_w_down: jax.Array,
    gate_w: jax.Array,
):
    n_sems = 2 + 2 + 1 + NJ * (1 + 3 + 6 + 1 + (S - LATE) // TM)
    scratch = [
        pltpu.VMEM((NJ, S, L), bf16),
        pltpu.VMEM((NJ, S, L), bf16),
        pltpu.VMEM((D, 3 * D), bf16),
        pltpu.VMEM((D, D), bf16),
        pltpu.VMEM((NJ, F, L), bf16),
        pltpu.VMEM((NJ, F, L), bf16),
        pltpu.VMEM((NJ, F, L), bf16),
        pltpu.VMEM((D,), bf16),
        pltpu.VMEM((D,), bf16),
        pltpu.VMEM((NJ, 3 * D, L), f32),
        pltpu.VMEM((NJ, 3 * D, L), bf16),
        pltpu.VMEM((NJ, D, L), f32),
        pltpu.VMEM((NJ, D, L), bf16),
        pltpu.VMEM((S, L), f32),
        pltpu.VMEM((6, RB, D), f32),
        pltpu.VMEM((2, RB, D), f32),
        pltpu.SMEM((2,), i32),
        pltpu.SemaphoreType.DMA((n_sems,)),
    ]
    scratch += [pltpu.VMEM((NJ, TM, L), f32)] * NT
    scratch += [pltpu.VMEM((NJ, HALO + TM, L), f32)] * (2 * NT)
    scratch += [pltpu.VMEM((NJ, TM, L), bf16)] * NT
    out = pl.pallas_call(
        _kernel,
        out_shape=jax.ShapeDtypeStruct((S, D), bf16),
        in_specs=[pl.BlockSpec(memory_space=pl.ANY)] * 8,
        out_specs=pl.BlockSpec(memory_space=pl.ANY),
        scratch_shapes=scratch,
        compiler_params=pltpu.CompilerParams(vmem_limit_bytes=100 * 2**20, flags=FLAGS),
        name="gated_mix",
    )(A_x.reshape(S, D), A_wqkv, A_wo, B_w_r,
      B_w_gate.T, B_w_up.T, B_w_down, gate_w)
    return out.reshape(1, S, D)
```

```python
import numpy as np

import jax
import jax.numpy as jnp
from jax import lax
import jax.experimental.pallas as pl
import jax.experimental.pallas.tpu as pltpu

S, D, F = 2048, 640, 1728
H, DH = 32, 20
WIN, DIL = 8, 2
HALO = 16
L = 128
NJ = D // L
TM = 256
NT = S // TM
RB = 16
SCALE = float(DH) ** -0.5
LOG2E = float(np.log2(np.e))

HEAD = 2
OUT_LAG = 2
LATE = (NT - OUT_LAG - 1) * TM
T_START = (-5.5, -4.5, 2.5, 36.0)
T_W = (None, 6.5, 15.0)
T_EARLY = (10.0, 15.0)
T_ROUTE = (27.0, 37.0)
T_SELECT = (38.0, 45.0)
T_FFN = (46.0, 138.0)
FFN_CUT = 640
FLAGS = None
NN = False
M_OUTER = True
MIX = False
ATT0 = 1
MS = 128
RA = 8
ATT_LAG = 1
FFN_LAG = 1
SKEW = 1.0
REV = False
ATT_DEPTH = 4
FFN_DEPTH = 4

f32, bf16, u32, i32 = jnp.float32, jnp.bfloat16, jnp.uint32, jnp.int32


class _Schedule:
    def __init__(self):
        self.items = []

    def at(self, pos, fn):
        self.items.append((pos, len(self.items), fn))

    def spread(self, t0, t1, fns):
        for n, fn in enumerate(fns):
            self.at(t0 + (n + 0.5) * (t1 - t0) / len(fns), fn)

    def pipeline(self, t0, t1, gens, depth, lag=1, warp=lambda t: t):
        step = (t1 - t0) / (len(gens) + (depth - 1) * lag)
        for n, gen in enumerate(gens):
            for s in range(depth):
                phase = (depth - s if REV else s) * SKEW / depth
                self.at(warp(t0 + (n + s * lag + 0.5 * (1 - SKEW) + phase) * step),
                        lambda gen=gen: next(gen, None))

    def emit(self):
        for _, _, fn in sorted(self.items, key=lambda it: it[:2]):
            fn()


class _Copies:
    def __init__(self, copies):
        self.copies = copies

    def start(self):
        for cp in self.copies:
            cp.start()

    def wait(self):
        for cp in self.copies:
            cp.wait()


def _recip(d):
    r = pl.reciprocal(d, approx=True)
    return r * (2.0 - d * r)


def _exp_neg(z):
    return jnp.minimum(jnp.exp2(z * -LOG2E), 1e38)


def _sigmoid(z):
    return _recip(1.0 + _exp_neg(z))


def _lanes(j):
    return slice(j * L, (j + 1) * L)


def _get(ref, j, r0, n):
    return pltpu.bitcast(ref[j, pl.ds(r0 // 2, n // 2), :], bf16)


def _full_rows(ref, r0, n):
    return jnp.concatenate([_get(ref, j, r0, n) for j in range(NJ)], axis=1)


def _put(ref, j, r0, val):
    ref[j, pl.ds(r0, val.shape[0]), :] = val.astype(bf16)


def _row_dots(rows_ref, r0, vec_ref, vs):
    acc = [None] * len(vs)
    for j in range(NJ):
        rows = _get(rows_ref, j, r0, RB).astype(f32)
        for n, v in enumerate(vs):
            vec = vec_ref[v, 0:8, _lanes(j)]
            t = rows * jnp.concatenate([vec, vec], axis=0)
            acc[n] = t if acc[n] is None else acc[n] + t
    return [jnp.broadcast_to(jnp.sum(a, axis=1, keepdims=True), (RB, L)) for a in acc]


def _kernel(x_hbm, wqkv_hbm, wo_hbm, wr_hbm, wg_hbm, wu_hbm, wd_hbm, gw_hbm,
            out_hbm,
            x_v, out_v, w_raw, wo_raw, wg_v, wu_v, wd_v, gw_v, wr_v,
            wt_s, wp_v, wo_s, wop_v, gate_s, vec_s, y_s, sel_s, sems, *tiles):
    q_t, k_t, v_t, o_t = (tiles[i * NT:(i + 1) * NT] for i in range(4))
    x_w, out_w, wg_w, wu_w, wd_w, wp_w, wop_w = (
        r.bitcast(u32) for r in (x_v, out_v, wg_v, wu_v, wd_v, wp_v, wop_v))
    o_w = [r.bitcast(u32) for r in o_t]

    sem_ids = iter(range(sems.shape[0]))

    def copy(src, dst):
        return pltpu.make_async_copy(src, dst, sems.at[next(sem_ids)])

    def load(src, dst, r0, n):
        return _Copies([copy(src.at[pl.ds(r0, n), pl.ds(j * L, L)], dst.at[j, pl.ds(r0, n), :])
                        for j in range(NJ)])

    def store(r0, n, groups):
        return _Copies([copy(out_v.at[j, pl.ds(r0, n), :], out_hbm.at[pl.ds(r0, n), pl.ds(j * L, L)])
                        for j in groups])

    def w_transpose(c, kb, cb):
        def fn():
            blk = w_raw[pl.ds(kb * L, L), pl.ds(c * D + cb * L, L)].astype(f32)
            wt_s[kb, pl.ds(c * D + cb * L, L), :] = blk.T
        return fn

    def w_gather(c, j):
        def fn():
            for kb in range(NJ):
                parts = [wt_s[kb, pl.ds(c * D + 4 * j + dd, H, stride=DH), :] for dd in range(4)]
                blk = jnp.concatenate(parts, axis=0)
                _put(wp_v, kb, c * D + j * L, blk.T if NN else blk)
        return fn

    def wo_widen(nb):
        def fn():
            wo_s[nb] = wo_raw[:, _lanes(nb)].astype(f32)
        return fn

    def wo_gather(nb):
        def fn():
            for j in range(NJ):
                parts = [wo_s[nb, pl.ds(4 * j + dd, H, stride=DH), :] for dd in range(4)]
                _put(wop_v, nb, j * L, jnp.concatenate(parts, axis=0))
        return fn

    def qkv(i, c, j, m0):
        def fn():
            w = jnp.concatenate([_get(wp_w, kb, c * D + j * L, L) for kb in range(NJ)], axis=0 if NN else 1)
            y = lax.dot_general(_full_rows(x_w, i * TM + m0, MS), w,
                                (((1,), (0 if NN else 1,)), ((), ())), preferred_element_type=f32)
            if c == 0:
                q_t[i][j, pl.ds(m0, MS), :] = y
                return
            dst = k_t if c == 1 else v_t
            dst[i][j, pl.ds(HALO + m0, MS), :] = y
            if i + 1 < NT and m0 + MS == TM:
                dst[i + 1][j, pl.ds(0, HALO), :] = y[MS - HALO:]
            if i == 0 and m0 == 0:
                dst[0][j, pl.ds(0, HALO), :] = jnp.broadcast_to(y[0:1], (HALO, L))
        return fn

    half = {}

    def attend(i, r0):
        q = [q_t[i][j, pl.ds(r0, RA), :] for j in range(NJ)]
        z = []
        for w in range(WIN):
            acc = None
            for j in range(NJ):
                t = q[j] * k_t[i][j, pl.ds(HALO + r0 - DIL * w, RA), :]
                acc = t if acc is None else acc + t
            z.append((acc, pltpu.roll(acc, 2 * H, 1)))
        yield
        z = [a + b for a, b in z]
        z = [(a, pltpu.roll(a, H, 1)) for a in z]
        yield
        z = [a + b for a, b in z]
        if i == 0 and r0 < DIL * (WIN - 1):
            pos = r0 + lax.broadcasted_iota(i32, (RA, L), 0)
            z = [jnp.where(pos >= DIL * w, z[w] * SCALE, -1e9) for w in range(WIN)]
            c = LOG2E
        else:
            c = SCALE * LOG2E
        m = z[0]
        for w in range(1, WIN):
            m = jnp.maximum(m, z[w])
        e = [jnp.exp2((z[w] - m) * c) for w in range(WIN)]
        if ATT_DEPTH == 4:
            yield
        den = e[0]
        for w in range(1, WIN):
            den = den + e[w]
        inv = _recip(den)
        for j in range(NJ):
            acc = None
            for w in range(WIN):
                t = e[w] * v_t[i][j, pl.ds(HALO + r0 - DIL * w, RA), :]
                acc = t if acc is None else acc + t
            o = acc * inv
            if RA == RB:
                _put(o_t[i], j, r0, o)
            elif r0 % RB == 0:
                half[i, j] = o
            else:
                _put(o_t[i], j, r0 - RA, jnp.concatenate([half.pop((i, j)), o], axis=0))

    def project(i, nb, m0):
        def fn():
            r0 = i * TM + m0
            a = jnp.dot(_full_rows(o_w[i], m0, MS), _get(wop_w, nb, 0, D), preferred_element_type=f32)
            g = gate_s[pl.ds(r0, MS), :]
            b = _get(x_w, nb, r0, MS).astype(f32)
            _put(out_v, nb, r0, b + g * (a - b))
        return fn

    lane = lax.broadcasted_iota(i32, (RB, L), 1)
    score = [jnp.zeros((RB, L), f32)]

    def route(n):
        g, r = _row_dots(x_w, n * RB, vec_s, (0, 1))
        yield
        score[0] = jnp.where(lane == n, r, score[0])
        e = _exp_neg(g)
        yield
        gate_s[pl.ds(n * RB, RB), :] = _recip(1.0 + e)

    def row_group(ref, base, idx):
        word = pl.multiple_of(base // 2, RB // 2)
        rows = [pltpu.bitcast(ref[j, pl.ds(word, RB // 2), :], bf16) for j in range(NJ)]
        hit = lax.broadcasted_iota(i32, (RB, D), 0) == idx - base
        return jnp.concatenate(rows, axis=1).astype(f32), hit, word

    def select_top2():
        r = score[0].astype(bf16).astype(f32)
        r = jnp.where(r == 0.0, 0.0, r)
        bits = pltpu.bitcast(r, i32) >> 16
        key = jnp.where(bits < 0, bits ^ 0x7FFF, bits)
        key = jnp.where(r != r, -(1 << 15) - 1, key).astype(f32)
        row = lax.broadcasted_iota(i32, (RB, L), 0).astype(f32)
        back = (L - 1 - lane[0:1]).astype(f32)
        in_lane = []
        for _ in range(2):
            best = jnp.max(key, axis=0, keepdims=True)
            first = jnp.min(jnp.where(key == best, row, float(RB)), axis=0, keepdims=True)
            here = row == first
            in_lane.append((best * L + back, first, jnp.sum(jnp.where(here, r, 0.0), axis=0, keepdims=True)))
            key = jnp.where(here, -float(1 << 16), key)
        top = jnp.max(in_lane[0][0], axis=1, keepdims=True)
        yield
        won = in_lane[0][0] == top
        rest = [jnp.where(won, b, a) for a, b in zip(*in_lane)]
        top = jnp.max(rest[0], axis=1, keepdims=True)
        yield
        picks = []
        for cand, hit in ((in_lane[0], won), (rest, rest[0] == top)):
            pos = (L - 1 - back) * RB + cand[1]
            picks.append([jnp.sum(jnp.where(hit, v, 0.0), axis=1, keepdims=True) for v in (pos, cand[2])])
        yield
        ids = [jnp.clip(pos.astype(i32)[0, 0], 0, S - 1) for pos, _ in picks]
        yield
        for t, idx in enumerate(ids):
            sel_s[t] = idx
            vec_s[4 + t, :, 0:L] = _sigmoid(jnp.broadcast_to(picks[t][1], (RB, L)))
            grp, hit, _ = row_group(x_w, (idx // RB) * RB, idx)
            vec_s[2 + t] = jnp.broadcast_to(
                jnp.sum(jnp.where(hit, grp, 0.0), axis=0, keepdims=True), (RB, D))

    y_acc = {}

    def ffn(f0):
        gp = _row_dots(wg_w, f0, vec_s, (2, 3))
        up = _row_dots(wu_w, f0, vec_s, (2, 3))
        yield
        e = [_exp_neg(a) for a in gp]
        if FFN_DEPTH >= 3:
            yield
        sig = [_recip(1.0 + a) for a in e]
        if FFN_DEPTH >= 4:
            yield
        h = [gp[t] * sig[t] * up[t] for t in range(2)]
        for j in range(NJ):
            wd = _get(wd_w, j, f0, RB).astype(f32)
            for t in range(2):
                p = h[t] * wd
                p = p[0:8] + p[8:16]
                y_acc[t, j] = y_acc[t, j] + p if (t, j) in y_acc else p

    def ffn_finish():
        for t in range(2):
            for j in range(NJ):
                y = jnp.sum(y_acc[t, j], axis=0, keepdims=True)
                y_s[t, :, _lanes(j)] = jnp.broadcast_to(y, (RB, L)) * vec_s[4 + t, :, 0:L]

    def add_to_row(ref, base, idx, term):
        old, hit, word = row_group(ref, base, idx)
        new = jnp.where(hit, old + term, old).astype(bf16)
        for j in range(NJ):
            ref[j, pl.ds(word, RB // 2), :] = pltpu.bitcast(new[:, _lanes(j)], u32)

    def patch_output(t):
        idx = sel_s[t]
        g = _sigmoid(jnp.sum(vec_s[2 + t] * vec_s[0], axis=1, keepdims=True))
        add_to_row(out_w, jnp.minimum((idx // RB) * RB, LATE - RB), idx, (1.0 - g) * y_s[t])

    def patch_residual(t):
        idx = sel_s[t]
        add_to_row(x_w, (idx // RB) * RB, idx, y_s[t])

    sch = _Schedule()
    halves = range(0, TM, MS)
    mxu = [("qkv", i, c, j, m0) for c in range(3) for i in range(HEAD) for m0 in halves for j in range(NJ)]
    for i in range(HEAD, NT + OUT_LAG):
        if M_OUTER:
            fwd = [[("qkv", i, c, j, m0)] for m0 in halves for c in range(3) for j in range(NJ)]
            out = [[("out", i - OUT_LAG, nb, m0)] for m0 in halves for nb in range(NJ)]
        else:
            fwd = [[("qkv", i, c, j, m0) for m0 in halves] for c in range(3) for j in range(NJ)]
            out = [[("out", i - OUT_LAG, nb, m0) for m0 in halves] for nb in range(NJ)]
        if i >= NT:
            fwd = []
        if MIX and fwd:
            fwd, out = [g for n in range(len(out)) for g in fwd[3 * n:3 * n + 3] + [out[n]]], []
        mxu += [op for g in fwd + out for op in g]
    dt = MS / 256
    slot = {op: n * dt for n, op in enumerate(mxu)}
    for op, t in slot.items():
        sch.at(t, (qkv if op[0] == "qkv" else project)(*op[1:]))

    cp_w0 = [copy(wqkv_hbm.at[pl.ds(kb * L, L), pl.ds(0, D)], w_raw.at[pl.ds(kb * L, L), pl.ds(0, D)])
             for kb in range(NJ)]
    cp_w = {c: copy(wqkv_hbm.at[:, pl.ds(c * D, D)], w_raw.at[:, pl.ds(c * D, D)]) for c in (1, 2)}
    cp_x = [load(x_hbm, x_v, 0, MS), load(x_hbm, x_v, MS, HEAD * TM - MS),
            load(x_hbm, x_v, HEAD * TM, S - HEAD * TM)]
    cp_vec = _Copies([copy(gw_hbm, gw_v), copy(wr_hbm, wr_v)])
    cp_wo = copy(wo_hbm, wo_raw)
    cuts = (0, FFN_CUT, F)
    cp_f = [_Copies([load(src, dst, cuts[n], cuts[n + 1] - cuts[n])
                     for src, dst in ((wg_hbm, wg_v), (wu_hbm, wu_v), (wd_hbm, wd_v))])
            for n in range(2)]
    for cp in [cp_x[0]] + cp_w0:
        sch.at(-9, cp.start)
    sch.at(-8.5, cp_x[0].wait)
    for kb in range(NJ):
        sch.at(-8 + kb, cp_w0[kb].wait)
        sch.spread(-8 + kb, -7 + kb, [w_transpose(0, kb, cb) for cb in range(NJ)])
    for pos, starts, waits in (
            (T_START[0], (cp_x[1], cp_vec), ()),
            (T_START[1], (cp_w[1],), ()),
            (NJ * dt - 0.1, (), (cp_x[1], cp_vec)),
            (T_START[2], (cp_w[2],), ()),
            (T_W[1], (cp_x[2],), (cp_w[1],)),
            (T_W[2], (cp_wo,), (cp_w[2],)),
            (T_ROUTE[0], (cp_f[0],), (cp_x[2], cp_wo)),
            (T_START[3], (cp_f[1],), ()),
            (T_FFN[0], (), (cp_f[0],)),
            (T_FFN[0] + (T_FFN[1] - T_FFN[0]) * FFN_CUT / F - 2, (), (cp_f[1],))):
        for cp in starts:
            sch.at(pos, cp.start)
        for cp in waits:
            sch.at(pos, cp.wait)

    for c in range(3):
        first = slot["qkv", 0, c, 0, 0]
        if c > 0:
            sch.spread(T_W[c], first - 0.8,
                       [w_transpose(c, kb, cb) for cb in range(NJ) for kb in range(NJ)])
        for j in range(NJ):
            sch.at(first + (j - 1.4) * dt, w_gather(c, j))
    first = slot["out", 0, 0, 0]
    sch.spread(T_ROUTE[0], min(first - 0.5, T_ROUTE[0] + 10), [fn for nb in range(NJ) for fn in (wo_widen(nb), wo_gather(nb))])

    def vectors():
        for n, ref in enumerate((gw_v, wr_v)):
            vec_s[n] = jnp.broadcast_to(ref[...].astype(f32).reshape(1, D), (RB, D))

    sch.at(5, vectors)
    early = HEAD * TM // RB
    sch.pipeline(*T_EARLY, [route(n) for n in range(early)], 3, 2)
    sch.pipeline(*T_ROUTE, [route(n) for n in range(early, S // RB)], 3, 2)
    picker = select_top2()
    sch.spread(*T_SELECT, [lambda: next(picker, None)] * 5)

    t0 = 0
    for i in range(NT):
        t0 = max(t0, slot["qkv", max(i, ATT0), 2, NJ - 1, TM - MS] + dt)
        t1 = t0 + min((slot["out", n, 0, 0] - 0.5 - t0) / (n - i + 1) for n in range(i, NT))
        sch.pipeline(t0, t1, [attend(i, r0) for r0 in range(0, TM, RA)], ATT_DEPTH, ATT_LAG)
        t0 = t1

    t0, t1 = T_FFN
    sch.pipeline(t0, t1, [ffn(f0) for f0 in range(0, F, RB)], FFN_DEPTH, FFN_LAG)
    sch.at(t1 + 0.1, ffn_finish)

    cp_out = [store(0, LATE, range(NJ))]
    for t in range(2):
        sch.at(t1 + 1 + t, lambda t=t: patch_output(t))
        sch.at(slot["qkv", NT - 1, 2, NJ - 1, TM - MS] + 0.1, lambda t=t: patch_residual(t))
    sch.at(t1 + 3.5, cp_out[0].start)
    for op, n in slot.items():
        if op[0] == "out" and op[1] * TM >= LATE and op[3] == TM - MS:
            cp_out.append(store(op[1] * TM, TM, [op[2]]))
            sch.at(n + 0.75, cp_out[-1].start)
    for cp in cp_out:
        sch.at(len(mxu) * dt + 2, cp.wait)
    sch.emit()


@jax.jit
def pallas_gated_mix__sliding_local_dilated__moe_arch_mod__prompt_kernel(
    A_x: jax.Array,
    A_wqkv: jax.Array,
    A_wo: jax.Array,
    B_x: jax.Array,
    B_w_r: jax.Array,
    B_w_gate: jax.Array,
    B_w_up: jax.Array,
    B_w_down: jax.Array,
    gate_w: jax.Array,
):
    n_sems = 2 + 2 + 1 + NJ * (1 + 3 + 6 + 1 + (S - LATE) // TM)
    scratch = [
        pltpu.VMEM((NJ, S, L), bf16),
        pltpu.VMEM((NJ, S, L), bf16),
        pltpu.VMEM((D, 3 * D), bf16),
        pltpu.VMEM((D, D), bf16),
        pltpu.VMEM((NJ, F, L), bf16),
        pltpu.VMEM((NJ, F, L), bf16),
        pltpu.VMEM((NJ, F, L), bf16),
        pltpu.VMEM((D,), bf16),
        pltpu.VMEM((D,), bf16),
        pltpu.VMEM((NJ, 3 * D, L), f32),
        pltpu.VMEM((NJ, 3 * D, L), bf16),
        pltpu.VMEM((NJ, D, L), f32),
        pltpu.VMEM((NJ, D, L), bf16),
        pltpu.VMEM((S, L), f32),
        pltpu.VMEM((6, RB, D), f32),
        pltpu.VMEM((2, RB, D), f32),
        pltpu.SMEM((2,), i32),
        pltpu.SemaphoreType.DMA((n_sems,)),
    ]
    scratch += [pltpu.VMEM((NJ, TM, L), f32)] * NT
    scratch += [pltpu.VMEM((NJ, HALO + TM, L), f32)] * (2 * NT)
    scratch += [pltpu.VMEM((NJ, TM, L), bf16)] * NT
    out = pl.pallas_call(
        _kernel,
        out_shape=jax.ShapeDtypeStruct((S, D), bf16),
        in_specs=[pl.BlockSpec(memory_space=pl.ANY)] * 8,
        out_specs=pl.BlockSpec(memory_space=pl.ANY),
        scratch_shapes=scratch,
        compiler_params=pltpu.CompilerParams(vmem_limit_bytes=100 * 2**20, flags=FLAGS),
        name="gated_mix",
    )(A_x.reshape(S, D), A_wqkv, A_wo, B_w_r,
      B_w_gate.T, B_w_up.T, B_w_down, gate_w)
    return out.reshape(1, S, D)
```

```python
import numpy as np

import jax
import jax.numpy as jnp
from jax import lax
import jax.experimental.pallas as pl
import jax.experimental.pallas.tpu as pltpu

S, D, F = 2048, 640, 1728
H, DH = 32, 20
WIN, DIL = 8, 2
HALO = 16
L = 128
NJ = D // L
TM = 256
NT = S // TM
RB = 16
SCALE = float(DH) ** -0.5
LOG2E = float(np.log2(np.e))

HEAD = 2
OUT_LAG = 2
LATE = (NT - OUT_LAG - 1) * TM
T_START = (-5.5, -4.5, 2.5, 36.0)
T_W = (None, 6.0, 14.0)
T_EARLY = (10.0, 15.0)
T_ROUTE = (27.0, 37.0)
T_SELECT = (38.0, 45.0)
T_FFN = (46.0, 138.0)
FFN_CUT = 640
FLAGS = None
NN = True
M_OUTER = True
MIX = False
ATT0 = 1
MS = 128
RA = 8
ATT_LAG = 1
FFN_LAG = 1
SKEW = 1.0
REV = False
ATT_DEPTH = 4
FFN_DEPTH = 4

f32, bf16, u32, i32 = jnp.float32, jnp.bfloat16, jnp.uint32, jnp.int32


class _Schedule:
    def __init__(self):
        self.items = []

    def at(self, pos, fn):
        self.items.append((pos, len(self.items), fn))

    def spread(self, t0, t1, fns):
        for n, fn in enumerate(fns):
            self.at(t0 + (n + 0.5) * (t1 - t0) / len(fns), fn)

    def pipeline(self, t0, t1, gens, depth, lag=1, warp=lambda t: t):
        step = (t1 - t0) / (len(gens) + (depth - 1) * lag)
        for n, gen in enumerate(gens):
            for s in range(depth):
                phase = (depth - s if REV else s) * SKEW / depth
                self.at(warp(t0 + (n + s * lag + 0.5 * (1 - SKEW) + phase) * step),
                        lambda gen=gen: next(gen, None))

    def emit(self):
        for _, _, fn in sorted(self.items, key=lambda it: it[:2]):
            fn()


class _Copies:
    def __init__(self, copies, totals):
        self.copies, self.totals = copies, totals

    def start(self):
        for cp in self.copies:
            cp.start()

    def wait(self):
        for cp in self.totals:
            cp.wait()


def _recip(d):
    r = pl.reciprocal(d, approx=True)
    return r * (2.0 - d * r)


def _exp_neg(z):
    return jnp.minimum(jnp.exp2(z * -LOG2E), 1e38)


def _sigmoid(z):
    return _recip(1.0 + _exp_neg(z))


def _lanes(j):
    return slice(j * L, (j + 1) * L)


def _get(ref, j, r0, n):
    return pltpu.bitcast(ref[j, pl.ds(r0 // 2, n // 2), :], bf16)


def _full_rows(ref, r0, n):
    return jnp.concatenate([_get(ref, j, r0, n) for j in range(NJ)], axis=1)


def _put(ref, j, r0, val):
    ref[j, pl.ds(r0, val.shape[0]), :] = val.astype(bf16)


def _row_dots(rows_ref, r0, vec_ref, vs):
    acc = [None] * len(vs)
    for j in range(NJ):
        rows = _get(rows_ref, j, r0, RB).astype(f32)
        for n, v in enumerate(vs):
            vec = vec_ref[v, 0:8, _lanes(j)]
            t = rows * jnp.concatenate([vec, vec], axis=0)
            acc[n] = t if acc[n] is None else acc[n] + t
    return [jnp.broadcast_to(jnp.sum(a, axis=1, keepdims=True), (RB, L)) for a in acc]


def _kernel(x_hbm, wqkv_hbm, wo_hbm, wr_hbm, wg_hbm, wu_hbm, wd_hbm, gw_hbm,
            out_hbm,
            x_v, out_v, w_raw, wo_raw, wg_v, wu_v, wd_v, gw_v, wr_v,
            wt_s, wp_v, wo_s, wop_v, gate_s, vec_s, y_s, sel_s, sems, *tiles):
    q_t, k_t, v_t, o_t = (tiles[i * NT:(i + 1) * NT] for i in range(4))
    x_w, out_w, wg_w, wu_w, wd_w, wp_w, wop_w = (
        r.bitcast(u32) for r in (x_v, out_v, wg_v, wu_v, wd_v, wp_v, wop_v))
    o_w = [r.bitcast(u32) for r in o_t]

    sem_ids = iter(range(sems.shape[0]))

    def copy(src, dst):
        return pltpu.make_async_copy(src, dst, sems.at[next(sem_ids)])

    def load(src, dst, r0, n):
        sem, region = sems.at[next(sem_ids)], dst.at[:, pl.ds(r0, n), :]
        return _Copies(
            [pltpu.make_async_copy(src.at[pl.ds(r0, n), pl.ds(j * L, L)], dst.at[j, pl.ds(r0, n), :], sem)
             for j in range(NJ)],
            [pltpu.make_async_copy(region, region, sem)])

    out_sem = sems.at[next(sem_ids)]

    def store(r0, n, j):
        return pltpu.make_async_copy(
            out_v.at[j, pl.ds(r0, n), :], out_hbm.at[pl.ds(r0, n), pl.ds(j * L, L)], out_sem).start

    def w_transpose(c, kb, cb):
        def fn():
            blk = w_raw[pl.ds(kb * L, L), pl.ds(c * D + cb * L, L)].astype(f32)
            wt_s[kb, pl.ds(c * D + cb * L, L), :] = blk.T
        return fn

    def w_gather(c, j):
        def fn():
            for kb in range(NJ):
                parts = [wt_s[kb, pl.ds(c * D + 4 * j + dd, H, stride=DH), :] for dd in range(4)]
                blk = jnp.concatenate(parts, axis=0)
                _put(wp_v, kb, c * D + j * L, blk.T if NN else blk)
        return fn

    def wo_widen(nb):
        def fn():
            wo_s[nb] = wo_raw[:, _lanes(nb)].astype(f32)
        return fn

    def wo_gather(nb):
        def fn():
            for j in range(NJ):
                parts = [wo_s[nb, pl.ds(4 * j + dd, H, stride=DH), :] for dd in range(4)]
                _put(wop_v, nb, j * L, jnp.concatenate(parts, axis=0))
        return fn

    def qkv(i, c, j, m0):
        def fn():
            w = jnp.concatenate([_get(wp_w, kb, c * D + j * L, L) for kb in range(NJ)], axis=0 if NN else 1)
            y = lax.dot_general(_full_rows(x_w, i * TM + m0, MS), w,
                                (((1,), (0 if NN else 1,)), ((), ())), preferred_element_type=f32)
            if c == 0:
                q_t[i][j, pl.ds(m0, MS), :] = y
                return
            dst = k_t if c == 1 else v_t
            dst[i][j, pl.ds(HALO + m0, MS), :] = y
            if i + 1 < NT and m0 + MS == TM:
                dst[i + 1][j, pl.ds(0, HALO), :] = y[MS - HALO:]
            if i == 0 and m0 == 0:
                dst[0][j, pl.ds(0, HALO), :] = jnp.broadcast_to(y[0:1], (HALO, L))
        return fn

    half = {}

    def attend(i, r0):
        q = [q_t[i][j, pl.ds(r0, RA), :] for j in range(NJ)]
        z = []
        for w in range(WIN):
            acc = None
            for j in range(NJ):
                t = q[j] * k_t[i][j, pl.ds(HALO + r0 - DIL * w, RA), :]
                acc = t if acc is None else acc + t
            z.append((acc, pltpu.roll(acc, 2 * H, 1)))
        yield
        z = [a + b for a, b in z]
        z = [(a, pltpu.roll(a, H, 1)) for a in z]
        yield
        z = [a + b for a, b in z]
        if i == 0 and r0 < DIL * (WIN - 1):
            pos = r0 + lax.broadcasted_iota(i32, (RA, L), 0)
            z = [jnp.where(pos >= DIL * w, z[w] * SCALE, -1e9) for w in range(WIN)]
            c = LOG2E
        else:
            c = SCALE * LOG2E
        m = z[0]
        for w in range(1, WIN):
            m = jnp.maximum(m, z[w])
        e = [jnp.exp2((z[w] - m) * c) for w in range(WIN)]
        if ATT_DEPTH == 4:
            yield
        den = e[0]
        for w in range(1, WIN):
            den = den + e[w]
        inv = _recip(den)
        for j in range(NJ):
            acc = None
            for w in range(WIN):
                t = e[w] * v_t[i][j, pl.ds(HALO + r0 - DIL * w, RA), :]
                acc = t if acc is None else acc + t
            o = acc * inv
            if RA == RB:
                _put(o_t[i], j, r0, o)
            elif r0 % RB == 0:
                half[i, j] = o
            else:
                _put(o_t[i], j, r0 - RA, jnp.concatenate([half.pop((i, j)), o], axis=0))

    def project(i, nb, m0):
        def fn():
            r0 = i * TM + m0
            a = jnp.dot(_full_rows(o_w[i], m0, MS), _get(wop_w, nb, 0, D), preferred_element_type=f32)
            g = gate_s[pl.ds(r0, MS), :]
            b = _get(x_w, nb, r0, MS).astype(f32)
            _put(out_v, nb, r0, b + g * (a - b))
        return fn

    lane = lax.broadcasted_iota(i32, (RB, L), 1)
    score = [jnp.zeros((RB, L), f32)]

    def route(n):
        g, r = _row_dots(x_w, n * RB, vec_s, (0, 1))
        yield
        score[0] = jnp.where(lane == n, r, score[0])
        e = _exp_neg(g)
        yield
        gate_s[pl.ds(n * RB, RB), :] = _recip(1.0 + e)

    def row_group(ref, base, idx):
        word = pl.multiple_of(base // 2, RB // 2)
        rows = [pltpu.bitcast(ref[j, pl.ds(word, RB // 2), :], bf16) for j in range(NJ)]
        hit = lax.broadcasted_iota(i32, (RB, D), 0) == idx - base
        return jnp.concatenate(rows, axis=1).astype(f32), hit, word

    def select_top2():
        r = score[0].astype(bf16).astype(f32)
        r = jnp.where(r == 0.0, 0.0, r)
        bits = pltpu.bitcast(r, i32) >> 16
        key = jnp.where(bits < 0, bits ^ 0x7FFF, bits)
        key = jnp.where(r != r, -(1 << 15) - 1, key).astype(f32)
        row = lax.broadcasted_iota(i32, (RB, L), 0).astype(f32)
        back = (L - 1 - lane[0:1]).astype(f32)
        in_lane = []
        for _ in range(2):
            best = jnp.max(key, axis=0, keepdims=True)
            first = jnp.min(jnp.where(key == best, row, float(RB)), axis=0, keepdims=True)
            here = row == first
            in_lane.append((best * L + back, first, jnp.sum(jnp.where(here, r, 0.0), axis=0, keepdims=True)))
            key = jnp.where(here, -float(1 << 16), key)
        top = jnp.max(in_lane[0][0], axis=1, keepdims=True)
        yield
        won = in_lane[0][0] == top
        rest = [jnp.where(won, b, a) for a, b in zip(*in_lane)]
        top = jnp.max(rest[0], axis=1, keepdims=True)
        yield
        picks = []
        for cand, hit in ((in_lane[0], won), (rest, rest[0] == top)):
            pos = (L - 1 - back) * RB + cand[1]
            picks.append([jnp.sum(jnp.where(hit, v, 0.0), axis=1, keepdims=True) for v in (pos, cand[2])])
        yield
        ids = [jnp.clip(pos.astype(i32)[0, 0], 0, S - 1) for pos, _ in picks]
        yield
        for t, idx in enumerate(ids):
            sel_s[t] = idx
            vec_s[4 + t, :, 0:L] = _sigmoid(jnp.broadcast_to(picks[t][1], (RB, L)))
            grp, hit, _ = row_group(x_w, (idx // RB) * RB, idx)
            vec_s[2 + t] = jnp.broadcast_to(
                jnp.sum(jnp.where(hit, grp, 0.0), axis=0, keepdims=True), (RB, D))

    y_acc = {}

    def ffn(f0):
        gp = _row_dots(wg_w, f0, vec_s, (2, 3))
        up = _row_dots(wu_w, f0, vec_s, (2, 3))
        yield
        e = [_exp_neg(a) for a in gp]
        if FFN_DEPTH >= 3:
            yield
        sig = [_recip(1.0 + a) for a in e]
        if FFN_DEPTH >= 4:
            yield
        h = [gp[t] * sig[t] * up[t] for t in range(2)]
        for j in range(NJ):
            wd = _get(wd_w, j, f0, RB).astype(f32)
            for t in range(2):
                p = h[t] * wd
                p = p[0:8] + p[8:16]
                y_acc[t, j] = y_acc[t, j] + p if (t, j) in y_acc else p

    def ffn_finish():
        for t in range(2):
            for j in range(NJ):
                y = jnp.sum(y_acc[t, j], axis=0, keepdims=True)
                y_s[t, :, _lanes(j)] = jnp.broadcast_to(y, (RB, L)) * vec_s[4 + t, :, 0:L]

    def add_to_row(ref, base, idx, term):
        old, hit, word = row_group(ref, base, idx)
        new = jnp.where(hit, old + term, old).astype(bf16)
        for j in range(NJ):
            ref[j, pl.ds(word, RB // 2), :] = pltpu.bitcast(new[:, _lanes(j)], u32)

    def patch_output(t):
        idx = sel_s[t]
        g = _sigmoid(jnp.sum(vec_s[2 + t] * vec_s[0], axis=1, keepdims=True))
        add_to_row(out_w, jnp.minimum((idx // RB) * RB, LATE - RB), idx, (1.0 - g) * y_s[t])

    def patch_residual(t):
        idx = sel_s[t]
        add_to_row(x_w, (idx // RB) * RB, idx, y_s[t])

    sch = _Schedule()
    halves = range(0, TM, MS)
    mxu = [("qkv", i, c, j, m0) for c in range(3) for i in range(HEAD) for m0 in halves for j in range(NJ)]
    for i in range(HEAD, NT + OUT_LAG):
        if M_OUTER:
            fwd = [[("qkv", i, c, j, m0)] for m0 in halves for c in range(3) for j in range(NJ)]
            out = [[("out", i - OUT_LAG, nb, m0)] for m0 in halves for nb in range(NJ)]
        else:
            fwd = [[("qkv", i, c, j, m0) for m0 in halves] for c in range(3) for j in range(NJ)]
            out = [[("out", i - OUT_LAG, nb, m0) for m0 in halves] for nb in range(NJ)]
        if i >= NT:
            fwd = []
        if MIX and fwd:
            fwd, out = [g for n in range(len(out)) for g in fwd[3 * n:3 * n + 3] + [out[n]]], []
        mxu += [op for g in fwd + out for op in g]
    dt = MS / 256
    slot = {op: n * dt for n, op in enumerate(mxu)}
    for op, t in slot.items():
        sch.at(t, (qkv if op[0] == "qkv" else project)(*op[1:]))

    cp_w0 = [copy(wqkv_hbm.at[pl.ds(kb * L, L), pl.ds(0, D)], w_raw.at[pl.ds(kb * L, L), pl.ds(0, D)])
             for kb in range(NJ)]
    cp_w = {c: copy(wqkv_hbm.at[:, pl.ds(c * D, D)], w_raw.at[:, pl.ds(c * D, D)]) for c in (1, 2)}
    cp_x = [load(x_hbm, x_v, 0, MS), load(x_hbm, x_v, MS, HEAD * TM - MS),
            load(x_hbm, x_v, HEAD * TM, S - HEAD * TM)]
    cp_vec = [copy(gw_hbm, gw_v), copy(wr_hbm, wr_v)]
    cp_wo = copy(wo_hbm, wo_raw)
    cuts = (0, FFN_CUT, F)
    cp_f = [[load(src, dst, cuts[n], cuts[n + 1] - cuts[n])
             for src, dst in ((wg_hbm, wg_v), (wu_hbm, wu_v), (wd_hbm, wd_v))] for n in range(2)]
    for cp in [cp_x[0]] + cp_w0:
        sch.at(-9, cp.start)
    sch.at(-8.5, cp_x[0].wait)
    for kb in range(NJ):
        sch.at(-8 + kb, cp_w0[kb].wait)
        sch.spread(-8 + kb, -7 + kb, [w_transpose(0, kb, cb) for cb in range(NJ)])
    for pos, starts, waits in (
            (T_START[0], (cp_x[1], *cp_vec), ()),
            (T_START[1], (cp_w[1],), ()),
            (NJ * dt - 0.1, (), (cp_x[1], *cp_vec)),
            (T_START[2], (cp_w[2],), ()),
            (T_W[1], (cp_x[2],), (cp_w[1],)),
            (T_W[2], (cp_wo,), (cp_w[2],)),
            (T_ROUTE[0], cp_f[0], (cp_x[2], cp_wo)),
            (T_START[3], cp_f[1], ()),
            (T_FFN[0], (), cp_f[0]),
            (T_FFN[0] + (T_FFN[1] - T_FFN[0]) * FFN_CUT / F - 2, (), cp_f[1])):
        for cp in starts:
            sch.at(pos, cp.start)
        for cp in waits:
            sch.at(pos, cp.wait)

    for c in range(3):
        first = slot["qkv", 0, c, 0, 0]
        if c > 0:
            sch.spread(T_W[c], first - 0.8,
                       [w_transpose(c, kb, cb) for cb in range(NJ) for kb in range(NJ)])
        for j in range(NJ):
            sch.at(first + (j - 1.4) * dt, w_gather(c, j))
    first = slot["out", 0, 0, 0]
    sch.spread(T_ROUTE[0], min(first - 0.5, T_ROUTE[0] + 10), [fn for nb in range(NJ) for fn in (wo_widen(nb), wo_gather(nb))])

    def vectors():
        for n, ref in enumerate((gw_v, wr_v)):
            vec_s[n] = jnp.broadcast_to(ref[...].astype(f32).reshape(1, D), (RB, D))

    sch.at(5, vectors)
    early = HEAD * TM // RB
    sch.pipeline(*T_EARLY, [route(n) for n in range(early)], 3, 2)
    sch.pipeline(*T_ROUTE, [route(n) for n in range(early, S // RB)], 3, 2)
    picker = select_top2()
    sch.spread(*T_SELECT, [lambda: next(picker, None)] * 5)

    t0 = 0
    for i in range(NT):
        t0 = max(t0, slot["qkv", max(i, ATT0), 2, NJ - 1, TM - MS] + dt)
        t1 = t0 + min((slot["out", n, 0, 0] - 0.5 - t0) / (n - i + 1) for n in range(i, NT))
        sch.pipeline(t0, t1, [attend(i, r0) for r0 in range(0, TM, RA)], ATT_DEPTH, ATT_LAG)
        t0 = t1

    t0, t1 = T_FFN
    sch.pipeline(t0, t1, [ffn(f0) for f0 in range(0, F, RB)], FFN_DEPTH, FFN_LAG)
    sch.at(t1 + 0.1, ffn_finish)

    for t in range(2):
        sch.at(t1 + 1 + t, lambda t=t: patch_output(t))
        sch.at(slot["qkv", NT - 1, 2, NJ - 1, TM - MS] + 0.1, lambda t=t: patch_residual(t))
    for j in range(NJ):
        sch.at(t1 + 3.5, store(0, LATE, j))
    for op, t in slot.items():
        if op[0] == "out" and op[1] * TM >= LATE:
            sch.at(t + 0.75, store(op[1] * TM + op[3], MS, op[2]))
    sch.at(len(mxu), pltpu.make_async_copy(out_v, out_v, out_sem).wait)
    sch.emit()


@jax.jit
def pallas_gated_mix__sliding_local_dilated__moe_arch_mod__prompt_kernel(
    A_x: jax.Array,
    A_wqkv: jax.Array,
    A_wo: jax.Array,
    B_x: jax.Array,
    B_w_r: jax.Array,
    B_w_gate: jax.Array,
    B_w_up: jax.Array,
    B_w_down: jax.Array,
    gate_w: jax.Array,
):
    n_sems = 1 + NJ + 2 + 3 + 2 + 1 + 6
    scratch = [
        pltpu.VMEM((NJ, S, L), bf16),
        pltpu.VMEM((NJ, S, L), bf16),
        pltpu.VMEM((D, 3 * D), bf16),
        pltpu.VMEM((D, D), bf16),
        pltpu.VMEM((NJ, F, L), bf16),
        pltpu.VMEM((NJ, F, L), bf16),
        pltpu.VMEM((NJ, F, L), bf16),
        pltpu.VMEM((D,), bf16),
        pltpu.VMEM((D,), bf16),
        pltpu.VMEM((NJ, 3 * D, L), f32),
        pltpu.VMEM((NJ, 3 * D, L), bf16),
        pltpu.VMEM((NJ, D, L), f32),
        pltpu.VMEM((NJ, D, L), bf16),
        pltpu.VMEM((S, L), f32),
        pltpu.VMEM((6, RB, D), f32),
        pltpu.VMEM((2, RB, D), f32),
        pltpu.SMEM((2,), i32),
        pltpu.SemaphoreType.DMA((n_sems,)),
    ]
    scratch += [pltpu.VMEM((NJ, TM, L), f32)] * NT
    scratch += [pltpu.VMEM((NJ, HALO + TM, L), f32)] * (2 * NT)
    scratch += [pltpu.VMEM((NJ, TM, L), bf16)] * NT
    out = pl.pallas_call(
        _kernel,
        out_shape=jax.ShapeDtypeStruct((S, D), bf16),
        in_specs=[pl.BlockSpec(memory_space=pl.ANY)] * 8,
        out_specs=pl.BlockSpec(memory_space=pl.ANY),
        scratch_shapes=scratch,
        compiler_params=pltpu.CompilerParams(vmem_limit_bytes=100 * 2**20, flags=FLAGS),
        name="gated_mix",
    )(A_x.reshape(S, D), A_wqkv, A_wo, B_w_r,
      B_w_gate.T, B_w_up.T, B_w_down, gate_w)
    return out.reshape(1, S, D)
```

```python
import numpy as np

import jax
import jax.numpy as jnp
from jax import lax
import jax.experimental.pallas as pl
import jax.experimental.pallas.tpu as pltpu

S, D, F = 2048, 640, 1728
H, DH = 32, 20
WIN, DIL = 8, 2
HALO = 16
L = 128
NJ = D // L
TM = 256
NT = S // TM
RB = 16
SCALE = float(DH) ** -0.5
LOG2E = float(np.log2(np.e))

HEAD = 2
OUT_LAG = 2
LATE = (NT - OUT_LAG - 1) * TM
T_START = (-5.5, -4.5, 2.5, 36.0)
T_W = (None, 6.0, 14.0)
T_EARLY = (10.0, 15.0)
T_ROUTE = (27.0, 37.0)
T_SELECT = (38.0, 45.0)
T_FFN = (46.0, 138.0)
FFN_CUT = 640
FLAGS = None
SPLIT_FROM = NT - 1
NN = True
M_OUTER = True
MIX = False
ATT0 = 1
MS = 128
RA = 8
ATT_LAG = 1
FFN_LAG = 1
SKEW = 1.0
REV = False
ATT_DEPTH = 4
FFN_DEPTH = 4

f32, bf16, u32, i32 = jnp.float32, jnp.bfloat16, jnp.uint32, jnp.int32


class _Schedule:
    def __init__(self):
        self.items = []

    def at(self, pos, fn):
        self.items.append((pos, len(self.items), fn))

    def spread(self, t0, t1, fns):
        for n, fn in enumerate(fns):
            self.at(t0 + (n + 0.5) * (t1 - t0) / len(fns), fn)

    def pipeline(self, t0, t1, gens, depth, lag=1, warp=lambda t: t):
        step = (t1 - t0) / (len(gens) + (depth - 1) * lag)
        for n, gen in enumerate(gens):
            for s in range(depth):
                phase = (depth - s if REV else s) * SKEW / depth
                self.at(warp(t0 + (n + s * lag + 0.5 * (1 - SKEW) + phase) * step),
                        lambda gen=gen: next(gen, None))

    def emit(self):
        for _, _, fn in sorted(self.items, key=lambda it: it[:2]):
            fn()


class _Copies:
    def __init__(self, copies, totals):
        self.copies, self.totals = copies, totals

    def start(self):
        for cp in self.copies:
            cp.start()

    def wait(self):
        for cp in self.totals:
            cp.wait()


def _recip(d):
    r = pl.reciprocal(d, approx=True)
    return r * (2.0 - d * r)


def _exp_neg(z):
    return jnp.minimum(jnp.exp2(z * -LOG2E), 1e38)


def _sigmoid(z):
    return _recip(1.0 + _exp_neg(z))


def _lanes(j):
    return slice(j * L, (j + 1) * L)


def _get(ref, j, r0, n):
    return pltpu.bitcast(ref[j, pl.ds(r0 // 2, n // 2), :], bf16)


def _full_rows(ref, r0, n):
    return jnp.concatenate([_get(ref, j, r0, n) for j in range(NJ)], axis=1)


def _put(ref, j, r0, val):
    ref[j, pl.ds(r0, val.shape[0]), :] = val.astype(bf16)


def _row_dots(rows_ref, j0, r0, vec_ref, vs):
    acc = [None] * len(vs)
    for j in range(NJ):
        rows = _get(rows_ref, j0 + j, r0, RB).astype(f32)
        for n, v in enumerate(vs):
            vec = vec_ref[v, 0:8, _lanes(j)]
            t = rows * jnp.concatenate([vec, vec], axis=0)
            acc[n] = t if acc[n] is None else acc[n] + t
    return [jnp.broadcast_to(jnp.sum(a, axis=1, keepdims=True), (RB, L)) for a in acc]


def _kernel(x_hbm, wqkv_hbm, wo_hbm, wr_hbm, wg_hbm, wu_hbm, wd_hbm, gw_hbm,
            out_hbm,
            x_v, out_v, w_raw, ffn_v, gw_v, wr_v,
            wt_s, wp_v, wo_s, wop_v, gate_s, vec_s, y_s, sel_s, sems, *tiles):
    q_t, k_t, v_t, o_t = (tiles[i * NT:(i + 1) * NT] for i in range(4))
    x_w, out_w, ffn_w, wp_w, wop_w = (r.bitcast(u32) for r in (x_v, out_v, ffn_v, wp_v, wop_v))
    o_w = [r.bitcast(u32) for r in o_t]

    sem_ids = iter(range(sems.shape[0]))

    def copy(src, dst):
        return pltpu.make_async_copy(src, dst, sems.at[next(sem_ids)])

    def load(dst, r0, n, pieces):
        sem, region = sems.at[next(sem_ids)], dst.at[:, pl.ds(r0, n), :]
        return _Copies(
            [pltpu.make_async_copy(src.at[pl.ds(s0, rows), pl.ds(j * L, L)],
                                   dst.at[j0 + j, pl.ds(d0, rows), :], sem)
             for src, s0, rows, j0, d0 in pieces for j in range(NJ)],
            [pltpu.make_async_copy(region, region, sem)])

    out_sem = sems.at[next(sem_ids)]

    def store(r0, n, j):
        return pltpu.make_async_copy(
            out_v.at[j, pl.ds(r0, n), :], out_hbm.at[pl.ds(r0, n), pl.ds(j * L, L)], out_sem).start

    def w_transpose(c, kb, cb):
        def fn():
            blk = w_raw[pl.ds(kb * L, L), pl.ds(c * D + cb * L, L)].astype(f32)
            wt_s[kb, pl.ds(c * D + cb * L, L), :] = blk.T
        return fn

    def w_gather(c, j):
        def fn():
            for kb in range(NJ):
                parts = [wt_s[kb, pl.ds(c * D + 4 * j + dd, H, stride=DH), :] for dd in range(4)]
                blk = jnp.concatenate(parts, axis=0)
                _put(wp_v, kb, c * D + j * L, blk.T if NN else blk)
        return fn

    def wo_widen(nb):
        def fn():
            wo_s[nb] = _get(x_w, nb, S, D).astype(f32)
        return fn

    def wo_gather(nb):
        def fn():
            for j in range(NJ):
                parts = [wo_s[nb, pl.ds(4 * j + dd, H, stride=DH), :] for dd in range(4)]
                _put(wop_v, nb, j * L, jnp.concatenate(parts, axis=0))
        return fn

    def qkv(i, c, j, m0):
        def fn():
            w = jnp.concatenate([_get(wp_w, kb, c * D + j * L, L) for kb in range(NJ)], axis=0 if NN else 1)
            y = lax.dot_general(_full_rows(x_w, i * TM + m0, MS), w,
                                (((1,), (0 if NN else 1,)), ((), ())), preferred_element_type=f32)
            if c == 0:
                q_t[i][j, pl.ds(m0, MS), :] = y
                return
            dst = k_t if c == 1 else v_t
            dst[i][j, pl.ds(HALO + m0, MS), :] = y
            if i + 1 < NT and m0 + MS == TM:
                dst[i + 1][j, pl.ds(0, HALO), :] = y[MS - HALO:]
            if i == 0 and m0 == 0:
                dst[0][j, pl.ds(0, HALO), :] = jnp.broadcast_to(y[0:1], (HALO, L))
        return fn

    half = {}

    def attend(i, r0):
        q = [q_t[i][j, pl.ds(r0, RA), :] for j in range(NJ)]
        z = []
        for w in range(WIN):
            acc = None
            for j in range(NJ):
                t = q[j] * k_t[i][j, pl.ds(HALO + r0 - DIL * w, RA), :]
                acc = t if acc is None else acc + t
            z.append((acc, pltpu.roll(acc, 2 * H, 1)))
        yield
        z = [a + b for a, b in z]
        z = [(a, pltpu.roll(a, H, 1)) for a in z]
        yield
        z = [a + b for a, b in z]
        if i == 0 and r0 < DIL * (WIN - 1):
            pos = r0 + lax.broadcasted_iota(i32, (RA, L), 0)
            z = [jnp.where(pos >= DIL * w, z[w] * SCALE, -1e9) for w in range(WIN)]
            c = LOG2E
        else:
            c = SCALE * LOG2E
        m = z[0]
        for w in range(1, WIN):
            m = jnp.maximum(m, z[w])
        e = [jnp.exp2((z[w] - m) * c) for w in range(WIN)]
        if ATT_DEPTH == 4:
            yield
        den = e[0]
        for w in range(1, WIN):
            den = den + e[w]
        inv = _recip(den)
        for j in range(NJ):
            acc = None
            for w in range(WIN):
                t = e[w] * v_t[i][j, pl.ds(HALO + r0 - DIL * w, RA), :]
                acc = t if acc is None else acc + t
            o = acc * inv
            if RA == RB:
                _put(o_t[i], j, r0, o)
            elif r0 % RB == 0:
                half[i, j] = o
            else:
                _put(o_t[i], j, r0 - RA, jnp.concatenate([half.pop((i, j)), o], axis=0))

    def project(i, nb, m0):
        def fn():
            r0 = i * TM + m0
            a = jnp.dot(_full_rows(o_w[i], m0, MS), _get(wop_w, nb, 0, D), preferred_element_type=f32)
            g = gate_s[pl.ds(r0, MS), :]
            b = _get(x_w, nb, r0, MS).astype(f32)
            _put(out_v, nb, r0, b + g * (a - b))
        return fn

    lane = lax.broadcasted_iota(i32, (RB, L), 1)
    score = [jnp.zeros((RB, L), f32)]

    def route(n):
        g, r = _row_dots(x_w, 0, n * RB, vec_s, (0, 1))
        yield
        score[0] = jnp.where(lane == n, r, score[0])
        e = _exp_neg(g)
        yield
        gate_s[pl.ds(n * RB, RB), :] = _recip(1.0 + e)

    def row_group(ref, base, idx):
        word = pl.multiple_of(base // 2, RB // 2)
        rows = [pltpu.bitcast(ref[j, pl.ds(word, RB // 2), :], bf16) for j in range(NJ)]
        hit = lax.broadcasted_iota(i32, (RB, D), 0) == idx - base
        return jnp.concatenate(rows, axis=1).astype(f32), hit, word

    def select_top2():
        r = score[0].astype(bf16).astype(f32)
        r = jnp.where(r == 0.0, 0.0, r)
        bits = pltpu.bitcast(r, i32) >> 16
        key = jnp.where(bits < 0, bits ^ 0x7FFF, bits)
        key = jnp.where(r != r, -(1 << 15) - 1, key).astype(f32)
        row = lax.broadcasted_iota(i32, (RB, L), 0).astype(f32)
        back = (L - 1 - lane[0:1]).astype(f32)
        in_lane = []
        for _ in range(2):
            best = jnp.max(key, axis=0, keepdims=True)
            first = jnp.min(jnp.where(key == best, row, float(RB)), axis=0, keepdims=True)
            here = row == first
            in_lane.append((best * L + back, first, jnp.sum(jnp.where(here, r, 0.0), axis=0, keepdims=True)))
            key = jnp.where(here, -float(1 << 16), key)
        top = jnp.max(in_lane[0][0], axis=1, keepdims=True)
        yield
        won = in_lane[0][0] == top
        rest = [jnp.where(won, b, a) for a, b in zip(*in_lane)]
        top = jnp.max(rest[0], axis=1, keepdims=True)
        yield
        picks = []
        for cand, hit in ((in_lane[0], won), (rest, rest[0] == top)):
            pos = (L - 1 - back) * RB + cand[1]
            picks.append([jnp.sum(jnp.where(hit, v, 0.0), axis=1, keepdims=True) for v in (pos, cand[2])])
        yield
        ids = [jnp.clip(pos.astype(i32)[0, 0], 0, S - 1) for pos, _ in picks]
        yield
        for t, idx in enumerate(ids):
            sel_s[t] = idx
            vec_s[4 + t, :, 0:L] = _sigmoid(jnp.broadcast_to(picks[t][1], (RB, L)))
            grp, hit, _ = row_group(x_w, (idx // RB) * RB, idx)
            vec_s[2 + t] = jnp.broadcast_to(
                jnp.sum(jnp.where(hit, grp, 0.0), axis=0, keepdims=True), (RB, D))

    y_acc = {}

    def ffn(f0):
        gp = _row_dots(ffn_w, 0, f0, vec_s, (2, 3))
        up = _row_dots(ffn_w, NJ, f0, vec_s, (2, 3))
        yield
        e = [_exp_neg(a) for a in gp]
        if FFN_DEPTH >= 3:
            yield
        sig = [_recip(1.0 + a) for a in e]
        if FFN_DEPTH >= 4:
            yield
        h = [gp[t] * sig[t] * up[t] for t in range(2)]
        for j in range(NJ):
            wd = _get(ffn_w, 2 * NJ + j, f0, RB).astype(f32)
            for t in range(2):
                p = h[t] * wd
                p = p[0:8] + p[8:16]
                y_acc[t, j] = y_acc[t, j] + p if (t, j) in y_acc else p

    def ffn_finish():
        for t in range(2):
            for j in range(NJ):
                y = jnp.sum(y_acc[t, j], axis=0, keepdims=True)
                y_s[t, :, _lanes(j)] = jnp.broadcast_to(y, (RB, L)) * vec_s[4 + t, :, 0:L]

    def add_to_row(ref, base, idx, term):
        old, hit, word = row_group(ref, base, idx)
        new = jnp.where(hit, old + term, old).astype(bf16)
        for j in range(NJ):
            ref[j, pl.ds(word, RB // 2), :] = pltpu.bitcast(new[:, _lanes(j)], u32)

    def patch_output(t):
        idx = sel_s[t]
        g = _sigmoid(jnp.sum(vec_s[2 + t] * vec_s[0], axis=1, keepdims=True))
        add_to_row(out_w, jnp.minimum((idx // RB) * RB, LATE - RB), idx, (1.0 - g) * y_s[t])

    def patch_residual(t):
        idx = sel_s[t]
        add_to_row(x_w, (idx // RB) * RB, idx, y_s[t])

    sch = _Schedule()
    halves = range(0, TM, MS)
    mxu = [("qkv", i, c, j, m0) for c in range(3) for i in range(HEAD) for m0 in halves for j in range(NJ)]
    for i in range(HEAD, NT + OUT_LAG):
        if M_OUTER:
            fwd = [[("qkv", i, c, j, m0)] for m0 in halves for c in range(3) for j in range(NJ)]
            out = [[("out", i - OUT_LAG, nb, m0)] for m0 in halves for nb in range(NJ)]
        else:
            fwd = [[("qkv", i, c, j, m0) for m0 in halves] for c in range(3) for j in range(NJ)]
            out = [[("out", i - OUT_LAG, nb, m0) for m0 in halves] for nb in range(NJ)]
        if i >= NT:
            fwd = []
        if MIX and fwd:
            fwd, out = [g for n in range(len(out)) for g in fwd[3 * n:3 * n + 3] + [out[n]]], []
        mxu += [op for g in fwd + out for op in g]
    dt = MS / 256
    slot = {op: n * dt for n, op in enumerate(mxu)}
    for op, t in slot.items():
        sch.at(t, (qkv if op[0] == "qkv" else project)(*op[1:]))

    cp_w0 = [copy(wqkv_hbm.at[pl.ds(kb * L, L), pl.ds(0, D)], w_raw.at[pl.ds(kb * L, L), pl.ds(0, D)])
             for kb in range(NJ)]
    cp_w = {c: copy(wqkv_hbm.at[:, pl.ds(c * D, D)], w_raw.at[:, pl.ds(c * D, D)]) for c in (1, 2)}
    cp_vec = [copy(gw_hbm, gw_v), copy(wr_hbm, wr_v)]
    rest = HEAD * TM
    cp_x = [load(x_v, 0, MS, [(x_hbm, 0, MS, 0, 0)]),
            load(x_v, MS, rest - MS, [(x_hbm, MS, rest - MS, 0, MS)]),
            load(x_v, rest, S + D - rest, [(x_hbm, rest, S - rest, 0, rest), (wo_hbm, 0, D, 0, S)])]
    cp_f = [load(ffn_v, r0, n, [(src, r0, n, m * NJ, r0) for m, src in enumerate((wg_hbm, wu_hbm, wd_hbm))])
            for r0, n in ((0, FFN_CUT), (FFN_CUT, F - FFN_CUT))]
    for cp in [cp_x[0]] + cp_w0 + cp_vec:
        sch.at(-9, cp.start)
    for cp in cp_vec:
        sch.at(-4.5, cp.wait)
    sch.at(-8.5, cp_x[0].wait)
    for kb in range(NJ):
        sch.at(-8 + kb, cp_w0[kb].wait)
        sch.spread(-8 + kb, -7 + kb, [w_transpose(0, kb, cb) for cb in range(NJ)])
    for pos, starts, waits in (
            (T_START[0], (cp_x[1],), ()),
            (T_START[1], (cp_w[1],), ()),
            (NJ * dt - 0.1, (), (cp_x[1],)),
            (T_START[2], (cp_w[2],), ()),
            (T_W[1], (cp_x[2],), (cp_w[1],)),
            (T_W[2], (), (cp_w[2],)),
            (T_ROUTE[0], (cp_f[0],), (cp_x[2],)),
            (T_START[3], (cp_f[1],), ()),
            (T_FFN[0], (), (cp_f[0],)),
            (T_FFN[0] + (T_FFN[1] - T_FFN[0]) * FFN_CUT / F - 2, (), (cp_f[1],))):
        for cp in starts:
            sch.at(pos, cp.start)
        for cp in waits:
            sch.at(pos, cp.wait)

    for c in range(3):
        first = slot["qkv", 0, c, 0, 0]
        if c > 0:
            sch.spread(T_W[c], first - 0.8,
                       [w_transpose(c, kb, cb) for cb in range(NJ) for kb in range(NJ)])
        for j in range(NJ):
            sch.at(first + (j - 1.4) * dt, w_gather(c, j))
    first = slot["out", 0, 0, 0]
    sch.spread(T_ROUTE[0], min(first - 0.5, T_ROUTE[0] + 10), [fn for nb in range(NJ) for fn in (wo_widen(nb), wo_gather(nb))])

    def vectors():
        for n, ref in enumerate((gw_v, wr_v)):
            vec_s[n] = jnp.broadcast_to(ref[...].astype(f32).reshape(1, D), (RB, D))

    sch.at(5, vectors)
    early = HEAD * TM // RB
    sch.pipeline(*T_EARLY, [route(n) for n in range(early)], 3, 2)
    sch.pipeline(*T_ROUTE, [route(n) for n in range(early, S // RB)], 3, 2)
    picker = select_top2()
    sch.spread(*T_SELECT, [lambda: next(picker, None)] * 5)

    t0 = 0
    for i in range(NT):
        t0 = max(t0, slot["qkv", max(i, ATT0), 2, NJ - 1, TM - MS] + dt)
        t1 = t0 + min((slot["out", n, 0, 0] - 0.5 - t0) / (n - i + 1) for n in range(i, NT))
        sch.pipeline(t0, t1, [attend(i, r0) for r0 in range(0, TM, RA)], ATT_DEPTH, ATT_LAG)
        t0 = t1

    t0, t1 = T_FFN
    sch.pipeline(t0, t1, [ffn(f0) for f0 in range(0, F, RB)], FFN_DEPTH, FFN_LAG)
    sch.at(t1 + 0.1, ffn_finish)

    for t in range(2):
        sch.at(t1 + 1 + t, lambda t=t: patch_output(t))
        sch.at(slot["qkv", NT - 1, 2, NJ - 1, TM - MS] + 0.1, lambda t=t: patch_residual(t))
    for j in range(NJ):
        sch.at(t1 + 3.5, store(0, LATE, j))
    for op, t in slot.items():
        if op[0] == "out" and op[1] * TM >= LATE:
            if op[1] >= SPLIT_FROM:
                sch.at(t + 0.75, store(op[1] * TM + op[3], MS, op[2]))
            elif op[3] == TM - MS:
                sch.at(t + 0.75, store(op[1] * TM, TM, op[2]))
    sch.at(len(mxu), pltpu.make_async_copy(out_v, out_v, out_sem).wait)
    sch.emit()


@jax.jit
def pallas_gated_mix__sliding_local_dilated__moe_arch_mod__prompt_kernel(
    A_x: jax.Array,
    A_wqkv: jax.Array,
    A_wo: jax.Array,
    B_x: jax.Array,
    B_w_r: jax.Array,
    B_w_gate: jax.Array,
    B_w_up: jax.Array,
    B_w_down: jax.Array,
    gate_w: jax.Array,
):
    n_sems = 1 + NJ + 2 + 2 + 3 + 2
    scratch = [
        pltpu.VMEM((NJ, S + D, L), bf16),
        pltpu.VMEM((NJ, S, L), bf16),
        pltpu.VMEM((D, 3 * D), bf16),
        pltpu.VMEM((3 * NJ, F, L), bf16),
        pltpu.VMEM((D,), bf16),
        pltpu.VMEM((D,), bf16),
        pltpu.VMEM((NJ, 3 * D, L), f32),
        pltpu.VMEM((NJ, 3 * D, L), bf16),
        pltpu.VMEM((NJ, D, L), f32),
        pltpu.VMEM((NJ, D, L), bf16),
        pltpu.VMEM((S, L), f32),
        pltpu.VMEM((6, RB, D), f32),
        pltpu.VMEM((2, RB, D), f32),
        pltpu.SMEM((2,), i32),
        pltpu.SemaphoreType.DMA((n_sems,)),
    ]
    scratch += [pltpu.VMEM((NJ, TM, L), f32)] * NT
    scratch += [pltpu.VMEM((NJ, HALO + TM, L), f32)] * (2 * NT)
    scratch += [pltpu.VMEM((NJ, TM, L), bf16)] * NT
    out = pl.pallas_call(
        _kernel,
        out_shape=jax.ShapeDtypeStruct((S, D), bf16),
        in_specs=[pl.BlockSpec(memory_space=pl.ANY)] * 8,
        out_specs=pl.BlockSpec(memory_space=pl.ANY),
        scratch_shapes=scratch,
        compiler_params=pltpu.CompilerParams(vmem_limit_bytes=100 * 2**20, flags=FLAGS),
        name="gated_mix",
    )(A_x.reshape(S, D), A_wqkv, A_wo, B_w_r,
      B_w_gate.T, B_w_up.T, B_w_down, gate_w)
    return out.reshape(1, S, D)
```

```python
import numpy as np

import jax
import jax.numpy as jnp
from jax import lax
import jax.experimental.pallas as pl
import jax.experimental.pallas.tpu as pltpu

S, D, F = 2048, 640, 1728
H, DH = 32, 20
WIN, DIL = 8, 2
HALO = 16
L = 128
NJ = D // L
TM = 256
NT = S // TM
MS = 128
RA = 8
RB = 16
SCALE = float(DH) ** -0.5
LOG2E = float(np.log2(np.e))

HEAD = 2
OUT_LAG = 2
LATE = (NT - OUT_LAG - 1) * TM
T_START = (-5.5, -4.5, 2.5, 36.0)
T_W = (None, 6.0, 14.0)
T_EARLY = (10.0, 15.0)
T_ROUTE = (27.0, 37.0)
T_SELECT = (38.0, 45.0)
T_FFN = (46.0, 138.0)
FFN_CUT = 640

f32, bf16, u32, i32 = jnp.float32, jnp.bfloat16, jnp.uint32, jnp.int32


class _Schedule:
    def __init__(self):
        self.items = []

    def at(self, pos, fn):
        self.items.append((pos, len(self.items), fn))

    def spread(self, t0, t1, fns):
        for n, fn in enumerate(fns):
            self.at(t0 + (n + 0.5) * (t1 - t0) / len(fns), fn)

    def pipeline(self, t0, t1, gens, depth, lag=1):
        step = (t1 - t0) / (len(gens) + (depth - 1) * lag)
        for n, gen in enumerate(gens):
            for s in range(depth):
                self.at(t0 + (n + s * lag + s / depth) * step, lambda gen=gen: next(gen, None))

    def emit(self):
        for _, _, fn in sorted(self.items, key=lambda it: it[:2]):
            fn()


class _Copies:
    def __init__(self, copies, totals):
        self.copies, self.totals = copies, totals

    def start(self):
        for cp in self.copies:
            cp.start()

    def wait(self):
        for cp in self.totals:
            cp.wait()


def _recip(d):
    r = pl.reciprocal(d, approx=True)
    return r * (2.0 - d * r)


def _exp_neg(z):
    return jnp.minimum(jnp.exp2(z * -LOG2E), 1e38)


def _sigmoid(z):
    return _recip(1.0 + _exp_neg(z))


def _lanes(j):
    return slice(j * L, (j + 1) * L)


def _get(ref, j, r0, n):
    return pltpu.bitcast(ref[j, pl.ds(r0 // 2, n // 2), :], bf16)


def _full_rows(ref, r0, n):
    return jnp.concatenate([_get(ref, j, r0, n) for j in range(NJ)], axis=1)


def _put(ref, j, r0, val):
    ref[j, pl.ds(r0, val.shape[0]), :] = val.astype(bf16)


def _row_dots(rows_ref, j0, r0, vec_ref, vs):
    acc = [None] * len(vs)
    for j in range(NJ):
        rows = _get(rows_ref, j0 + j, r0, RB).astype(f32)
        for n, v in enumerate(vs):
            vec = vec_ref[v, 0:8, _lanes(j)]
            t = rows * jnp.concatenate([vec, vec], axis=0)
            acc[n] = t if acc[n] is None else acc[n] + t
    return [jnp.broadcast_to(jnp.sum(a, axis=1, keepdims=True), (RB, L)) for a in acc]


def _kernel(x_hbm, wqkv_hbm, wo_hbm, wr_hbm, wg_hbm, wu_hbm, wd_hbm, gw_hbm,
            out_hbm,
            x_v, out_v, w_raw, ffn_v, gw_v, wr_v,
            wt_s, wp_v, wo_s, wop_v, gate_s, vec_s, y_s, sel_s, sems, *tiles):
    q_t, k_t, v_t, o_t = (tiles[i * NT:(i + 1) * NT] for i in range(4))
    x_w, out_w, ffn_w, wp_w, wop_w = (r.bitcast(u32) for r in (x_v, out_v, ffn_v, wp_v, wop_v))
    o_w = [r.bitcast(u32) for r in o_t]

    sem_ids = iter(range(sems.shape[0]))

    def copy(src, dst):
        return pltpu.make_async_copy(src, dst, sems.at[next(sem_ids)])

    def load(dst, r0, n, pieces):
        sem, region = sems.at[next(sem_ids)], dst.at[:, pl.ds(r0, n), :]
        return _Copies(
            [pltpu.make_async_copy(src.at[pl.ds(s0, rows), pl.ds(j * L, L)],
                                   dst.at[j0 + j, pl.ds(d0, rows), :], sem)
             for src, s0, rows, j0, d0 in pieces for j in range(NJ)],
            [pltpu.make_async_copy(region, region, sem)])

    out_sem = sems.at[next(sem_ids)]

    def store(r0, n, j):
        return pltpu.make_async_copy(
            out_v.at[j, pl.ds(r0, n), :], out_hbm.at[pl.ds(r0, n), pl.ds(j * L, L)], out_sem).start

    def w_transpose(c, kb, cb):
        def fn():
            blk = w_raw[pl.ds(kb * L, L), pl.ds(c * D + cb * L, L)].astype(f32)
            wt_s[kb, pl.ds(c * D + cb * L, L), :] = blk.T
        return fn

    def w_gather(c, j):
        def fn():
            for kb in range(NJ):
                parts = [wt_s[kb, pl.ds(c * D + 4 * j + dd, H, stride=DH), :] for dd in range(4)]
                blk = jnp.concatenate(parts, axis=0)
                _put(wp_v, kb, c * D + j * L, blk.T)
        return fn

    def wo_widen(nb):
        def fn():
            wo_s[nb, pl.ds(0, D), :] = _get(x_w, nb, S, D).astype(f32)
        return fn

    def wo_gather(nb):
        def fn():
            for j in range(NJ):
                parts = [wo_s[nb, pl.ds(4 * j + dd, H, stride=DH), :] for dd in range(4)]
                _put(wop_v, nb, j * L, jnp.concatenate(parts, axis=0))
        return fn

    def qkv(i, c, j, m0):
        def fn():
            w = jnp.concatenate([_get(wp_w, kb, c * D + j * L, L) for kb in range(NJ)], axis=0)
            y = jnp.dot(_full_rows(x_w, i * TM + m0, MS), w, preferred_element_type=f32)
            if c == 0:
                q_t[i][j, pl.ds(m0, MS), :] = y
                return
            dst = k_t if c == 1 else v_t
            dst[i][j, pl.ds(HALO + m0, MS), :] = y
            if i + 1 < NT and m0 + MS == TM:
                dst[i + 1][j, pl.ds(0, HALO), :] = y[MS - HALO:]
            if i == 0 and m0 == 0:
                dst[0][j, pl.ds(0, HALO), :] = jnp.broadcast_to(y[0:1], (HALO, L))
        return fn

    half = {}

    def attend(i, r0):
        q = [q_t[i][j, pl.ds(r0, RA), :] for j in range(NJ)]
        acc = {}
        for j in range(NJ):
            for w in range(WIN):
                t = q[j] * k_t[i][j, pl.ds(HALO + r0 - DIL * w, RA), :]
                acc[w] = acc[w] + t if j else t
                if j == NJ - 1:
                    acc[w] = (acc[w], pltpu.roll(acc[w], 2 * H, 1))
        z = [acc[w] for w in range(WIN)]
        yield
        z = [a + b for a, b in z]
        z = [(a, pltpu.roll(a, H, 1)) for a in z]
        yield
        z = [a + b for a, b in z]
        if i == 0 and r0 < DIL * (WIN - 1):
            pos = r0 + lax.broadcasted_iota(i32, (RA, L), 0)
            z = [jnp.where(pos >= DIL * w, z[w] * SCALE, -1e9) for w in range(WIN)]
            c = LOG2E
        else:
            c = SCALE * LOG2E
        m = z[0]
        for w in range(1, WIN):
            m = jnp.maximum(m, z[w])
        e = [jnp.exp2((z[w] - m) * c) for w in range(WIN)]
        yield
        den = e[0]
        for w in range(1, WIN):
            den = den + e[w]
        inv = _recip(den)
        for j in range(NJ):
            for w in range(WIN):
                t = e[w] * v_t[i][j, pl.ds(HALO + r0 - DIL * w, RA), :]
                o = o + t if w else t
            if r0 % RB == 0:
                half[i, j] = o * inv
            else:
                _put(o_t[i], j, r0 - RA, jnp.concatenate([half.pop((i, j)), o * inv], axis=0))

    def project(i, nb, m0):
        def fn():
            r0 = i * TM + m0
            a = jnp.dot(_full_rows(o_w[i], m0, MS), _get(wop_w, nb, 0, D), preferred_element_type=f32)
            g = gate_s[pl.ds(r0, MS), :]
            b = _get(x_w, nb, r0, MS).astype(f32)
            _put(out_v, nb, r0, b + g * (a - b))
        return fn

    lane = lax.broadcasted_iota(i32, (RB, L), 1)
    score = [jnp.zeros((RB, L), f32)]

    def route(n):
        g, r = _row_dots(x_w, 0, n * RB, vec_s, (0, 1))
        yield
        score[0] = jnp.where(lane == n, r, score[0])
        e = _exp_neg(g)
        yield
        gate_s[pl.ds(n * RB, RB), :] = _recip(1.0 + e)

    def row_group(ref, base, idx):
        word = pl.multiple_of(base // 2, RB // 2)
        rows = [pltpu.bitcast(ref[j, pl.ds(word, RB // 2), :], bf16) for j in range(NJ)]
        hit = lax.broadcasted_iota(i32, (RB, D), 0) == idx - base
        return jnp.concatenate(rows, axis=1).astype(f32), hit, word

    def select_top2():
        r = score[0].astype(bf16).astype(f32)
        r = jnp.where(r == 0.0, 0.0, r)
        bits = pltpu.bitcast(r, i32) >> 16
        key = jnp.where(bits < 0, bits ^ 0x7FFF, bits)
        key = jnp.where(r != r, -(1 << 15) - 1, key).astype(f32)
        row = lax.broadcasted_iota(i32, (RB, L), 0).astype(f32)
        back = (L - 1 - lane[0:1]).astype(f32)
        in_lane = []
        for _ in range(2):
            best = jnp.max(key, axis=0, keepdims=True)
            first = jnp.min(jnp.where(key == best, row, float(RB)), axis=0, keepdims=True)
            here = row == first
            in_lane.append((best * L + back, first, jnp.sum(jnp.where(here, r, 0.0), axis=0, keepdims=True)))
            key = jnp.where(here, -float(1 << 16), key)
        top = jnp.max(in_lane[0][0], axis=1, keepdims=True)
        yield
        won = in_lane[0][0] == top
        rest = [jnp.where(won, b, a) for a, b in zip(*in_lane)]
        top = jnp.max(rest[0], axis=1, keepdims=True)
        yield
        picks = []
        for cand, hit in ((in_lane[0], won), (rest, rest[0] == top)):
            pos = (L - 1 - back) * RB + cand[1]
            picks.append([jnp.sum(jnp.where(hit, v, 0.0), axis=1, keepdims=True) for v in (pos, cand[2])])
        yield
        ids = [jnp.clip(pos.astype(i32)[0, 0], 0, S - 1) for pos, _ in picks]
        yield
        for t, idx in enumerate(ids):
            sel_s[t] = idx
            vec_s[4 + t, :, 0:L] = _sigmoid(jnp.broadcast_to(picks[t][1], (RB, L)))
            grp, hit, _ = row_group(x_w, (idx // RB) * RB, idx)
            vec_s[2 + t] = jnp.broadcast_to(
                jnp.sum(jnp.where(hit, grp, 0.0), axis=0, keepdims=True), (RB, D))

    y_acc = {}

    def ffn(f0):
        gp = _row_dots(ffn_w, 0, f0, vec_s, (2, 3))
        up = _row_dots(ffn_w, NJ, f0, vec_s, (2, 3))
        yield
        e = [_exp_neg(a) for a in gp]
        yield
        sig = [_recip(1.0 + a) for a in e]
        yield
        h = [gp[t] * sig[t] * up[t] for t in range(2)]
        for j in range(NJ):
            wd = _get(ffn_w, 2 * NJ + j, f0, RB).astype(f32)
            for t in range(2):
                p = h[t] * wd
                p = p[0:8] + p[8:16]
                y_acc[t, j] = y_acc[t, j] + p if (t, j) in y_acc else p

    def ffn_finish():
        for t in range(2):
            for j in range(NJ):
                y = jnp.sum(y_acc[t, j], axis=0, keepdims=True)
                y_s[t, :, _lanes(j)] = jnp.broadcast_to(y, (RB, L)) * vec_s[4 + t, :, 0:L]

    def add_to_row(ref, base, idx, term):
        old, hit, word = row_group(ref, base, idx)
        new = jnp.where(hit, old + term, old).astype(bf16)
        for j in range(NJ):
            ref[j, pl.ds(word, RB // 2), :] = pltpu.bitcast(new[:, _lanes(j)], u32)

    def patch_output(t):
        idx = sel_s[t]
        g = _sigmoid(jnp.sum(vec_s[2 + t] * vec_s[0], axis=1, keepdims=True))
        add_to_row(out_w, jnp.minimum((idx // RB) * RB, LATE - RB), idx, (1.0 - g) * y_s[t])

    def patch_residual(t):
        idx = sel_s[t]
        add_to_row(x_w, (idx // RB) * RB, idx, y_s[t])

    sch = _Schedule()
    halves = range(0, TM, MS)
    mxu = [("qkv", i, c, j, m0) for c in range(3) for i in range(HEAD) for m0 in halves for j in range(NJ)]
    for i in range(HEAD, NT + OUT_LAG):
        if i < NT:
            mxu += [("qkv", i, c, j, m0) for m0 in halves for c in range(3) for j in range(NJ)]
        if i >= OUT_LAG:
            mxu += [("out", i - OUT_LAG, nb, m0) for m0 in halves for nb in range(NJ)]
    dt = MS / 256
    slot = {op: n * dt for n, op in enumerate(mxu)}
    for op, t in slot.items():
        sch.at(t, (qkv if op[0] == "qkv" else project)(*op[1:]))

    cp_w0 = [copy(wqkv_hbm.at[pl.ds(kb * L, L), pl.ds(0, D)], w_raw.at[pl.ds(kb * L, L), pl.ds(0, D)])
             for kb in range(NJ)]
    cp_w = {c: copy(wqkv_hbm.at[:, pl.ds(c * D, D)], w_raw.at[:, pl.ds(c * D, D)]) for c in (1, 2)}
    cp_vec = [copy(gw_hbm, gw_v), copy(wr_hbm, wr_v)]
    rest = HEAD * TM
    cp_x = [load(x_v, 0, MS, [(x_hbm, 0, MS, 0, 0)]),
            load(x_v, MS, rest - MS, [(x_hbm, MS, rest - MS, 0, MS)]),
            load(x_v, rest, S + D - rest, [(x_hbm, rest, S - rest, 0, rest), (wo_hbm, 0, D, 0, S)])]
    cp_f = [load(ffn_v, r0, n, [(src, r0, n, m * NJ, r0) for m, src in enumerate((wg_hbm, wu_hbm, wd_hbm))])
            for r0, n in ((0, FFN_CUT), (FFN_CUT, F - FFN_CUT))]
    for cp in [cp_x[0]] + cp_w0 + cp_vec:
        sch.at(-9, cp.start)
    sch.at(-8.5, cp_x[0].wait)
    for kb in range(NJ):
        sch.at(-8 + kb, cp_w0[kb].wait)
        sch.spread(-8 + kb, -7 + kb, [w_transpose(0, kb, cb) for cb in range(NJ)])
    for pos, starts, waits in (
            (T_START[0], (cp_x[1],), ()),
            (T_START[1], (cp_w[1],), ()),
            (NJ * dt - 0.1, (), (*cp_vec, cp_x[1])),
            (T_START[2], (cp_w[2],), ()),
            (T_W[1], (cp_x[2],), (cp_w[1],)),
            (T_W[2], (), (cp_w[2],)),
            (T_ROUTE[0], (cp_f[0],), (cp_x[2],)),
            (T_START[3], (cp_f[1],), ()),
            (T_FFN[0], (), (cp_f[0],)),
            (T_FFN[0] + (T_FFN[1] - T_FFN[0]) * FFN_CUT / F - 2, (), (cp_f[1],))):
        for cp in starts:
            sch.at(pos, cp.start)
        for cp in waits:
            sch.at(pos, cp.wait)

    for c in range(3):
        first = slot["qkv", 0, c, 0, 0]
        if c > 0:
            sch.spread(T_W[c], first - 0.8,
                       [w_transpose(c, kb, cb) for cb in range(NJ) for kb in range(NJ)])
        for j in range(NJ):
            sch.at(first + (j - 1.4) * dt, w_gather(c, j))
    first = slot["out", 0, 0, 0]
    sch.spread(T_ROUTE[0], min(first - 0.5, T_ROUTE[0] + 10), [fn for nb in range(NJ) for fn in (wo_widen(nb), wo_gather(nb))])

    def vectors():
        for n, ref in enumerate((gw_v, wr_v)):
            vec_s[n] = jnp.broadcast_to(ref[...].astype(f32).reshape(1, D), (RB, D))

    sch.at(5, vectors)
    early = HEAD * TM // RB
    sch.pipeline(*T_EARLY, [route(n) for n in range(early)], 3, 2)
    sch.pipeline(*T_ROUTE, [route(n) for n in range(early, S // RB)], 3, 2)
    picker = select_top2()
    sch.spread(*T_SELECT, [lambda: next(picker, None)] * 5)

    t0 = 0
    for i in range(NT):
        t0 = max(t0, slot["qkv", max(i, HEAD - 1), 2, NJ - 1, TM - MS] + dt)
        t1 = t0 + min((slot["out", n, 0, 0] - 0.5 - t0) / (n - i + 1) for n in range(i, NT))
        sch.pipeline(t0, t1, [attend(i, r0) for r0 in range(0, TM, RA)], 4)
        t0 = t1

    t0, t1 = T_FFN
    sch.pipeline(t0, t1, [ffn(f0) for f0 in range(0, F, RB)], 4)
    sch.at(t1 + 0.1, ffn_finish)

    for t in range(2):
        sch.at(t1 + 1 + t, lambda t=t: patch_output(t))
        sch.at(slot["qkv", NT - 1, 2, NJ - 1, TM - MS] + 0.1, lambda t=t: patch_residual(t))
    for j in range(NJ):
        sch.at(t1 + 3.5, store(0, LATE, j))
    for op, t in slot.items():
        if op[0] == "out" and op[1] * TM >= LATE:
            if op[1] == NT - 1:
                sch.at(t + 0.75, store(op[1] * TM + op[3], MS, op[2]))
            elif op[3] == TM - MS:
                sch.at(t + 0.75, store(op[1] * TM, TM, op[2]))
    sch.at(len(mxu), pltpu.make_async_copy(out_v, out_v, out_sem).wait)
    sch.emit()


@jax.jit
def pallas_gated_mix__sliding_local_dilated__moe_arch_mod__prompt_kernel(
    A_x: jax.Array,
    A_wqkv: jax.Array,
    A_wo: jax.Array,
    B_x: jax.Array,
    B_w_r: jax.Array,
    B_w_gate: jax.Array,
    B_w_up: jax.Array,
    B_w_down: jax.Array,
    gate_w: jax.Array,
):
    n_sems = 1 + NJ + 2 + 2 + 3 + 2
    scratch = [
        pltpu.VMEM((NJ, S + D, L), bf16),
        pltpu.VMEM((NJ, S, L), bf16),
        pltpu.VMEM((D, 3 * D), bf16),
        pltpu.VMEM((3 * NJ, F, L), bf16),
        pltpu.VMEM((D,), bf16),
        pltpu.VMEM((D,), bf16),
        pltpu.VMEM((NJ, 3 * D + 24, L), f32),
        pltpu.VMEM((NJ, 3 * D, L), bf16),
        pltpu.VMEM((NJ, D + 24, L), f32),
        pltpu.VMEM((NJ, D, L), bf16),
        pltpu.VMEM((S, L), f32),
        pltpu.VMEM((6, RB, D), f32),
        pltpu.VMEM((2, RB, D), f32),
        pltpu.SMEM((2,), i32),
        pltpu.SemaphoreType.DMA((n_sems,)),
    ]
    scratch += [pltpu.VMEM((NJ, TM, L), f32)] * NT
    scratch += [pltpu.VMEM((NJ, HALO + TM, L), f32)] * (2 * NT)
    scratch += [pltpu.VMEM((NJ, TM, L), bf16)] * NT
    out = pl.pallas_call(
        _kernel,
        out_shape=jax.ShapeDtypeStruct((S, D), bf16),
        in_specs=[pl.BlockSpec(memory_space=pl.ANY)] * 8,
        out_specs=pl.BlockSpec(memory_space=pl.ANY),
        scratch_shapes=scratch,
        compiler_params=pltpu.CompilerParams(vmem_limit_bytes=100 * 2**20),
        name="gated_mix",
    )(A_x.reshape(S, D), A_wqkv, A_wo, B_w_r,
      B_w_gate.T, B_w_up.T, B_w_down, gate_w)
    return out.reshape(1, S, D)
```
